```python
import os as _os
_os.environ.setdefault("JAX_PLATFORMS", "cpu")
import jax
import jax.numpy as jnp

def _softmax(x, axis=-1):
    return jax.nn.softmax(x, axis=axis)
def _gelu(x):
    return jax.nn.gelu(x, approximate=True)
def _silu(x):
    return jax.nn.silu(x)
def _sigmoid(x):
    return jax.nn.sigmoid(x)
def _layernorm(x, axis=-1, eps=1e-5):
    m = jnp.mean(x, axis=axis, keepdims=True)
    v = jnp.var(x, axis=axis, keepdims=True)
    return (x - m) / jnp.sqrt(v + eps)
def _scatter_add(tgt, idx, src, axis=0):
    return tgt.at[idx].add(src)
def _segment_sum(src, seg, n):
    return jax.ops.segment_sum(src, seg, n)
class _Rng:
    def __init__(self, key):
        self._k = key
    def _next(self):
        self._k, sub = jax.random.split(self._k)
        return sub
    def normal(self, shape):
        return jax.random.normal(self._next(), shape, dtype=jnp.bfloat16)
    def randint(self, lo, hi, shape):
        return jax.random.randint(self._next(), shape, lo, hi, dtype=jnp.int32)
    def uniform(self, shape, lo=0.0, hi=1.0):
        return jax.random.uniform(self._next(), shape, jnp.bfloat16, lo, hi)
    def permutation(self, n):
        return jax.random.permutation(self._next(), n)


kernel_name = 'concat_heads__spectral_gfnet__mha_block__prompt'

def setup_inputs():
    _rng = _Rng(jax.random.key(int.from_bytes(__import__("os").urandom(4), "little")))
    _w = (lambda a: (lambda t: t.astype(jnp.bfloat16) if jnp.issubdtype(t.dtype, jnp.floating) else t)(jnp.asarray(a)))
    def _A_setup():
        B, S, D = 1, 2048, 576
        Df = D // 2 + 1
        return {
            "x": _w((lambda *s: _rng.normal(s) * 0.05)(B, S, D)),
            "w_r": _w((lambda *s: _rng.normal(s) * 0.05)(S, Df) * 0.02),
            "w_i": _w((lambda *s: _rng.normal(s) * 0.05)(S, Df) * 0.02),
        }
    _A_in = _A_setup()

    def _B_setup():
        B, S, D, H = 1, 2048, 576, 32
        return {
            "x": _w((lambda *s: _rng.normal(s) * 0.1)(B, S, D)),
            "wqkv": _w((lambda *s: _rng.normal(s) * 0.1)(D, 3 * D)),
            "wo": _w((lambda *s: _rng.normal(s) * 0.05)(D, D)),
        }
    _B_in = _B_setup()

    return {
        "A_x": _A_in["x"],
        "A_w_r": _A_in["w_r"],
        "A_w_i": _A_in["w_i"],
        "B_x": _B_in["x"],
        "B_wqkv": _B_in["wqkv"],
        "B_wo": _B_in["wo"],
    }

def reference(A_x, A_w_r, A_w_i, B_x, B_wqkv, B_wo):
    def _A_ref(x, w_r, w_i):
        B, S, D = x.shape
        X = (lambda x, axes=(-2,-1): jnp.fft.rfft2(x.astype(jnp.float32), axes=axes))(x, axes=(-2, -1))
        W = w_r + 1j * w_i
        X = X * W
        y = (lambda x, s, axes=(-2,-1): jnp.fft.irfft2(x, s=s, axes=axes).astype(jnp.bfloat16))(X, (S, D), axes=(-2, -1))
        return y

    def _B_ref(x, wqkv, wo):
        B, S, D = x.shape
        H = 32
        Dh = D // H
        qkv = (lambda x, *d: x.transpose(*d))((x @ wqkv).reshape(B, S, 3, H, Dh), 2, 0, 3, 1, 4)
        q, k, v = qkv[0], qkv[1], qkv[2]
        scores = jnp.einsum("bhqd,bhkd->bhqk", q, k) * (Dh ** -0.5)
        p = _softmax(scores, axis=-1)
        o = jnp.einsum("bhqk,bhkd->bhqd", p, v)
        return (lambda x, *d: x.transpose(*d))(o, 0, 2, 1, 3).reshape(B, S, D) @ wo

    a = _A_ref(A_x, A_w_r, A_w_i)
    b = _B_ref(B_x, B_wqkv, B_wo)
    return jnp.concatenate([a, b], axis=-1)
```

```python
import functools, math
import numpy as np
import jax, jax.numpy as jnp
from jax.experimental import pallas as pl
from jax.experimental.pallas import tpu as pltpu

S, D, H, DH = 2048, 576, 32, 18
DF = D // 2 + 1
R = 304
N1, N2 = 16, 128
LOG2E = 1.4426950408889634
BF = jnp.bfloat16
F32 = jnp.float32


def _consts():
    f = np.arange(R)[:, None].astype(np.float64)
    d = np.arange(D)[None, :].astype(np.float64)
    valid = (f < DF)
    ang = 2 * np.pi * ((f * d) % D) / D
    f1 = np.concatenate([np.where(valid, np.cos(ang), 0.0), np.where(valid, -np.sin(ang), 0.0)], axis=0)
    cf = np.where((f == 0) | (f == DF - 1), 1.0, 2.0) / (S * D)
    finv = np.concatenate([np.where(valid, cf * np.cos(ang), 0.0), np.where(valid, -cf * np.sin(ang), 0.0)], axis=0)
    finv = np.pad(finv, ((0, 0), (0, 64)))
    n2 = np.arange(N2)[:, None]
    k2 = np.arange(N2)[None, :]
    ms = []
    for k1 in range(N1):
        th = 2 * np.pi * ((n2 * (k1 + N1 * k2)) % S) / S
        c, s = np.cos(th), np.sin(th)
        ms.append(np.block([[c, -s], [s, c]]))
    m = np.stack(ms)
    return (jnp.asarray(f1, BF), jnp.asarray(m, BF), jnp.asarray(finv, BF))


def _cmul_const(a, w):
    ar, ai = a
    wr, wi = float(np.real(w)), float(np.imag(w))
    eps = 1e-12
    if abs(wi) < eps and abs(wr - 1) < eps:
        return ar, ai
    if abs(wi) < eps and abs(wr + 1) < eps:
        return -ar, -ai
    if abs(wr) < eps and abs(wi + 1) < eps:
        return ai, -ar
    if abs(wr) < eps and abs(wi - 1) < eps:
        return -ai, ar
    if abs(abs(wr) - abs(wi)) < eps:
        c = abs(wr)
        sr, si = np.sign(wr), np.sign(wi)
        t1 = (ar - ai) if sr * si > 0 else (ar + ai)
        t2 = (ar + ai) if sr * si > 0 else (ar - ai)
        return t1 * (c * sr), t2 * (c * si)
    return ar * wr - ai * wi, ar * wi + ai * wr


def _fft_list(xs, sign):
    n = len(xs)
    if n == 1:
        return xs
    ev = _fft_list(xs[0::2], sign)
    od = _fft_list(xs[1::2], sign)
    out = [None] * n
    for k in range(n // 2):
        t = _cmul_const(od[k], np.exp(sign * 2j * np.pi * k / n))
        out[k] = (ev[k][0] + t[0], ev[k][1] + t[1])
        out[k + n // 2] = (ev[k][0] - t[0], ev[k][1] - t[1])
    return out


def make(TQ=1024, KC=128, RC=16):
    NQ = S // TQ
    NI = H * NQ
    NC = S // KC

    def kern(xa_ref, wr_ref, wi_ref, xb_ref, w_ref, wo_ref, f1_ref, m_ref, finv_ref, o_ref,
             qT_ref, k_ref, vT_ref, oT_ref, sa_ref, sb_ref, xf_ref, t_ref, g_ref):
        xf_ref[...] = jnp.dot(f1_ref[...], xa_ref[...], preferred_element_type=F32)

        def stage_a_fwd(rc, carry):
            r0 = pl.multiple_of(rc * RC, RC)
            xs = [(xf_ref[pl.ds(r0, RC), n1*128:(n1+1)*128], xf_ref[pl.ds(R + r0, RC), n1*128:(n1+1)*128]) for n1 in range(N1)]
            ys = _fft_list(xs, -1)
            for k1 in range(N1):
                t_ref[k1, pl.ds(r0, RC), 0:128] = ys[k1][0].astype(BF)
                t_ref[k1, pl.ds(r0, RC), 128:256] = ys[k1][1].astype(BF)
            return carry
        jax.lax.fori_loop(0, R // RC, stage_a_fwd, 0)

        def mid(k1, carry):
            c0 = pl.multiple_of(k1 * 128, 128)
            mk = m_ref[k1]
            z = jnp.dot(t_ref[k1], mk, preferred_element_type=F32)
            zr, zi = z[:, :128], z[:, 128:]
            wr = wr_ref[:, pl.ds(c0, 128)].astype(F32)
            wi = wi_ref[:, pl.ds(c0, 128)].astype(F32)
            yr = zr * wr - zi * wi
            yi = zr * wi + zi * wr
            y = jnp.concatenate([yr, yi], axis=1).astype(BF)
            tp = jax.lax.dot_general(y, mk, (((1,), (1,)), ((), ())), preferred_element_type=F32)
            xf_ref[0:R, pl.ds(c0, 128)] = tp[:, :128]
            xf_ref[R:2*R, pl.ds(c0, 128)] = tp[:, 128:]
            return carry
        jax.lax.fori_loop(0, N1, mid, 0)

        def stage_a_inv(rc, carry):
            r0 = pl.multiple_of(rc * RC, RC)
            xs = [(xf_ref[pl.ds(r0, RC), k1*128:(k1+1)*128], xf_ref[pl.ds(R + r0, RC), k1*128:(k1+1)*128]) for k1 in range(N1)]
            ys = _fft_list(xs, +1)
            for n1 in range(N1):
                g_ref[pl.ds(r0, RC), n1*128:(n1+1)*128] = ys[n1][0].astype(BF)
                g_ref[pl.ds(R + r0, RC), n1*128:(n1+1)*128] = ys[n1][1].astype(BF)
            return carry
        jax.lax.fori_loop(0, R // RC, stage_a_inv, 0)
        ya = jax.lax.dot_general(g_ref[...], finv_ref[...], (((0,), (0,)), ((), ())), preferred_element_type=F32)
        o_ref[:, 0:640] = ya.astype(BF)

        xT = xb_ref[...]
        x = xT.T
        c = (DH ** -0.5) * LOG2E
        for g in range(5):
            wq = w_ref[:, 126*g:126*g+128]
            wk = w_ref[:, 576+126*g:576+126*g+128]
            k_ref[:, 128*g:128*(g+1)] = jnp.dot(x, wk, preferred_element_type=F32).astype(BF)
            qT = jnp.dot(wq.T, xT, preferred_element_type=F32)
            qT_ref[128*g:128*(g+1), :] = (qT * c).astype(BF)
        wv = w_ref[:, 1152:1728]
        vT_ref[...] = jnp.dot(wv.T, xT, preferred_element_type=F32).astype(BF)
        oT_ref[...] = jnp.zeros_like(oT_ref)

        def prep_scores(i):
            i = jnp.minimum(i, NI - 1)
            h = i // NQ
            qs = pl.multiple_of((i % NQ) * TQ, TQ)
            g = h // 7
            j = h % 7
            g128 = pl.multiple_of(g * 128, 128)
            row128 = jax.lax.broadcasted_iota(jnp.int32, (128, TQ), 0)
            qm = qT_ref[pl.ds(g128, 128), pl.ds(qs, TQ)]
            qm = jnp.where((row128 >= 18*j) & (row128 < 18*j+18), qm, jnp.zeros_like(qm))
            return qm, g128

        def score_chunk(cidx, qm, g128, s_ref, m8):
            sT = jnp.dot(k_ref[cidx*KC:(cidx+1)*KC, pl.ds(g128, 128)], qm, preferred_element_type=F32)
            s_ref[cidx*KC:(cidx+1)*KC, :] = sT
            mc = jnp.max(sT.reshape(KC // 8, 8, TQ), axis=0)
            return mc if m8 is None else jnp.maximum(m8, mc)

        def prep_finish(i):
            h = i // NQ
            qs = pl.multiple_of((i % NQ) * TQ, TQ)
            start = pl.multiple_of((18 * h) // 16 * 16, 16)
            off = (18 * h) % 16
            ones_row = jnp.where(off >= 1, 0, 31)
            row32 = jax.lax.broadcasted_iota(jnp.int32, (32, S), 0)
            vw = vT_ref[pl.ds(start, 32), :]
            vw = jnp.where(row32 == ones_row, jnp.ones_like(vw), vw)
            return vw, (qs, start, off, ones_row)

        def finish_chunk(cidx, vw, s_ref, m, acc):
            p = jnp.exp2(s_ref[cidx*KC:(cidx+1)*KC, :] - m).astype(BF)
            d = jnp.dot(vw[:, cidx*KC:(cidx+1)*KC], p, preferred_element_type=F32)
            return d if acc is None else acc + d

        def finish_store(acc, info):
            qs, start, off, ones_row = info
            r32 = jax.lax.broadcasted_iota(jnp.int32, (32, TQ), 0)
            l = jnp.sum(jnp.where(r32 == ones_row, acc, 0.0), axis=0, keepdims=True)
            res = acc / l
            old = oT_ref[pl.ds(start, 32), pl.ds(qs, TQ)]
            oT_ref[pl.ds(start, 32), pl.ds(qs, TQ)] = jnp.where((r32 >= off) & (r32 < off + 18), res, old)

        def step(i_next, s_next, i_cur, s_cur, m_cur):
            qm, g128 = prep_scores(i_next)
            vw, info = prep_finish(i_cur)
            m8 = None; acc = None
            for cidx in range(NC):
                acc = finish_chunk(cidx, vw, s_cur, m_cur, acc)
                if cidx == NC - 1:
                    finish_store(acc, info)
                m8 = score_chunk(cidx, qm, g128, s_next, m8)
            return jnp.max(m8, axis=0, keepdims=True)

        qm, g128 = prep_scores(0)
        m8 = None
        for cidx in range(NC):
            m8 = score_chunk(cidx, qm, g128, sa_ref, m8)
        m0 = jnp.max(m8, axis=0, keepdims=True)

        def body(i, m):
            return jax.lax.cond(i % 2 == 0,
                                lambda: step(i + 1, sb_ref, i, sa_ref, m),
                                lambda: step(i + 1, sa_ref, i, sb_ref, m))
        jax.lax.fori_loop(0, NI, body, m0)
        oT = oT_ref[...].astype(BF)
        yb = jax.lax.dot_general(oT, wo_ref[...], (((0,), (0,)), ((), ())), preferred_element_type=F32)
        lane = jax.lax.broadcasted_iota(jnp.int32, (S, 128), 1)
        o_ref[:, 512:640] = jnp.where(lane < 64, o_ref[:, 512:640], yb[:, 0:128].astype(BF))
        o_ref[:, 640:1152] = yb[:, 128:640].astype(BF)

    f1, m, finv = _consts()

    @jax.jit
    def f(A_x, A_w_r, A_w_i, B_x, B_wqkv, B_wo):
        xaT = A_x[0].T
        xbT = B_x[0].T
        def perm(w):
            return jnp.pad(w.reshape(N2, N1, DF).transpose(2, 1, 0).reshape(DF, S), ((0, R - DF), (0, 0)))
        wo_p = jnp.pad(B_wo, ((0, 0), (64, 0)))
        out = pl.pallas_call(kern, out_shape=jax.ShapeDtypeStruct((S, 2 * D), BF),
            scratch_shapes=[pltpu.VMEM((640, S), BF), pltpu.VMEM((S, 640), BF),
                            pltpu.VMEM((D, S), BF), pltpu.VMEM((D, S), F32),
                            pltpu.VMEM((S, TQ), F32), pltpu.VMEM((S, TQ), F32),
                            pltpu.VMEM((2 * R, S), F32), pltpu.VMEM((N1, R, 256), BF), pltpu.VMEM((2 * R, S), BF)],
            compiler_params=pltpu.CompilerParams(vmem_limit_bytes=110 << 20))(
                xaT, perm(A_w_r), perm(A_w_i), xbT, B_wqkv, wo_p, f1, m, finv)
        return out[None]
    return f


_impl = make()


def pallas_concat_heads__spectral_gfnet__mha_block__prompt_kernel(A_x, A_w_r, A_w_i, B_x, B_wqkv, B_wo):
    return _impl(A_x, A_w_r, A_w_i, B_x, B_wqkv, B_wo)
```

```python
import functools, math
import numpy as np
import jax, jax.numpy as jnp
from jax.experimental import pallas as pl
from jax.experimental.pallas import tpu as pltpu

S, D, H, DH = 2048, 576, 32, 18
DF = D // 2 + 1
R = 304
N1, N2 = 16, 128
LOG2E = 1.4426950408889634
BF = jnp.bfloat16
F32 = jnp.float32


def _consts():
    f = np.arange(R)[:, None].astype(np.float64)
    d = np.arange(D)[None, :].astype(np.float64)
    valid = (f < DF)
    ang = 2 * np.pi * ((f * d) % D) / D
    f1 = np.concatenate([np.where(valid, np.cos(ang), 0.0), np.where(valid, -np.sin(ang), 0.0)], axis=0)
    cf = np.where((f == 0) | (f == DF - 1), 1.0, 2.0) / (S * D)
    finv = np.concatenate([np.where(valid, cf * np.cos(ang), 0.0), np.where(valid, -cf * np.sin(ang), 0.0)], axis=0)
    finv = np.pad(finv, ((0, 0), (0, 64)))
    n2 = np.arange(N2)[:, None]
    k2 = np.arange(N2)[None, :]
    ms = []
    for k1 in range(N1):
        th = 2 * np.pi * ((n2 * (k1 + N1 * k2)) % S) / S
        c, s = np.cos(th), np.sin(th)
        ms.append(np.block([[c, -s], [s, c]]))
    m = np.stack(ms)
    return (f1.astype(BF), m.astype(BF), finv.astype(BF))


def _cmul_const(a, w):
    ar, ai = a
    wr, wi = float(np.real(w)), float(np.imag(w))
    eps = 1e-12
    if abs(wi) < eps and abs(wr - 1) < eps:
        return ar, ai
    if abs(wi) < eps and abs(wr + 1) < eps:
        return -ar, -ai
    if abs(wr) < eps and abs(wi + 1) < eps:
        return ai, -ar
    if abs(wr) < eps and abs(wi - 1) < eps:
        return -ai, ar
    if abs(abs(wr) - abs(wi)) < eps:
        c = abs(wr)
        sr, si = np.sign(wr), np.sign(wi)
        t1 = (ar - ai) if sr * si > 0 else (ar + ai)
        t2 = (ar + ai) if sr * si > 0 else (ar - ai)
        return t1 * (c * sr), t2 * (c * si)
    return ar * wr - ai * wi, ar * wi + ai * wr


def _fft_list(xs, sign):
    n = len(xs)
    if n == 1:
        return xs
    ev = _fft_list(xs[0::2], sign)
    od = _fft_list(xs[1::2], sign)
    out = [None] * n
    for k in range(n // 2):
        t = _cmul_const(od[k], np.exp(sign * 2j * np.pi * k / n))
        out[k] = (ev[k][0] + t[0], ev[k][1] + t[1])
        out[k + n // 2] = (ev[k][0] - t[0], ev[k][1] - t[1])
    return out


def make(TQ=1024, KC=128, RC=16, OC=512, HH=H, UN=2, LA=1, PC=512, TB=40.0, FORCE_SLOW=False, SQ=128, L5=1024):
    NQ = S // TQ
    NC = S // KC
    XC = 4

    def kern(xa_hbm, wr_hbm, wi_hbm, xb_hbm, w_hbm, wo_hbm, f1_hbm, m_hbm, finv_hbm, o_hbm,
             xa_ref, wr_ref, wi_ref, xb_ref, w_ref, wo_ref, f1_ref, m_ref, finv_ref, ob_ref,
             qT_ref, k_ref, vT_ref, oT_ref, xf_ref, t_ref, g_ref, wn_ref, wp_ref, x_ref, wT_ref, am_ref,
             in_sems, out_sems):
        cp_f1 = pltpu.make_async_copy(f1_hbm, f1_ref, in_sems.at[0])
        cp_xa = [pltpu.make_async_copy(xa_hbm.at[:, c*(S//XC):(c+1)*(S//XC)], xa_ref.at[:, c*(S//XC):(c+1)*(S//XC)], in_sems.at[1 + c]) for c in range(XC)]
        cp_wr = pltpu.make_async_copy(wr_hbm, wr_ref, in_sems.at[5])
        cp_wi = pltpu.make_async_copy(wi_hbm, wi_ref, in_sems.at[6])
        cp_m = pltpu.make_async_copy(m_hbm, m_ref, in_sems.at[7])
        cp_finv = pltpu.make_async_copy(finv_hbm, finv_ref, in_sems.at[8])
        cp_xb = pltpu.make_async_copy(xb_hbm, xb_ref, in_sems.at[9])
        cp_w = pltpu.make_async_copy(w_hbm, w_ref, in_sems.at[10])
        cp_wo = pltpu.make_async_copy(wo_hbm, wo_ref, in_sems.at[11])
        for cp in [cp_f1, cp_xa[0]]:
            cp.start()

        c = (DH ** -0.5) * LOG2E
        am_ref[...] = jnp.zeros_like(am_ref)
        frow = jax.lax.broadcasted_iota(jnp.int32, (R - 256, 128), 0)

        def wperm_a(a):
            wref = (wr_ref, wi_ref)[a]
            wn_ref[a, 0] = wref[0:128, :].T.astype(F32)
            wn_ref[a, 1] = wref[128:256, :].T.astype(F32)
            wn_ref[a, 2, :, 0:DF-256] = wref[256:DF, :].T.astype(F32)
        def wperm_b(a, k1):
            for j in range(2):
                wp_ref[a, j*128:(j+1)*128, k1*128:(k1+1)*128] = wn_ref[a, j, pl.ds(k1, N2, stride=N1), :].T
            blk = wn_ref[a, 2, pl.ds(k1, N2, stride=N1), :].T[0:R-256, :]
            wp_ref[a, 256:R, k1*128:(k1+1)*128] = jnp.where(frow < DF - 256, blk, 0.0)

        def stage_a_fwd(rc):
            r0 = rc * RC
            xs = [(xf_ref[r0:r0+RC, n1*128:(n1+1)*128], xf_ref[R+r0:R+r0+RC, n1*128:(n1+1)*128]) for n1 in range(N1)]
            ys = _fft_list(xs, -1)
            for k1 in range(N1):
                t_ref[k1, r0:r0+RC, 0:128] = ys[k1][0].astype(BF)
                t_ref[k1, r0:r0+RC, 128:256] = ys[k1][1].astype(BF)

        def stage_a_inv(rc):
            r0 = rc * RC
            xs = [(xf_ref[r0:r0+RC, k1*128:(k1+1)*128], xf_ref[R+r0:R+r0+RC, k1*128:(k1+1)*128]) for k1 in range(N1)]
            ys = _fft_list(xs, +1)
            for n1 in range(N1):
                g_ref[r0:r0+RC, n1*128:(n1+1)*128] = ys[n1][0].astype(BF)
                g_ref[R+r0:R+r0+RC, n1*128:(n1+1)*128] = ys[n1][1].astype(BF)

        def track(idx, val):
            a = jnp.abs(val)
            a = jnp.max(a.reshape(a.shape[0] // 8, 8, a.shape[1]), axis=0)
            a = functools.reduce(jnp.maximum, [a[:, l*128:(l+1)*128] for l in range(a.shape[1] // 128)])
            am_ref[idx] = jnp.maximum(am_ref[idx], a)
        def proj_k(g, pc):
            wk = w_ref[:, 576+126*g:576+126*g+128]
            kk = jnp.dot(x_ref[pc*PC:(pc+1)*PC, :], wk, preferred_element_type=F32)
            track(1, kk)
            k_ref[pc*PC:(pc+1)*PC, 128*g:128*(g+1)] = kk.astype(BF)
        def proj_q(g, pc):
            qT = jnp.dot(wT_ref[128*g:128*(g+1), :], xb_ref[:, pc*PC:(pc+1)*PC], preferred_element_type=F32) * c
            track(0, qT)
            qT_ref[128*g:128*(g+1), pc*PC:(pc+1)*PC] = qT.astype(BF)
        def proj_v(r, pc):
            rr = slice(640 + r*192, 640 + (r+1)*192)
            vv = jnp.dot(wT_ref[rr, :], xb_ref[:, pc*PC:(pc+1)*PC], preferred_element_type=F32)
            track(2, vv)
            vT_ref[r*192:(r+1)*192, pc*PC:(pc+1)*PC] = vv.astype(BF)

        def interleave(mx, vp):
            n = max(len(mx), 1)
            done = 0
            for i, f in enumerate(mx):
                f()
                upto = (i + 1) * len(vp) // n
                for g_ in vp[done:upto]:
                    g_()
                done = upto
            for g_ in vp[done:]:
                g_()

        cp_f1.wait()
        cp_xa[0].wait()
        for cp in cp_xa[1:] + [cp_xb, cp_w]:
            cp.start()
        for cc in range(XC):
            if cc > 0:
                cp_xa[cc].wait()
            sl = slice(cc*(S//XC), (cc+1)*(S//XC))
            xf_ref[:, sl] = jnp.dot(f1_ref[...], xa_ref[:, sl], preferred_element_type=F32)
        for rc in range(R // RC):
            stage_a_fwd(rc)
        cp_xb.wait()
        cp_w.wait()
        for cp in [cp_wr, cp_wi, cp_m, cp_finv, cp_wo]:
            cp.start()
        def prep_b():
            x_ref[...] = xb_ref[...].T
            for g in range(5):
                wT_ref[128*g:128*(g+1), :] = w_ref[:, 126*g:126*g+128].T
            wT_ref[640:640+D, :] = w_ref[:, 1152:1728].T
        prep_b()
        NPC = S // PC
        mx1 = [functools.partial(proj_q, g, pc) for g in range(5) for pc in range(NPC)] + [functools.partial(proj_v, 0, pc) for pc in range(NPC)]
        for f_ in mx1[:2*NPC]:
            f_()
        cp_wr.wait()
        cp_wi.wait()
        vp = [functools.partial(wperm_a, 0), functools.partial(wperm_a, 1)] + [functools.partial(wperm_b, a, k1) for a in range(2) for k1 in range(N1)]
        interleave(mx1[2*NPC:], vp)
        cp_m.wait()

        def mid(k1, carry):
            c0 = pl.multiple_of(k1 * 128, 128)
            mk = m_ref[k1]
            z = jnp.dot(t_ref[k1], mk, preferred_element_type=F32)
            zr, zi = z[:, :128], z[:, 128:]
            wr = wp_ref[0, :, pl.ds(c0, 128)]
            wi = wp_ref[1, :, pl.ds(c0, 128)]
            yr = zr * wr - zi * wi
            yi = zr * wi + zi * wr
            y = jnp.concatenate([yr, yi], axis=1).astype(BF)
            tp = jax.lax.dot_general(y, mk, (((1,), (1,)), ((), ())), preferred_element_type=F32)
            xf_ref[0:R, pl.ds(c0, 128)] = tp[:, :128]
            xf_ref[R:2*R, pl.ds(c0, 128)] = tp[:, 128:]
            return carry
        jax.lax.fori_loop(0, N1, mid, 0)

        mx2 = [functools.partial(proj_k, g, pc) for g in range(5) for pc in range(NPC)] + [functools.partial(proj_v, r, pc) for r in (1, 2) for pc in range(NPC)]
        interleave(mx2, [functools.partial(stage_a_inv, rc) for rc in range(R // RC)])
        oT_ref[...] = jnp.zeros_like(oT_ref)
        cp_finv.wait()
        if L5:
            def step5(pc, carry):
                c0 = pl.multiple_of(pc * L5, L5)
                ya = jax.lax.dot_general(g_ref[:, pl.ds(c0, L5)], finv_ref[...], (((0,), (0,)), ((), ())), preferred_element_type=F32)
                ob_ref[pl.ds(c0, L5), 0:640] = ya.astype(BF)
                return carry
            jax.lax.fori_loop(0, S // L5, step5, 0)
        else:
            ya = jax.lax.dot_general(g_ref[...], finv_ref[...], (((0,), (0,)), ((), ())), preferred_element_type=F32)
            ob_ref[:, 0:640] = ya.astype(BF)
        cp_oa = pltpu.make_async_copy(ob_ref.at[:, 0:512], o_hbm.at[:, 0:512], out_sems.at[0])
        cp_oa.start()

        def prep_scores(h, qt, TQ=TQ):
            g = h // 7
            j = h % 7
            g128 = pl.multiple_of(g * 128, 128)
            row128 = jax.lax.broadcasted_iota(jnp.int32, (128, TQ), 0)
            qm = qT_ref[pl.ds(g128, 128), qt*TQ:(qt+1)*TQ]
            qm = jnp.where((row128 >= 18*j) & (row128 < 18*j+18), qm, jnp.zeros_like(qm))
            return qm, g128

        def prep_finish(h, vscale=None):
            start = pl.multiple_of((18 * h) // 16 * 16, 16)
            off = (18 * h) % 16
            ones_row = jnp.where(off >= 1, 0, 31)
            row32 = jax.lax.broadcasted_iota(jnp.int32, (32, S), 0)
            vw = vT_ref[pl.ds(start, 32), :]
            vw = jnp.where(row32 == ones_row, jnp.ones_like(vw), vw)
            if vscale is not None:
                vw = (vw.astype(F32) * vscale).astype(BF)
            return vw, (start, off, ones_row)

        def finish_store(acc, qt, info, TQ=TQ):
            start, off, ones_row = info
            r32 = jax.lax.broadcasted_iota(jnp.int32, (32, TQ), 0)
            l = jnp.sum(jnp.where(r32 == ones_row, acc, 0.0), axis=0, keepdims=True)
            res = acc / l
            old = oT_ref[pl.ds(start, 32), qt*TQ:(qt+1)*TQ]
            oT_ref[pl.ds(start, 32), qt*TQ:(qt+1)*TQ] = jnp.where((r32 >= off) & (r32 < off + 18), res, old)

        def body(t, c):
            items = [(u, qt, cidx) for u in range(UN) for qt in range(NQ) for cidx in range(NC)]
            vws = {}; qms = {}; ss = {}; accs = {}
            def qk(n):
                u, qt, cidx = items[n]
                if (u, qt) not in qms:
                    qms[(u, qt)] = prep_scores(UN * t + u, qt)
                qm, g128 = qms[(u, qt)]
                ss[n] = jnp.dot(k_ref[cidx*KC:(cidx+1)*KC, pl.ds(g128, 128)], qm, preferred_element_type=F32)
            def pv(n):
                u, qt, cidx = items[n]
                if u not in vws:
                    vws[u] = prep_finish(UN * t + u, 2.0 ** TB)
                vw, info = vws[u]
                p = jnp.exp2(ss.pop(n)).astype(BF)
                d = jnp.dot(vw[:, cidx*KC:(cidx+1)*KC], p, preferred_element_type=F32)
                accs[(u, qt)] = d if cidx == 0 else accs[(u, qt)] + d
                if cidx == NC - 1:
                    finish_store(accs.pop((u, qt)), qt, info)
            for n in range(len(items) + LA):
                if n < len(items):
                    qk(n)
                if n >= LA:
                    pv(n - LA)
            return c
        def slow_tile(i, c):
            h = i // (S // SQ)
            q0 = pl.multiple_of((i % (S // SQ)) * SQ, SQ)
            vw, (start, off, ones_row) = prep_finish(h)
            g128 = pl.multiple_of((h // 7) * 128, 128)
            j = h % 7
            row128 = jax.lax.broadcasted_iota(jnp.int32, (128, SQ), 0)
            qm = qT_ref[pl.ds(g128, 128), pl.ds(q0, SQ)]
            qm = jnp.where((row128 >= 18*j) & (row128 < 18*j+18), qm, jnp.zeros_like(qm))
            sT = jnp.dot(k_ref[:, pl.ds(g128, 128)], qm, preferred_element_type=F32)
            mx = jnp.max(sT, axis=0, keepdims=True)
            p = jnp.exp2(sT - mx).astype(BF)
            acc = jnp.dot(vw, p, preferred_element_type=F32)
            r32 = jax.lax.broadcasted_iota(jnp.int32, (32, SQ), 0)
            l = jnp.sum(jnp.where(r32 == ones_row, acc, 0.0), axis=0, keepdims=True)
            res = acc / l
            old = oT_ref[pl.ds(start, 32), pl.ds(q0, SQ)]
            oT_ref[pl.ds(start, 32), pl.ds(q0, SQ)] = jnp.where((r32 >= off) & (r32 < off + 18), res, old)
            return c

        qmax = jnp.max(am_ref[0])
        kmax = jnp.max(am_ref[1])
        vmax = jnp.max(am_ref[2])
        safe = jnp.logical_and(qmax * kmax * (DH * 1.02) <= TB, vmax <= 2.0 ** 30)
        if FORCE_SLOW:
            safe = jnp.logical_and(safe, qmax < 0.0)

        @pl.when(safe)
        def _():
            jax.lax.fori_loop(0, HH // UN, body, 0)

        @pl.when(jnp.logical_not(safe))
        def _():
            jax.lax.fori_loop(0, H * (S // SQ), slow_tile, 0)

        cp_wo.wait()
        wo = wo_ref[...]
        wo_p = jnp.concatenate([jnp.zeros((D, 64), BF), wo], axis=1)
        lane = jax.lax.broadcasted_iota(jnp.int32, (OC, 128), 1)
        cps = []
        for oc in range(S // OC):
            rs = slice(oc*OC, (oc+1)*OC)
            oT = oT_ref[:, rs].astype(BF)
            yb = jax.lax.dot_general(oT, wo_p, (((0,), (0,)), ((), ())), preferred_element_type=F32)
            ob_ref[rs, 512:640] = jnp.where(lane < 64, ob_ref[rs, 512:640], yb[:, 0:128].astype(BF))
            ob_ref[rs, 640:1152] = yb[:, 128:640].astype(BF)
            cp = pltpu.make_async_copy(ob_ref.at[rs, 512:1152], o_hbm.at[rs, 512:1152], out_sems.at[1 + oc])
            cp.start()
            cps.append(cp)
        cp_oa.wait()
        for cp in cps:
            cp.wait()

    f1, m, finv = _consts()

    @jax.jit
    def f(A_x, A_w_r, A_w_i, B_x, B_wqkv, B_wo):
        xaT = A_x[0].T
        xbT = B_x[0].T
        anyspec = pl.BlockSpec(memory_space=pl.ANY)
        out = pl.pallas_call(kern, out_shape=jax.ShapeDtypeStruct((S, 2 * D), BF),
            in_specs=[anyspec] * 9, out_specs=anyspec,
            scratch_shapes=[pltpu.VMEM((D, S), BF), pltpu.VMEM((DF, S), BF), pltpu.VMEM((DF, S), BF), pltpu.VMEM((D, S), BF),
                            pltpu.VMEM((D, 3 * D), BF), pltpu.VMEM((D, D), BF), pltpu.VMEM((2 * R, D), BF),
                            pltpu.VMEM((N1, 256, 256), BF), pltpu.VMEM((2 * R, 640), BF), pltpu.VMEM((S, 2 * D), BF),
                            pltpu.VMEM((640, S), BF), pltpu.VMEM((S, 640), BF),
                            pltpu.VMEM((D, S), BF), pltpu.VMEM((D, S), F32),
                            pltpu.VMEM((2 * R, S), F32), pltpu.VMEM((N1, R, 256), BF), pltpu.VMEM((2 * R, S), BF),
                            pltpu.VMEM((2, 3, S, 128), F32), pltpu.VMEM((2, R, S), F32),
                            pltpu.VMEM((S, D), BF), pltpu.VMEM((640 + D, D), BF), pltpu.VMEM((3, 8, 128), F32),
                            pltpu.SemaphoreType.DMA((12,)), pltpu.SemaphoreType.DMA((1 + S // OC,))],
            compiler_params=pltpu.CompilerParams(vmem_limit_bytes=110 << 20))(
                xaT, A_w_r.T, A_w_i.T, xbT, B_wqkv, B_wo, jnp.asarray(f1), jnp.asarray(m), jnp.asarray(finv))
        return out[None]
    return f


_impl = make()


def pallas_concat_heads__spectral_gfnet__mha_block__prompt_kernel(A_x, A_w_r, A_w_i, B_x, B_wqkv, B_wo):
    return _impl(A_x, A_w_r, A_w_i, B_x, B_wqkv, B_wo)
```

```python
import functools, math
import numpy as np
import jax, jax.numpy as jnp
from jax.experimental import pallas as pl
from jax.experimental.pallas import tpu as pltpu

S, D, H, DH = 2048, 576, 32, 18
DF = D // 2 + 1
R = 304
N1, N2 = 16, 128
LOG2E = 1.4426950408889634
BF = jnp.bfloat16
F32 = jnp.float32


def _consts():
    f = np.arange(R)[:, None].astype(np.float64)
    d = np.arange(D)[None, :].astype(np.float64)
    valid = (f < DF)
    ang = 2 * np.pi * ((f * d) % D) / D
    f1 = np.concatenate([np.where(valid, np.cos(ang), 0.0), np.where(valid, -np.sin(ang), 0.0)], axis=0)
    cf = np.where((f == 0) | (f == DF - 1), 1.0, 2.0) / (S * D)
    finv = np.concatenate([np.where(valid, cf * np.cos(ang), 0.0), np.where(valid, -cf * np.sin(ang), 0.0)], axis=0)
    finv = np.pad(finv, ((0, 0), (0, 64)))
    n2 = np.arange(N2)[:, None]
    k2 = np.arange(N2)[None, :]
    ms = []
    for k1 in range(N1):
        th = 2 * np.pi * ((n2 * (k1 + N1 * k2)) % S) / S
        c, s = np.cos(th), np.sin(th)
        ms.append(np.block([[c, -s], [s, c]]))
    m = np.stack(ms)
    return (f1.astype(BF), m.astype(BF), finv.astype(BF))


def _cmul_const(a, w):
    ar, ai = a
    wr, wi = float(np.real(w)), float(np.imag(w))
    eps = 1e-12
    if abs(wi) < eps and abs(wr - 1) < eps:
        return ar, ai
    if abs(wi) < eps and abs(wr + 1) < eps:
        return -ar, -ai
    if abs(wr) < eps and abs(wi + 1) < eps:
        return ai, -ar
    if abs(wr) < eps and abs(wi - 1) < eps:
        return -ai, ar
    if abs(abs(wr) - abs(wi)) < eps:
        c = abs(wr)
        sr, si = np.sign(wr), np.sign(wi)
        t1 = (ar - ai) if sr * si > 0 else (ar + ai)
        t2 = (ar + ai) if sr * si > 0 else (ar - ai)
        return t1 * (c * sr), t2 * (c * si)
    return ar * wr - ai * wi, ar * wi + ai * wr


def _fft_list(xs, sign):
    n = len(xs)
    if n == 1:
        return xs
    ev = _fft_list(xs[0::2], sign)
    od = _fft_list(xs[1::2], sign)
    out = [None] * n
    for k in range(n // 2):
        t = _cmul_const(od[k], np.exp(sign * 2j * np.pi * k / n))
        out[k] = (ev[k][0] + t[0], ev[k][1] + t[1])
        out[k + n // 2] = (ev[k][0] - t[0], ev[k][1] - t[1])
    return out


def make(TQ=1024, KC=128, RC=16, OC=512, HH=H, UN=2, LA=1, PC=512, TB=40.0, FORCE_SLOW=False, SQ=128, L5=1024):
    NQ = S // TQ
    NC = S // KC
    XC = 4

    def kern(xa_hbm, wr_hbm, wi_hbm, xb_hbm, w_hbm, wo_hbm, f1_hbm, m_hbm, finv_hbm, o_hbm,
             xa_ref, wr_ref, wi_ref, xb_ref, w_ref, wo_ref, f1_ref, m_ref, finv_ref, ob_ref,
             qT_ref, k_ref, vT_ref, oT_ref, xf_ref, t_ref, g_ref, wn_ref, wp_ref, x_ref, wT_ref, am_ref, vl_ref, vb_ref,
             in_sems, out_sems):
        cp_f1 = pltpu.make_async_copy(f1_hbm, f1_ref, in_sems.at[0])
        cp_xa = [pltpu.make_async_copy(xa_hbm.at[:, c*(S//XC):(c+1)*(S//XC)], xa_ref.at[:, c*(S//XC):(c+1)*(S//XC)], in_sems.at[1 + c]) for c in range(XC)]
        cp_wr = pltpu.make_async_copy(wr_hbm, wr_ref, in_sems.at[5])
        cp_wi = pltpu.make_async_copy(wi_hbm, wi_ref, in_sems.at[6])
        cp_m = pltpu.make_async_copy(m_hbm, m_ref, in_sems.at[7])
        cp_finv = pltpu.make_async_copy(finv_hbm, finv_ref, in_sems.at[8])
        cp_xb = pltpu.make_async_copy(xb_hbm, xb_ref, in_sems.at[9])
        cp_w = pltpu.make_async_copy(w_hbm, w_ref, in_sems.at[10])
        cp_wo = pltpu.make_async_copy(wo_hbm, wo_ref, in_sems.at[11])
        for cp in [cp_f1, cp_xa[0]]:
            cp.start()

        c = (DH ** -0.5) * LOG2E
        am_ref[...] = jnp.zeros_like(am_ref)
        frow = jax.lax.broadcasted_iota(jnp.int32, (R - 256, 128), 0)

        def wperm_a(a):
            wref = (wr_ref, wi_ref)[a]
            wn_ref[a, 0] = wref[0:128, :].T.astype(F32)
            wn_ref[a, 1] = wref[128:256, :].T.astype(F32)
            wn_ref[a, 2, :, 0:DF-256] = wref[256:DF, :].T.astype(F32)
        def wperm_b(a, k1):
            for j in range(2):
                wp_ref[a, j*128:(j+1)*128, k1*128:(k1+1)*128] = wn_ref[a, j, pl.ds(k1, N2, stride=N1), :].T
            blk = wn_ref[a, 2, pl.ds(k1, N2, stride=N1), :].T[0:R-256, :]
            wp_ref[a, 256:R, k1*128:(k1+1)*128] = jnp.where(frow < DF - 256, blk, 0.0)

        def stage_a_fwd(rc):
            r0 = rc * RC
            xs = [(xf_ref[r0:r0+RC, n1*128:(n1+1)*128], xf_ref[R+r0:R+r0+RC, n1*128:(n1+1)*128]) for n1 in range(N1)]
            ys = _fft_list(xs, -1)
            for k1 in range(N1):
                t_ref[k1, r0:r0+RC, 0:128] = ys[k1][0].astype(BF)
                t_ref[k1, r0:r0+RC, 128:256] = ys[k1][1].astype(BF)

        def stage_a_inv(rc):
            r0 = rc * RC
            xs = [(xf_ref[r0:r0+RC, k1*128:(k1+1)*128], xf_ref[R+r0:R+r0+RC, k1*128:(k1+1)*128]) for k1 in range(N1)]
            ys = _fft_list(xs, +1)
            for n1 in range(N1):
                g_ref[r0:r0+RC, n1*128:(n1+1)*128] = ys[n1][0].astype(BF)
                g_ref[R+r0:R+r0+RC, n1*128:(n1+1)*128] = ys[n1][1].astype(BF)

        def track(idx, val):
            a = jnp.abs(val)
            a = jnp.max(a.reshape(a.shape[0] // 8, 8, a.shape[1]), axis=0)
            a = functools.reduce(jnp.maximum, [a[:, l*128:(l+1)*128] for l in range(a.shape[1] // 128)])
            am_ref[idx] = jnp.maximum(am_ref[idx], a)
        def proj_k(g, pc):
            wk = w_ref[:, 576+126*g:576+126*g+128]
            kk = jnp.dot(x_ref[pc*PC:(pc+1)*PC, :], wk, preferred_element_type=F32)
            track(1, kk)
            for j in range(min(7, H - 7 * g)):
                kr = kk if j == 0 else pltpu.roll(kk, 128 - 18 * j, 1)
                k_ref[7*g + j, pc*PC:(pc+1)*PC, :] = kr.astype(BF)
        def proj_q(g, pc):
            qT = jnp.dot(wT_ref[128*g:128*(g+1), :], xb_ref[:, pc*PC:(pc+1)*PC], preferred_element_type=F32) * c
            track(0, qT)
            for j in range(min(7, H - 7 * g)):
                qT_ref[7*g + j, :, pc*PC:(pc+1)*PC] = jnp.concatenate([qT[18*j:18*j+18], jnp.zeros((14, PC), F32)], axis=0).astype(BF)
        def proj_v(r, pc):
            rr = slice(640 + r*192, 640 + (r+1)*192)
            vv = jnp.dot(wT_ref[rr, :], xb_ref[:, pc*PC:(pc+1)*PC], preferred_element_type=F32)
            track(2, vv)
            vT_ref[r*192:(r+1)*192, pc*PC:(pc+1)*PC] = vv.astype(BF)

        def interleave(mx, vp):
            n = max(len(mx), 1)
            done = 0
            for i, f in enumerate(mx):
                f()
                upto = (i + 1) * len(vp) // n
                for g_ in vp[done:upto]:
                    g_()
                done = upto
            for g_ in vp[done:]:
                g_()

        cp_f1.wait()
        cp_xa[0].wait()
        for cp in cp_xa[1:] + [cp_xb, cp_w]:
            cp.start()
        for cc in range(XC):
            if cc > 0:
                cp_xa[cc].wait()
            sl = slice(cc*(S//XC), (cc+1)*(S//XC))
            xf_ref[:, sl] = jnp.dot(f1_ref[...], xa_ref[:, sl], preferred_element_type=F32)
        for rc in range(R // RC):
            stage_a_fwd(rc)
        cp_xb.wait()
        cp_w.wait()
        for cp in [cp_wr, cp_wi, cp_m, cp_finv, cp_wo]:
            cp.start()
        def prep_b():
            x_ref[...] = xb_ref[...].T
            for g in range(5):
                wT_ref[128*g:128*(g+1), :] = w_ref[:, 126*g:126*g+128].T
            wvT = w_ref[:, 1152:1728].T.astype(F32)
            wT_ref[640:640+512, :] = jnp.concatenate([wvT[18*h:18*h+16] for h in range(H)], axis=0).astype(BF)
            wT_ref[640+512:640+D, :] = jnp.concatenate([wvT[18*h+16:18*h+17] for h in range(H)] + [wvT[18*h+17:18*h+18] for h in range(H)], axis=0).astype(BF)
        prep_b()
        NPC = S // PC
        mx1 = [functools.partial(proj_q, g, pc) for g in range(5) for pc in range(NPC)] + [functools.partial(proj_v, 0, pc) for pc in range(NPC)]
        for f_ in mx1[:2*NPC]:
            f_()
        cp_wr.wait()
        cp_wi.wait()
        vp = [functools.partial(wperm_a, 0), functools.partial(wperm_a, 1)] + [functools.partial(wperm_b, a, k1) for a in range(2) for k1 in range(N1)]
        interleave(mx1[2*NPC:], vp)
        cp_m.wait()

        def mid(k1, carry):
            c0 = pl.multiple_of(k1 * 128, 128)
            mk = m_ref[k1]
            z = jnp.dot(t_ref[k1], mk, preferred_element_type=F32)
            zr, zi = z[:, :128], z[:, 128:]
            wr = wp_ref[0, :, pl.ds(c0, 128)]
            wi = wp_ref[1, :, pl.ds(c0, 128)]
            yr = zr * wr - zi * wi
            yi = zr * wi + zi * wr
            y = jnp.concatenate([yr, yi], axis=1).astype(BF)
            tp = jax.lax.dot_general(y, mk, (((1,), (1,)), ((), ())), preferred_element_type=F32)
            xf_ref[0:R, pl.ds(c0, 128)] = tp[:, :128]
            xf_ref[R:2*R, pl.ds(c0, 128)] = tp[:, 128:]
            return carry
        jax.lax.fori_loop(0, N1, mid, 0)

        mx2 = [functools.partial(proj_k, g, pc) for g in range(5) for pc in range(NPC)] + [functools.partial(proj_v, r, pc) for r in (1, 2) for pc in range(NPC)]
        interleave(mx2, [functools.partial(stage_a_inv, rc) for rc in range(R // RC)])
        vlt = vT_ref[512:D, :].T.astype(F32) * (2.0 ** TB)
        vlt = jnp.concatenate([vlt, jnp.zeros((S, 64), F32)], axis=1)
        vl_ref[0] = vlt
        vl_ref[1] = pltpu.roll(vlt, 96, 1)
        oT_ref[512:D, :] = jnp.zeros((64, S), F32)
        cp_finv.wait()
        if L5:
            def step5(pc, carry):
                c0 = pl.multiple_of(pc * L5, L5)
                ya = jax.lax.dot_general(g_ref[:, pl.ds(c0, L5)], finv_ref[...], (((0,), (0,)), ((), ())), preferred_element_type=F32)
                ob_ref[pl.ds(c0, L5), 0:640] = ya.astype(BF)
                return carry
            jax.lax.fori_loop(0, S // L5, step5, 0)
        else:
            ya = jax.lax.dot_general(g_ref[...], finv_ref[...], (((0,), (0,)), ((), ())), preferred_element_type=F32)
            ob_ref[:, 0:640] = ya.astype(BF)
        cp_oa = pltpu.make_async_copy(ob_ref.at[:, 0:512], o_hbm.at[:, 0:512], out_sems.at[0])
        cp_oa.start()

        def prep_finish(h, u):
            r0 = pl.multiple_of(16 * h, 16)
            vw = (vT_ref[pl.ds(r0, 16), :].astype(F32) * (2.0 ** TB)).astype(BF)
            return vw

        def store_left(h, a0, a1, qsl, n):
            o8 = h % 8
            r8 = jax.lax.broadcasted_iota(jnp.int32, (8, n), 0)
            for base, a in ((512, a0), (544, a1)):
                l8 = pl.multiple_of(base + h // 8 * 8, 8)
                oT_ref[pl.ds(l8, 8), qsl] = jnp.where(r8 == o8, a, oT_ref[pl.ds(l8, 8), qsl])

        def finish_store(h, acc, lacc, qt):
            r0 = pl.multiple_of(16 * h, 16)
            l = jnp.sum(lacc[2], axis=0, keepdims=True) * (2.0 ** TB)
            inv = 1.0 / l
            oT_ref[pl.ds(r0, 16), qt*TQ:(qt+1)*TQ] = acc * inv
            store_left(h, jnp.sum(lacc[0], axis=0, keepdims=True) * inv, jnp.sum(lacc[1], axis=0, keepdims=True) * inv, slice(qt*TQ, (qt+1)*TQ), TQ)

        def body(t, c):
            items = [(u, qt, cidx) for u in range(UN) for qt in range(NQ) for cidx in range(NC)]
            vws = {}; qms = {}; ss = {}; accs = {}; laccs = {}
            for u in range(UN):
                vws[u] = prep_finish(UN * t + u, u)
            def qk(n):
                u, qt, cidx = items[n]
                h = UN * t + u
                ss[n] = jnp.dot(k_ref[h, cidx*KC:(cidx+1)*KC, 0:32], qT_ref[h, :, qt*TQ:(qt+1)*TQ], preferred_element_type=F32)
            def pv(n):
                u, qt, cidx = items[n]
                vw = vws[u]
                p32 = jnp.exp2(ss.pop(n))
                p = p32.astype(BF)
                d = jnp.dot(vw[:, cidx*KC:(cidx+1)*KC], p, preferred_element_type=F32)
                accs[(u, qt)] = d if cidx == 0 else accs[(u, qt)] + d
                la = laccs.get((u, qt), [None, None, None])
                idx = jnp.full((KC, 128), UN * t + u, jnp.int32)
                vbs = [jnp.take_along_axis(vl_ref[r, cidx*KC:(cidx+1)*KC, :], idx, axis=1) for r in range(2)]
                for gi in range(KC // 8):
                    pg = p32[gi*8:(gi+1)*8, :]
                    la[2] = pg if la[2] is None else la[2] + pg
                    for r in range(2):
                        vb = vbs[r][gi*8:(gi+1)*8, :]
                        term = pg * jnp.concatenate([vb] * (TQ // 128), axis=1)
                        la[r] = term if la[r] is None else la[r] + term
                laccs[(u, qt)] = la
                if cidx == NC - 1:
                    finish_store(UN * t + u, accs.pop((u, qt)), laccs.pop((u, qt)), qt)
            for n in range(len(items) + LA):
                if n < len(items):
                    qk(n)
                if n >= LA:
                    pv(n - LA)
            return c

        def slow_tile(i, c):
            h = i // (S // SQ)
            q0 = pl.multiple_of((i % (S // SQ)) * SQ, SQ)
            r0 = pl.multiple_of(16 * h, 16)
            l0 = pl.multiple_of(512 + h // 16 * 16, 16)
            off = h % 16
            ones_row = (off + 1) % 16
            row16 = jax.lax.broadcasted_iota(jnp.int32, (16, S), 0)
            vl = vT_ref[pl.ds(l0, 16), :]
            vl = jnp.where(row16 == ones_row, jnp.ones_like(vl), vl)
            vw = jnp.concatenate([vT_ref[pl.ds(r0, 16), :], vl, vT_ref[pl.ds(l0 + 32, 16), :]], axis=0)
            sT = jnp.dot(k_ref[h, :, 0:32], qT_ref[h, :, pl.ds(q0, SQ)], preferred_element_type=F32)
            mx = jnp.max(sT, axis=0, keepdims=True)
            p = jnp.exp2(sT - mx).astype(BF)
            acc = jnp.dot(vw, p, preferred_element_type=F32)
            r16 = jax.lax.broadcasted_iota(jnp.int32, (16, SQ), 0)
            lo = acc[16:32]
            l = jnp.sum(jnp.where(r16 == ones_row, lo, 0.0), axis=0, keepdims=True)
            inv = 1.0 / l
            oT_ref[pl.ds(r0, 16), pl.ds(q0, SQ)] = acc[0:16] * inv
            store_left(h, jnp.sum(jnp.where(r16 == off, lo, 0.0), axis=0, keepdims=True) * inv,
                       jnp.sum(jnp.where(r16 == off, acc[32:48], 0.0), axis=0, keepdims=True) * inv, pl.ds(q0, SQ), SQ)
            return c

        qmax = jnp.max(am_ref[0])
        kmax = jnp.max(am_ref[1])
        vmax = jnp.max(am_ref[2])
        safe = jnp.logical_and(qmax * kmax * (DH * 1.02) <= TB, vmax <= 2.0 ** 30)
        if FORCE_SLOW:
            safe = jnp.logical_and(safe, qmax < 0.0)

        @pl.when(safe)
        def _():
            jax.lax.fori_loop(0, HH // UN, body, 0)

        @pl.when(jnp.logical_not(safe))
        def _():
            jax.lax.fori_loop(0, H * (S // SQ), slow_tile, 0)

        cp_wo.wait()
        wo = wo_ref[...].astype(F32)
        wo = jnp.concatenate([wo[18*h:18*h+16] for h in range(H)] + [wo[18*h+16:18*h+17] for h in range(H)] + [wo[18*h+17:18*h+18] for h in range(H)], axis=0).astype(BF)
        wo_p = jnp.concatenate([jnp.zeros((D, 64), BF), wo], axis=1)
        lane = jax.lax.broadcasted_iota(jnp.int32, (OC, 128), 1)
        cps = []
        for oc in range(S // OC):
            rs = slice(oc*OC, (oc+1)*OC)
            oT = oT_ref[:, rs].astype(BF)
            yb = jax.lax.dot_general(oT, wo_p, (((0,), (0,)), ((), ())), preferred_element_type=F32)
            ob_ref[rs, 512:640] = jnp.where(lane < 64, ob_ref[rs, 512:640], yb[:, 0:128].astype(BF))
            ob_ref[rs, 640:1152] = yb[:, 128:640].astype(BF)
            cp = pltpu.make_async_copy(ob_ref.at[rs, 512:1152], o_hbm.at[rs, 512:1152], out_sems.at[1 + oc])
            cp.start()
            cps.append(cp)
        cp_oa.wait()
        for cp in cps:
            cp.wait()

    f1, m, finv = _consts()

    @jax.jit
    def f(A_x, A_w_r, A_w_i, B_x, B_wqkv, B_wo):
        xaT = A_x[0].T
        xbT = B_x[0].T
        anyspec = pl.BlockSpec(memory_space=pl.ANY)
        out = pl.pallas_call(kern, out_shape=jax.ShapeDtypeStruct((S, 2 * D), BF),
            in_specs=[anyspec] * 9, out_specs=anyspec,
            scratch_shapes=[pltpu.VMEM((D, S), BF), pltpu.VMEM((DF, S), BF), pltpu.VMEM((DF, S), BF), pltpu.VMEM((D, S), BF),
                            pltpu.VMEM((D, 3 * D), BF), pltpu.VMEM((D, D), BF), pltpu.VMEM((2 * R, D), BF),
                            pltpu.VMEM((N1, 256, 256), BF), pltpu.VMEM((2 * R, 640), BF), pltpu.VMEM((S, 2 * D), BF),
                            pltpu.VMEM((H, 32, S), BF), pltpu.VMEM((H, S, 128), BF),
                            pltpu.VMEM((D, S), BF), pltpu.VMEM((D, S), F32),
                            pltpu.VMEM((2 * R, S), F32), pltpu.VMEM((N1, R, 256), BF), pltpu.VMEM((2 * R, S), BF),
                            pltpu.VMEM((2, 3, S, 128), F32), pltpu.VMEM((2, R, S), F32),
                            pltpu.VMEM((S, D), BF), pltpu.VMEM((640 + D, D), BF), pltpu.VMEM((3, 8, 128), F32), pltpu.VMEM((2, S, 128), F32), pltpu.VMEM((8, 128), F32),
                            pltpu.SemaphoreType.DMA((12,)), pltpu.SemaphoreType.DMA((1 + S // OC,))],
            compiler_params=pltpu.CompilerParams(vmem_limit_bytes=110 << 20))(
                xaT, A_w_r.T, A_w_i.T, xbT, B_wqkv, B_wo, jnp.asarray(f1), jnp.asarray(m), jnp.asarray(finv))
        return out[None]
    return f


_impl = make()


def pallas_concat_heads__spectral_gfnet__mha_block__prompt_kernel(A_x, A_w_r, A_w_i, B_x, B_wqkv, B_wo):
    return _impl(A_x, A_w_r, A_w_i, B_x, B_wqkv, B_wo)
```

```python
import functools, math
import numpy as np
import jax, jax.numpy as jnp
from jax.experimental import pallas as pl
from jax.experimental.pallas import tpu as pltpu

S, D, H, DH = 2048, 576, 32, 18
DF = D // 2 + 1
R = 304
N1, N2 = 16, 128
LOG2E = 1.4426950408889634
BF = jnp.bfloat16
F32 = jnp.float32


RE, RO, HD = 160, 144, D // 2


def _consts():
    r = np.arange(R)
    f = np.where(r < RE, 2 * r, 2 * (r - RE) + 1).astype(np.float64)[:, None]
    valid = (f < DF)
    d = np.arange(HD)[None, :].astype(np.float64)
    ang = 2 * np.pi * ((f * d) % D) / D
    c_, s_ = np.where(valid, np.cos(ang), 0.0), np.where(valid, -np.sin(ang), 0.0)
    f1 = np.concatenate([c_[:RE], s_[:RE], c_[RE:], s_[RE:]], axis=0)
    cf = np.where((f == 0) | (f == DF - 1), 1.0, 2.0) / (S * D)
    ci, si = cf * c_, cf * s_
    finv = np.concatenate([ci[:RE], si[:RE], ci[RE:], si[RE:]], axis=0).T
    n2 = np.arange(N2)[:, None]
    k2 = np.arange(N2)[None, :]
    ms = []
    for k1 in range(N1):
        th = 2 * np.pi * ((n2 * (k1 + N1 * k2)) % S) / S
        c, s = np.cos(th), np.sin(th)
        ms.append(np.block([[c, -s], [s, c]]))
    m = np.stack(ms)
    return (f1.astype(BF), m.astype(BF), np.ascontiguousarray(finv).astype(BF))


def _cmul_const(a, w):
    ar, ai = a
    wr, wi = float(np.real(w)), float(np.imag(w))
    eps = 1e-12
    if abs(wi) < eps and abs(wr - 1) < eps:
        return ar, ai
    if abs(wi) < eps and abs(wr + 1) < eps:
        return -ar, -ai
    if abs(wr) < eps and abs(wi + 1) < eps:
        return ai, -ar
    if abs(wr) < eps and abs(wi - 1) < eps:
        return -ai, ar
    if abs(abs(wr) - abs(wi)) < eps:
        c = abs(wr)
        sr, si = np.sign(wr), np.sign(wi)
        t1 = (ar - ai) if sr * si > 0 else (ar + ai)
        t2 = (ar + ai) if sr * si > 0 else (ar - ai)
        return t1 * (c * sr), t2 * (c * si)
    return ar * wr - ai * wi, ar * wi + ai * wr


def _fft_list(xs, sign):
    n = len(xs)
    if n == 1:
        return xs
    ev = _fft_list(xs[0::2], sign)
    od = _fft_list(xs[1::2], sign)
    out = [None] * n
    for k in range(n // 2):
        t = _cmul_const(od[k], np.exp(sign * 2j * np.pi * k / n))
        out[k] = (ev[k][0] + t[0], ev[k][1] + t[1])
        out[k + n // 2] = (ev[k][0] - t[0], ev[k][1] - t[1])
    return out


def make(TQ=1024, KC=128, RC=16, OC=512, HH=H, UN=2, LA=1, PC=512, TB=40.0, FORCE_SLOW=False, SQ=128, L5=1024, MU=2):
    NQ = S // TQ
    NC = S // KC
    XC = 4

    def kern(xa_hbm, wr_hbm, wi_hbm, xb_hbm, w_hbm, wo_hbm, f1_hbm, m_hbm, finv_hbm, o_hbm,
             xa_ref, wr_ref, wi_ref, xb_ref, w_ref, wo_ref, f1_ref, m_ref, finv_ref, ob_ref,
             qT_ref, k_ref, vT_ref, oT_ref, xf_ref, t_ref, g_ref, wn_ref, wp_ref, x_ref, wT_ref, am_ref, vl_ref, yT_ref, wk_ref,
             in_sems, out_sems):
        cp_f1 = pltpu.make_async_copy(f1_hbm, f1_ref, in_sems.at[0])
        cp_xa = [pltpu.make_async_copy(xa_hbm.at[:, c*(S//XC):(c+1)*(S//XC)], xa_ref.at[:, c*(S//XC):(c+1)*(S//XC)], in_sems.at[1 + c]) for c in range(XC)]
        cp_wr = pltpu.make_async_copy(wr_hbm, wr_ref, in_sems.at[5])
        cp_wi = pltpu.make_async_copy(wi_hbm, wi_ref, in_sems.at[6])
        cp_m = pltpu.make_async_copy(m_hbm, m_ref, in_sems.at[7])
        cp_finv = pltpu.make_async_copy(finv_hbm, finv_ref, in_sems.at[8])
        cp_xb = pltpu.make_async_copy(xb_hbm, xb_ref, in_sems.at[9])
        cp_w = pltpu.make_async_copy(w_hbm.at[:, 0:640], w_ref.at[:, 0:640], in_sems.at[10])
        cp_w2 = pltpu.make_async_copy(w_hbm.at[:, 640:3*D], w_ref.at[:, 640:3*D], in_sems.at[12])
        cp_wo = pltpu.make_async_copy(wo_hbm, wo_ref, in_sems.at[11])
        for cp in [cp_f1, cp_xa[0]]:
            cp.start()

        c = (DH ** -0.5) * LOG2E
        am_ref[...] = jnp.zeros_like(am_ref)
        frow = jax.lax.broadcasted_iota(jnp.int32, (R - 256, 128), 0)

        def wperm_a(a):
            wref = (wr_ref, wi_ref)[a]
            wn_ref[a, 0] = wref[0:128, :].T.astype(F32)
            wn_ref[a, 1] = wref[128:256, :].T.astype(F32)
            wn_ref[a, 2, :, 0:DF-256] = wref[256:DF, :].T.astype(F32)
        def wperm_b(a, k1):
            for j in range(2):
                wp_ref[a, k1, j*128:(j+1)*128, :] = wn_ref[a, j, pl.ds(k1, N2, stride=N1), :].T
            blk = wn_ref[a, 2, pl.ds(k1, N2, stride=N1), :].T[0:R-256, :]
            wp_ref[a, k1, 256:R, :] = jnp.where(frow < DF - 256, blk, 0.0)

        def stage_a_fwd(rc):
            r0 = rc * RC
            xs = [(xf_ref[r0:r0+RC, n1*128:(n1+1)*128], xf_ref[R+r0:R+r0+RC, n1*128:(n1+1)*128]) for n1 in range(N1)]
            ys = _fft_list(xs, -1)
            for k1 in range(N1):
                t_ref[k1, r0:r0+RC, 0:128] = ys[k1][0].astype(BF)
                t_ref[k1, r0:r0+RC, 128:256] = ys[k1][1].astype(BF)

        def stage_a_inv(rc):
            r0 = rc * RC
            xs = [(xf_ref[r0:r0+RC, k1*128:(k1+1)*128], xf_ref[R+r0:R+r0+RC, k1*128:(k1+1)*128]) for k1 in range(N1)]
            ys = _fft_list(xs, +1)
            gr0, gi0 = (r0, RE + r0) if r0 < RE else (RE + r0, RE + RO + r0)
            for n1 in range(N1):
                g_ref[gr0:gr0+RC, n1*128:(n1+1)*128] = ys[n1][0].astype(BF)
                g_ref[gi0:gi0+RC, n1*128:(n1+1)*128] = ys[n1][1].astype(BF)

        def track(idx, val):
            a = jnp.abs(val)
            a = jnp.max(a.reshape(a.shape[0] // 8, 8, a.shape[1]), axis=0)
            a = functools.reduce(jnp.maximum, [a[:, l*128:(l+1)*128] for l in range(a.shape[1] // 128)])
            am_ref[idx] = jnp.maximum(am_ref[idx], a)
        def proj_k(g, pc):
            wk = wk_ref[:, 128*g:128*(g+1)]
            kk = jnp.dot(x_ref[pc*PC:(pc+1)*PC, :], wk, preferred_element_type=F32)
            track(1, kk)
            kb = kk.astype(BF)
            k32 = pltpu.bitcast(kb, jnp.uint32)
            for j in range(min(7, H - 7 * g)):
                kr = kb if j == 0 else pltpu.bitcast(pltpu.roll(k32, 128 - 18 * j, 1), BF)
                k_ref[7*g + j, pc*PC:(pc+1)*PC, :] = kr
        def proj_q(g, pc):
            qT = jnp.dot(wT_ref[128*g:128*(g+1), :], xb_ref[:, pc*PC:(pc+1)*PC], preferred_element_type=F32) * c
            track(0, qT)
            for j in range(min(7, H - 7 * g)):
                qT_ref[7*g + j, :, pc*PC:(pc+1)*PC] = jnp.concatenate([qT[18*j:18*j+18], jnp.zeros((14, PC), F32)], axis=0).astype(BF)
        def proj_v(r, pc):
            rr = slice(640 + r*192, 640 + (r+1)*192)
            vv = jnp.dot(wT_ref[rr, :], xb_ref[:, pc*PC:(pc+1)*PC], preferred_element_type=F32)
            track(2, vv)
            vT_ref[r*192:(r+1)*192, pc*PC:(pc+1)*PC] = vv.astype(BF)

        def interleave(mx, vp):
            n = max(len(mx), 1)
            done = 0
            for i, f in enumerate(mx):
                f()
                upto = (i + 1) * len(vp) // n
                for g_ in vp[done:upto]:
                    g_()
                done = upto
            for g_ in vp[done:]:
                g_()

        cp_f1.wait()
        cp_xa[0].wait()
        for cp in cp_xa[1:] + [cp_xb, cp_w]:
            cp.start()
        for cc in range(XC):
            if cc > 0:
                cp_xa[cc].wait()
            sl = slice(cc*(S//XC), (cc+1)*(S//XC))
            x0 = xa_ref[0:HD, sl].astype(F32)
            x1 = xa_ref[HD:D, sl].astype(F32)
            xe = jnp.dot(f1_ref[0:2*RE, :], (x0 + x1).astype(BF), preferred_element_type=F32)
            xo = jnp.dot(f1_ref[2*RE:2*R, :], (x0 - x1).astype(BF), preferred_element_type=F32)
            xf_ref[0:RE, sl] = xe[0:RE]
            xf_ref[R:R+RE, sl] = xe[RE:2*RE]
            xf_ref[RE:R, sl] = xo[0:RO]
            xf_ref[R+RE:2*R, sl] = xo[RO:2*RO]
        for rc in range(R // RC):
            stage_a_fwd(rc)
        cp_xb.wait()
        cp_w.wait()
        for cp in [cp_w2, cp_wr, cp_wi, cp_m, cp_finv, cp_wo]:
            cp.start()
        for g in range(5):
            wT_ref[128*g:128*(g+1), :] = w_ref[:, 126*g:126*g+128].T
        x_ref[...] = xb_ref[...].T
        NPC = S // PC
        mx1 = [functools.partial(proj_q, g, pc) for g in range(5) for pc in range(NPC)] + [functools.partial(proj_v, 0, pc) for pc in range(NPC)]
        for f_ in mx1[:2*NPC]:
            f_()
        cp_w2.wait()
        wvT = w_ref[:, 1152:1728].T.astype(F32)
        wT_ref[640:640+512, :] = jnp.concatenate([wvT[18*h:18*h+16] for h in range(H)], axis=0).astype(BF)
        wT_ref[640+512:640+D, :] = jnp.concatenate([wvT[18*h+16:18*h+17] for h in range(H)] + [wvT[18*h+17:18*h+18] for h in range(H)], axis=0).astype(BF)
        for g in range(5):
            wk_ref[:, 128*g:128*(g+1)] = w_ref[:, 576+126*g:576+126*g+128]
        cp_wr.wait()
        cp_wi.wait()
        vp = [functools.partial(wperm_a, 0), functools.partial(wperm_a, 1)] + [functools.partial(wperm_b, a, k1) for a in range(2) for k1 in range(N1)]
        interleave(mx1[2*NPC:], vp)
        cp_m.wait()

        def mid(k1, carry):
            c0 = pl.multiple_of(k1 * 128, 128)
            mk = m_ref[k1]
            z = jnp.dot(t_ref[k1], mk, preferred_element_type=F32)
            zr, zi = z[:, :128], z[:, 128:]
            wr, wi = [jnp.concatenate([wp_ref[a, k1, pl.ds(0, 152, stride=2), :], jnp.zeros((8, 128), F32),
                                       wp_ref[a, k1, pl.ds(1, RO, stride=2), :]], axis=0) for a in range(2)]
            yr = zr * wr - zi * wi
            yi = zr * wi + zi * wr
            y = jnp.concatenate([yr, yi], axis=1).astype(BF)
            tp = jax.lax.dot_general(y, mk, (((1,), (1,)), ((), ())), preferred_element_type=F32)
            xf_ref[0:R, pl.ds(c0, 128)] = tp[:, :128]
            xf_ref[R:2*R, pl.ds(c0, 128)] = tp[:, 128:]
            return carry
        jax.lax.fori_loop(0, N1, mid, 0, unroll=MU)

        mx2 = [functools.partial(proj_k, g, pc) for g in range(5) for pc in range(NPC)] + [functools.partial(proj_v, r, pc) for r in (1, 2) for pc in range(NPC)]
        interleave(mx2, [functools.partial(stage_a_inv, rc) for rc in range(R // RC)])
        vlt = vT_ref[512:D, :].T.astype(F32) * (2.0 ** TB)
        vlt = jnp.concatenate([vlt, jnp.zeros((S, 64), F32)], axis=1)
        vl_ref[0] = vlt
        vl_ref[1] = pltpu.roll(vlt, 96, 1)
        oT_ref[512:D, :] = jnp.zeros((64, S), F32)
        cp_finv.wait()
        for pc in range(S // L5):
            sl = slice(pc * L5, (pc + 1) * L5)
            ee = jnp.dot(finv_ref[:, 0:2*RE], g_ref[0:2*RE, sl], preferred_element_type=F32)
            oo = jnp.dot(finv_ref[:, 2*RE:2*R], g_ref[2*RE:2*R, sl], preferred_element_type=F32)
            yT_ref[0:HD, sl] = (ee + oo).astype(BF)
            yT_ref[HD:D, sl] = (ee - oo).astype(BF)
            for t_ in range(4):
                ob_ref[sl, 128*t_:128*(t_+1)] = yT_ref[128*t_:128*(t_+1), sl].T
        cp_oa = pltpu.make_async_copy(ob_ref.at[:, 0:512], o_hbm.at[:, 0:512], out_sems.at[0])
        cp_oa.start()

        def prep_finish(h, u):
            r0 = pl.multiple_of(16 * h, 16)
            vw = (vT_ref[pl.ds(r0, 16), :].astype(F32) * (2.0 ** TB)).astype(BF)
            return vw

        def store_left(h, a0, a1, qsl, n):
            o8 = h % 8
            r8 = jax.lax.broadcasted_iota(jnp.int32, (8, n), 0)
            for base, a in ((512, a0), (544, a1)):
                l8 = pl.multiple_of(base + h // 8 * 8, 8)
                oT_ref[pl.ds(l8, 8), qsl] = jnp.where(r8 == o8, a, oT_ref[pl.ds(l8, 8), qsl])

        def finish_store(h, acc, lacc, qt):
            r0 = pl.multiple_of(16 * h, 16)
            l = jnp.sum(lacc[2], axis=0, keepdims=True) * (2.0 ** TB)
            inv = 1.0 / l
            oT_ref[pl.ds(r0, 16), qt*TQ:(qt+1)*TQ] = acc * inv
            store_left(h, jnp.sum(lacc[0], axis=0, keepdims=True) * inv, jnp.sum(lacc[1], axis=0, keepdims=True) * inv, slice(qt*TQ, (qt+1)*TQ), TQ)

        def body(t, c):
            items = [(u, qt, cidx) for u in range(UN) for qt in range(NQ) for cidx in range(NC)]
            vws = {}; qms = {}; ss = {}; accs = {}; laccs = {}
            for u in range(UN):
                vws[u] = prep_finish(UN * t + u, u)
            def qk(n):
                u, qt, cidx = items[n]
                h = UN * t + u
                ss[n] = jnp.dot(k_ref[h, cidx*KC:(cidx+1)*KC, 0:32], qT_ref[h, :, qt*TQ:(qt+1)*TQ], preferred_element_type=F32)
            def pv(n):
                u, qt, cidx = items[n]
                vw = vws[u]
                p32 = jnp.exp2(ss.pop(n))
                p = p32.astype(BF)
                d = jnp.dot(vw[:, cidx*KC:(cidx+1)*KC], p, preferred_element_type=F32)
                accs[(u, qt)] = d if cidx == 0 else accs[(u, qt)] + d
                la = laccs.get((u, qt), [None, None, None])
                idx = jnp.full((KC, 128), UN * t + u, jnp.int32)
                vbs = [jnp.take_along_axis(vl_ref[r, cidx*KC:(cidx+1)*KC, :], idx, axis=1) for r in range(2)]
                for gi in range(KC // 8):
                    pg = p32[gi*8:(gi+1)*8, :]
                    la[2] = pg if la[2] is None else la[2] + pg
                    for r in range(2):
                        vb = vbs[r][gi*8:(gi+1)*8, :]
                        term = pg * jnp.concatenate([vb] * (TQ // 128), axis=1)
                        la[r] = term if la[r] is None else la[r] + term
                laccs[(u, qt)] = la
                if cidx == NC - 1:
                    finish_store(UN * t + u, accs.pop((u, qt)), laccs.pop((u, qt)), qt)
            for n in range(len(items) + LA):
                if n < len(items):
                    qk(n)
                if n >= LA:
                    pv(n - LA)
            return c

        def slow_tile(i, c):
            h = i // (S // SQ)
            q0 = pl.multiple_of((i % (S // SQ)) * SQ, SQ)
            r0 = pl.multiple_of(16 * h, 16)
            l0 = pl.multiple_of(512 + h // 16 * 16, 16)
            off = h % 16
            ones_row = (off + 1) % 16
            row16 = jax.lax.broadcasted_iota(jnp.int32, (16, S), 0)
            vl = vT_ref[pl.ds(l0, 16), :]
            vl = jnp.where(row16 == ones_row, jnp.ones_like(vl), vl)
            vw = jnp.concatenate([vT_ref[pl.ds(r0, 16), :], vl, vT_ref[pl.ds(l0 + 32, 16), :]], axis=0)
            sT = jnp.dot(k_ref[h, :, 0:32], qT_ref[h, :, pl.ds(q0, SQ)], preferred_element_type=F32)
            mx = jnp.max(sT, axis=0, keepdims=True)
            p = jnp.exp2(sT - mx).astype(BF)
            acc = jnp.dot(vw, p, preferred_element_type=F32)
            r16 = jax.lax.broadcasted_iota(jnp.int32, (16, SQ), 0)
            lo = acc[16:32]
            l = jnp.sum(jnp.where(r16 == ones_row, lo, 0.0), axis=0, keepdims=True)
            inv = 1.0 / l
            oT_ref[pl.ds(r0, 16), pl.ds(q0, SQ)] = acc[0:16] * inv
            store_left(h, jnp.sum(jnp.where(r16 == off, lo, 0.0), axis=0, keepdims=True) * inv,
                       jnp.sum(jnp.where(r16 == off, acc[32:48], 0.0), axis=0, keepdims=True) * inv, pl.ds(q0, SQ), SQ)
            return c

        qmax = jnp.max(am_ref[0])
        kmax = jnp.max(am_ref[1])
        vmax = jnp.max(am_ref[2])
        safe = jnp.logical_and(qmax * kmax * (DH * 1.02) <= TB, vmax <= 2.0 ** 30)
        if FORCE_SLOW:
            safe = jnp.logical_and(safe, qmax < 0.0)

        @pl.when(safe)
        def _():
            jax.lax.fori_loop(0, HH // UN, body, 0)

        @pl.when(jnp.logical_not(safe))
        def _():
            jax.lax.fori_loop(0, H * (S // SQ), slow_tile, 0)

        cp_wo.wait()
        wo = wo_ref[...].astype(F32)
        wo = jnp.concatenate([wo[18*h:18*h+16] for h in range(H)] + [wo[18*h+16:18*h+17] for h in range(H)] + [wo[18*h+17:18*h+18] for h in range(H)], axis=0).astype(BF)
        woT = wo.T
        cps = []
        for oc in range(S // OC):
            rs = slice(oc*OC, (oc+1)*OC)
            yT_ref[D:2*D, rs] = jnp.dot(woT, oT_ref[:, rs].astype(BF), preferred_element_type=F32).astype(BF)
            for t_ in range(4, 9):
                ob_ref[rs, 128*t_:128*(t_+1)] = yT_ref[128*t_:128*(t_+1), rs].T
            cp = pltpu.make_async_copy(ob_ref.at[rs, 512:1152], o_hbm.at[rs, 512:1152], out_sems.at[1 + oc])
            cp.start()
            cps.append(cp)
        cp_oa.wait()
        for cp in cps:
            cp.wait()

    f1, m, finv = _consts()

    @jax.jit
    def f(A_x, A_w_r, A_w_i, B_x, B_wqkv, B_wo):
        xaT = A_x[0].T
        xbT = B_x[0].T
        anyspec = pl.BlockSpec(memory_space=pl.ANY)
        out = pl.pallas_call(kern, out_shape=jax.ShapeDtypeStruct((S, 2 * D), BF),
            in_specs=[anyspec] * 9, out_specs=anyspec,
            scratch_shapes=[pltpu.VMEM((D, S), BF), pltpu.VMEM((DF, S), BF), pltpu.VMEM((DF, S), BF), pltpu.VMEM((D, S), BF),
                            pltpu.VMEM((D, 3 * D), BF), pltpu.VMEM((D, D), BF), pltpu.VMEM((2 * R, HD), BF),
                            pltpu.VMEM((N1, 256, 256), BF), pltpu.VMEM((HD, 2 * R), BF), pltpu.VMEM((S, 2 * D), BF),
                            pltpu.VMEM((H, 32, S), BF), pltpu.VMEM((H, S, 128), BF),
                            pltpu.VMEM((D, S), BF), pltpu.VMEM((D, S), F32),
                            pltpu.VMEM((2 * R, S), F32), pltpu.VMEM((N1, R, 256), BF), pltpu.VMEM((2 * R, S), BF),
                            pltpu.VMEM((2, 3, S, 128), F32), pltpu.VMEM((2, N1, R, 128), F32),
                            pltpu.VMEM((S, D), BF), pltpu.VMEM((640 + D, D), BF), pltpu.VMEM((3, 8, 128), F32), pltpu.VMEM((2, S, 128), F32), pltpu.VMEM((2 * D, S), BF), pltpu.VMEM((D, 640), BF),
                            pltpu.SemaphoreType.DMA((13,)), pltpu.SemaphoreType.DMA((1 + S // OC,))],
            compiler_params=pltpu.CompilerParams(vmem_limit_bytes=110 << 20))(
                xaT, A_w_r.T, A_w_i.T, xbT, B_wqkv, B_wo, jnp.asarray(f1), jnp.asarray(m), jnp.asarray(finv))
        return out[None]
    return f


_impl = make()


def pallas_concat_heads__spectral_gfnet__mha_block__prompt_kernel(A_x, A_w_r, A_w_i, B_x, B_wqkv, B_wo):
    return _impl(A_x, A_w_r, A_w_i, B_x, B_wqkv, B_wo)
```

```python
import functools

import numpy as np
import jax
import jax.numpy as jnp
from jax.experimental import pallas as pl
from jax.experimental.pallas import tpu as pltpu

S, D, H, DH = 2048, 576, 32, 18
DF = D // 2 + 1
HD = D // 2
RE, RO = 160, 144
R = RE + RO
N1, N2 = 16, 128
LOG2E = 1.4426950408889634
BF = jnp.bfloat16
F32 = jnp.float32

TQ, KC, UN = 1024, 128, 2
RC = 16
PC = 512
XC = 4
OC = 512
L5 = 1024
SQ = 128
TB = 40.0


def _consts():
    r = np.arange(R)
    f = np.where(r < RE, 2 * r, 2 * (r - RE) + 1).astype(np.float64)[:, None]
    valid = (f < DF)
    d = np.arange(HD)[None, :].astype(np.float64)
    ang = 2 * np.pi * ((f * d) % D) / D
    c_, s_ = np.where(valid, np.cos(ang), 0.0), np.where(valid, -np.sin(ang), 0.0)
    f1 = np.concatenate([c_[:RE], s_[:RE], c_[RE:], s_[RE:]], axis=0)
    cf = np.where((f == 0) | (f == DF - 1), 1.0, 2.0) / (S * D)
    ci, si = cf * c_, cf * s_
    finv = np.concatenate([ci[:RE], si[:RE], ci[RE:], si[RE:]], axis=0).T
    n2 = np.arange(N2)[:, None]
    k2 = np.arange(N2)[None, :]
    ms = []
    for k1 in range(N1):
        th = 2 * np.pi * ((n2 * (k1 + N1 * k2)) % S) / S
        c, s = np.cos(th), np.sin(th)
        ms.append(np.block([[c, -s], [s, c]]))
    m = np.stack(ms)
    return (f1.astype(BF), m.astype(BF), np.ascontiguousarray(finv).astype(BF))


def _cmul_const(a, w):
    ar, ai = a
    wr, wi = float(np.real(w)), float(np.imag(w))
    eps = 1e-12
    if abs(wi) < eps and abs(wr - 1) < eps:
        return ar, ai
    if abs(wi) < eps and abs(wr + 1) < eps:
        return -ar, -ai
    if abs(wr) < eps and abs(wi + 1) < eps:
        return ai, -ar
    if abs(wr) < eps and abs(wi - 1) < eps:
        return -ai, ar
    if abs(abs(wr) - abs(wi)) < eps:
        c = abs(wr)
        sr, si = np.sign(wr), np.sign(wi)
        t1 = (ar - ai) if sr * si > 0 else (ar + ai)
        t2 = (ar + ai) if sr * si > 0 else (ar - ai)
        return t1 * (c * sr), t2 * (c * si)
    return ar * wr - ai * wi, ar * wi + ai * wr


def _fft_list(xs, sign):
    n = len(xs)
    if n == 1:
        return xs
    ev = _fft_list(xs[0::2], sign)
    od = _fft_list(xs[1::2], sign)
    out = [None] * n
    for k in range(n // 2):
        t = _cmul_const(od[k], np.exp(sign * 2j * np.pi * k / n))
        out[k] = (ev[k][0] + t[0], ev[k][1] + t[1])
        out[k + n // 2] = (ev[k][0] - t[0], ev[k][1] - t[1])
    return out


def _split_heads_rows(a):
    return jnp.concatenate([a[18*h:18*h+16] for h in range(H)] + [a[18*h+16:18*h+17] for h in range(H)]
                           + [a[18*h+17:18*h+18] for h in range(H)], axis=0)


def _kernel(xa_hbm, wr_hbm, wi_hbm, xb_hbm, w_hbm, wo_hbm, f1_hbm, m_hbm, finv_hbm, o_hbm,
            xa_ref, wr_ref, wi_ref, xb_ref, w_ref, wo_ref, f1_ref, m_ref, finv_ref, ob_ref,
            qT_ref, k_ref, vT_ref, oT_ref, xf_ref, t_ref, g_ref, wn_ref, wp_ref, x_ref, wT_ref, am_ref,
            vl_ref, yT_ref, wk_ref, woT_ref, in_sems, out_sems):
    NQ = S // TQ
    NC = S // KC
    NPC = S // PC
    cp_f1 = pltpu.make_async_copy(f1_hbm, f1_ref, in_sems.at[0])
    cp_xa = [pltpu.make_async_copy(xa_hbm.at[:, c*(S//XC):(c+1)*(S//XC)], xa_ref.at[:, c*(S//XC):(c+1)*(S//XC)],
                                   in_sems.at[1 + c]) for c in range(XC)]
    cp_wr = pltpu.make_async_copy(wr_hbm, wr_ref, in_sems.at[5])
    cp_wi = pltpu.make_async_copy(wi_hbm, wi_ref, in_sems.at[6])
    cp_m = pltpu.make_async_copy(m_hbm, m_ref, in_sems.at[7])
    cp_finv = pltpu.make_async_copy(finv_hbm, finv_ref, in_sems.at[8])
    cp_xb = pltpu.make_async_copy(xb_hbm, xb_ref, in_sems.at[9])
    cp_w = pltpu.make_async_copy(w_hbm.at[:, 0:640], w_ref.at[:, 0:640], in_sems.at[10])
    cp_w2 = pltpu.make_async_copy(w_hbm.at[:, 640:3*D], w_ref.at[:, 640:3*D], in_sems.at[12])
    cp_wo = pltpu.make_async_copy(wo_hbm, wo_ref, in_sems.at[11])
    for cp in [cp_f1, cp_xa[0]]:
        cp.start()

    c = (DH ** -0.5) * LOG2E
    am_ref[...] = jnp.zeros_like(am_ref)
    frow = jax.lax.broadcasted_iota(jnp.int32, (R - 256, 128), 0)

    def wperm_a(a):
        wref = (wr_ref, wi_ref)[a]
        wn_ref[a, 0] = wref[0:128, :].T.astype(F32)
        wn_ref[a, 1] = wref[128:256, :].T.astype(F32)
        wn_ref[a, 2, :, 0:DF-256] = wref[256:DF, :].T.astype(F32)

    def wperm_b(a, k1):
        for j in range(2):
            wp_ref[a, k1, j*128:(j+1)*128, :] = wn_ref[a, j, pl.ds(k1, N2, stride=N1), :].T
        blk = wn_ref[a, 2, pl.ds(k1, N2, stride=N1), :].T[0:R-256, :]
        wp_ref[a, k1, 256:R, :] = jnp.where(frow < DF - 256, blk, 0.0)

    def stage_a_fwd(rc):
        r0 = rc * RC
        xs = [(xf_ref[r0:r0+RC, n1*128:(n1+1)*128], xf_ref[R+r0:R+r0+RC, n1*128:(n1+1)*128]) for n1 in range(N1)]
        ys = _fft_list(xs, -1)
        for k1 in range(N1):
            t_ref[k1, r0:r0+RC, 0:128] = ys[k1][0].astype(BF)
            t_ref[k1, r0:r0+RC, 128:256] = ys[k1][1].astype(BF)

    def stage_a_inv(rc):
        r0 = rc * RC
        xs = [(xf_ref[r0:r0+RC, k1*128:(k1+1)*128], xf_ref[R+r0:R+r0+RC, k1*128:(k1+1)*128]) for k1 in range(N1)]
        ys = _fft_list(xs, +1)
        gr0, gi0 = (r0, RE + r0) if r0 < RE else (RE + r0, RE + RO + r0)
        for n1 in range(N1):
            g_ref[gr0:gr0+RC, n1*128:(n1+1)*128] = ys[n1][0].astype(BF)
            g_ref[gi0:gi0+RC, n1*128:(n1+1)*128] = ys[n1][1].astype(BF)

    def track(idx, val):
        a = jnp.abs(val)
        a = jnp.max(a.reshape(a.shape[0] // 8, 8, a.shape[1]), axis=0)
        a = functools.reduce(jnp.maximum, [a[:, l*128:(l+1)*128] for l in range(a.shape[1] // 128)])
        am_ref[idx] = jnp.maximum(am_ref[idx], a)

    def proj_k(g, pc):
        wk = wk_ref[:, 128*g:128*(g+1)]
        kk = jnp.dot(x_ref[pc*PC:(pc+1)*PC, :], wk, preferred_element_type=F32)
        track(1, kk)
        kb = kk.astype(BF)
        k32 = pltpu.bitcast(kb, jnp.uint32)
        for j in range(min(7, H - 7 * g)):
            kr = kb if j == 0 else pltpu.bitcast(pltpu.roll(k32, 128 - 18 * j, 1), BF)
            k_ref[7*g + j, pc*PC:(pc+1)*PC, :] = kr

    def proj_q(g, pc):
        qT = jnp.dot(wT_ref[128*g:128*(g+1), :], xb_ref[:, pc*PC:(pc+1)*PC], preferred_element_type=F32) * c
        track(0, qT)
        for j in range(min(7, H - 7 * g)):
            qT_ref[7*g + j, :, pc*PC:(pc+1)*PC] = jnp.concatenate(
                [qT[18*j:18*j+18], jnp.zeros((14, PC), F32)], axis=0).astype(BF)

    def proj_v(r, pc):
        rr = slice(640 + r*192, 640 + (r+1)*192)
        vv = jnp.dot(wT_ref[rr, :], xb_ref[:, pc*PC:(pc+1)*PC], preferred_element_type=F32)
        track(2, vv)
        vT_ref[r*192:(r+1)*192, pc*PC:(pc+1)*PC] = vv.astype(BF)

    def interleave(mx, vp):
        n = max(len(mx), 1)
        done = 0
        for i, f in enumerate(mx):
            f()
            upto = (i + 1) * len(vp) // n
            for g_ in vp[done:upto]:
                g_()
            done = upto
        for g_ in vp[done:]:
            g_()

    cp_f1.wait()
    cp_xa[0].wait()
    for cp in cp_xa[1:] + [cp_xb, cp_w, cp_w2, cp_wr, cp_wi, cp_m, cp_finv, cp_wo]:
        cp.start()
    for cc in range(XC):
        if cc > 0:
            cp_xa[cc].wait()
        sl = slice(cc*(S//XC), (cc+1)*(S//XC))
        x0 = xa_ref[0:HD, sl].astype(F32)
        x1 = xa_ref[HD:D, sl].astype(F32)
        xe = jnp.dot(f1_ref[0:2*RE, :], (x0 + x1).astype(BF), preferred_element_type=F32)
        xo = jnp.dot(f1_ref[2*RE:2*R, :], (x0 - x1).astype(BF), preferred_element_type=F32)
        xf_ref[0:RE, sl] = xe[0:RE]
        xf_ref[R:R+RE, sl] = xe[RE:2*RE]
        xf_ref[RE:R, sl] = xo[0:RO]
        xf_ref[R+RE:2*R, sl] = xo[RO:2*RO]
    for rc in range(R // RC):
        stage_a_fwd(rc)
    cp_xb.wait()
    cp_w.wait()

    for g in range(5):
        wT_ref[128*g:128*(g+1), :] = w_ref[:, 126*g:126*g+128].T
    x_ref[...] = xb_ref[...].T
    mx1 = ([functools.partial(proj_q, g, pc) for g in range(5) for pc in range(NPC)]
           + [functools.partial(proj_v, 0, pc) for pc in range(NPC)])
    for f_ in mx1[:2*NPC]:
        f_()
    cp_w2.wait()
    wvT = w_ref[:, 1152:1728].T.astype(F32)
    wT_ref[640:640+512, :] = jnp.concatenate([wvT[18*h:18*h+16] for h in range(H)], axis=0).astype(BF)
    wT_ref[640+512:640+D, :] = jnp.concatenate(
        [wvT[18*h+16:18*h+17] for h in range(H)] + [wvT[18*h+17:18*h+18] for h in range(H)], axis=0).astype(BF)
    for g in range(5):
        wk_ref[:, 128*g:128*(g+1)] = w_ref[:, 576+126*g:576+126*g+128]
    cp_wr.wait()
    cp_wi.wait()
    vp = ([functools.partial(wperm_a, 0), functools.partial(wperm_a, 1)]
          + [functools.partial(wperm_b, a, k1) for a in range(2) for k1 in range(N1)])
    interleave(mx1[2*NPC:], vp)
    cp_m.wait()

    def mid(k1, carry):
        c0 = pl.multiple_of(k1 * 128, 128)
        mk = m_ref[k1]
        z = jnp.dot(t_ref[k1], mk, preferred_element_type=F32)
        zr, zi = z[:, :128], z[:, 128:]
        wr, wi = [jnp.concatenate([wp_ref[a, k1, pl.ds(0, 152, stride=2), :], jnp.zeros((8, 128), F32),
                                   wp_ref[a, k1, pl.ds(1, RO, stride=2), :]], axis=0) for a in range(2)]
        yr = zr * wr - zi * wi
        yi = zr * wi + zi * wr
        y = jnp.concatenate([yr, yi], axis=1).astype(BF)
        tp = jax.lax.dot_general(y, mk, (((1,), (1,)), ((), ())), preferred_element_type=F32)
        xf_ref[0:R, pl.ds(c0, 128)] = tp[:, :128]
        xf_ref[R:2*R, pl.ds(c0, 128)] = tp[:, 128:]
        return carry
    jax.lax.fori_loop(0, N1, mid, 0, unroll=2)

    mx2 = ([functools.partial(proj_k, g, pc) for g in range(5) for pc in range(NPC)]
           + [functools.partial(proj_v, r, pc) for r in (1, 2) for pc in range(NPC)])
    interleave(mx2, [functools.partial(stage_a_inv, rc) for rc in range(R // RC)])
    vlt = vT_ref[512:D, :].T.astype(F32) * (2.0 ** TB)
    vlt = jnp.concatenate([vlt, jnp.zeros((S, 64), F32)], axis=1)
    vl_ref[0] = vlt
    vl_ref[1] = pltpu.roll(vlt, 96, 1)
    oT_ref[512:D, :] = jnp.zeros((64, S), F32)
    cp_finv.wait()
    cp_wo.wait()
    woT_ref[...] = _split_heads_rows(wo_ref[...].astype(F32)).astype(BF).T

    for pc in range(S // L5):
        sl = slice(pc * L5, (pc + 1) * L5)
        ee = jnp.dot(finv_ref[:, 0:2*RE], g_ref[0:2*RE, sl], preferred_element_type=F32)
        oo = jnp.dot(finv_ref[:, 2*RE:2*R], g_ref[2*RE:2*R, sl], preferred_element_type=F32)
        yT_ref[0:HD, sl] = (ee + oo).astype(BF)
        yT_ref[HD:D, sl] = (ee - oo).astype(BF)
        for t_ in range(4):
            ob_ref[sl, 128*t_:128*(t_+1)] = yT_ref[128*t_:128*(t_+1), sl].T
    cp_oa = pltpu.make_async_copy(ob_ref.at[:, 0:512], o_hbm.at[:, 0:512], out_sems.at[0])
    cp_oa.start()

    def store_left(h, a0, a1, qsl, n):
        o8 = h % 8
        r8 = jax.lax.broadcasted_iota(jnp.int32, (8, n), 0)
        for base, a in ((512, a0), (544, a1)):
            l8 = pl.multiple_of(base + h // 8 * 8, 8)
            oT_ref[pl.ds(l8, 8), qsl] = jnp.where(r8 == o8, a, oT_ref[pl.ds(l8, 8), qsl])

    def finish_store(h, acc, lacc, qt):
        r0 = pl.multiple_of(16 * h, 16)
        l = jnp.sum(lacc[2], axis=0, keepdims=True) * (2.0 ** TB)
        inv = 1.0 / l
        oT_ref[pl.ds(r0, 16), qt*TQ:(qt+1)*TQ] = acc * inv
        store_left(h, jnp.sum(lacc[0], axis=0, keepdims=True) * inv, jnp.sum(lacc[1], axis=0, keepdims=True) * inv,
                   slice(qt*TQ, (qt+1)*TQ), TQ)

    def fast_heads(t, carry):
        items = [(u, qt, cidx) for u in range(UN) for qt in range(NQ) for cidx in range(NC)]
        vws = {}; ss = {}; accs = {}; laccs = {}
        for u in range(UN):
            r0 = pl.multiple_of(16 * (UN * t + u), 16)
            vws[u] = (vT_ref[pl.ds(r0, 16), :].astype(F32) * (2.0 ** TB)).astype(BF)

        def qk(n):
            u, qt, cidx = items[n]
            h = UN * t + u
            ss[n] = jnp.dot(k_ref[h, cidx*KC:(cidx+1)*KC, 0:32], qT_ref[h, :, qt*TQ:(qt+1)*TQ],
                            preferred_element_type=F32)

        def pv(n):
            u, qt, cidx = items[n]
            vw = vws[u]
            p32 = jnp.exp2(ss.pop(n))
            p = p32.astype(BF)
            d = jnp.dot(vw[:, cidx*KC:(cidx+1)*KC], p, preferred_element_type=F32)
            accs[(u, qt)] = d if cidx == 0 else accs[(u, qt)] + d
            la = laccs.get((u, qt), [None, None, None])
            idx = jnp.full((KC, 128), UN * t + u, jnp.int32)
            vbs = [jnp.take_along_axis(vl_ref[r, cidx*KC:(cidx+1)*KC, :], idx, axis=1) for r in range(2)]
            for gi in range(KC // 8):
                pg = p32[gi*8:(gi+1)*8, :]
                la[2] = pg if la[2] is None else la[2] + pg
                for r in range(2):
                    vb = vbs[r][gi*8:(gi+1)*8, :]
                    term = pg * jnp.concatenate([vb] * (TQ // 128), axis=1)
                    la[r] = term if la[r] is None else la[r] + term
            laccs[(u, qt)] = la
            if cidx == NC - 1:
                finish_store(UN * t + u, accs.pop((u, qt)), laccs.pop((u, qt)), qt)

        for n in range(len(items) + 1):
            if n < len(items):
                qk(n)
            if n >= 1:
                pv(n - 1)
        return carry

    def slow_tile(i, carry):
        h = i // (S // SQ)
        q0 = pl.multiple_of((i % (S // SQ)) * SQ, SQ)
        r0 = pl.multiple_of(16 * h, 16)
        l0 = pl.multiple_of(512 + h // 16 * 16, 16)
        off = h % 16
        ones_row = (off + 1) % 16
        row16 = jax.lax.broadcasted_iota(jnp.int32, (16, S), 0)
        vl = vT_ref[pl.ds(l0, 16), :]
        vl = jnp.where(row16 == ones_row, jnp.ones_like(vl), vl)
        vw = jnp.concatenate([vT_ref[pl.ds(r0, 16), :], vl, vT_ref[pl.ds(l0 + 32, 16), :]], axis=0)
        sT = jnp.dot(k_ref[h, :, 0:32], qT_ref[h, :, pl.ds(q0, SQ)], preferred_element_type=F32)
        mx = jnp.max(sT, axis=0, keepdims=True)
        p = jnp.exp2(sT - mx).astype(BF)
        acc = jnp.dot(vw, p, preferred_element_type=F32)
        r16 = jax.lax.broadcasted_iota(jnp.int32, (16, SQ), 0)
        lo = acc[16:32]
        l = jnp.sum(jnp.where(r16 == ones_row, lo, 0.0), axis=0, keepdims=True)
        inv = 1.0 / l
        oT_ref[pl.ds(r0, 16), pl.ds(q0, SQ)] = acc[0:16] * inv
        store_left(h, jnp.sum(jnp.where(r16 == off, lo, 0.0), axis=0, keepdims=True) * inv,
                   jnp.sum(jnp.where(r16 == off, acc[32:48], 0.0), axis=0, keepdims=True) * inv, pl.ds(q0, SQ), SQ)
        return carry

    qmax = jnp.max(am_ref[0])
    kmax = jnp.max(am_ref[1])
    vmax = jnp.max(am_ref[2])
    safe = jnp.logical_and(qmax * kmax * (DH * 1.02) <= TB, vmax <= 2.0 ** 30)

    @pl.when(safe)
    def _():
        jax.lax.fori_loop(0, H // UN, fast_heads, 0)

    @pl.when(jnp.logical_not(safe))
    def _():
        jax.lax.fori_loop(0, H * (S // SQ), slow_tile, 0)

    woT = woT_ref[...]
    cps = []
    for oc in range(S // OC):
        rs = slice(oc*OC, (oc+1)*OC)
        yT_ref[D:2*D, rs] = jnp.dot(woT, oT_ref[:, rs].astype(BF), preferred_element_type=F32).astype(BF)
        for t_ in range(4, 9):
            ob_ref[rs, 128*t_:128*(t_+1)] = yT_ref[128*t_:128*(t_+1), rs].T
        cp = pltpu.make_async_copy(ob_ref.at[rs, 512:1152], o_hbm.at[rs, 512:1152], out_sems.at[1 + oc])
        cp.start()
        cps.append(cp)
    cp_oa.wait()
    for cp in cps:
        cp.wait()


_F1, _M, _FINV = _consts()


@jax.jit
def pallas_concat_heads__spectral_gfnet__mha_block__prompt_kernel(A_x, A_w_r, A_w_i, B_x, B_wqkv, B_wo):
    anyspec = pl.BlockSpec(memory_space=pl.ANY)
    out = pl.pallas_call(
        _kernel,
        out_shape=jax.ShapeDtypeStruct((S, 2 * D), BF),
        in_specs=[anyspec] * 9,
        out_specs=anyspec,
        scratch_shapes=[
            pltpu.VMEM((D, S), BF), pltpu.VMEM((DF, S), BF), pltpu.VMEM((DF, S), BF), pltpu.VMEM((D, S), BF),
            pltpu.VMEM((D, 3 * D), BF), pltpu.VMEM((D, D), BF), pltpu.VMEM((2 * R, HD), BF),
            pltpu.VMEM((N1, 256, 256), BF), pltpu.VMEM((HD, 2 * R), BF), pltpu.VMEM((S, 2 * D), BF),
            pltpu.VMEM((H, 32, S), BF), pltpu.VMEM((H, S, 128), BF),
            pltpu.VMEM((D, S), BF), pltpu.VMEM((D, S), F32),
            pltpu.VMEM((2 * R, S), F32), pltpu.VMEM((N1, R, 256), BF), pltpu.VMEM((2 * R, S), BF),
            pltpu.VMEM((2, 3, S, 128), F32), pltpu.VMEM((2, N1, R, 128), F32),
            pltpu.VMEM((S, D), BF), pltpu.VMEM((640 + D, D), BF), pltpu.VMEM((3, 8, 128), F32),
            pltpu.VMEM((2, S, 128), F32), pltpu.VMEM((2 * D, S), BF), pltpu.VMEM((D, 640), BF), pltpu.VMEM((D, D), BF),
            pltpu.SemaphoreType.DMA((13,)), pltpu.SemaphoreType.DMA((1 + S // OC,)),
        ],
        compiler_params=pltpu.CompilerParams(vmem_limit_bytes=110 << 20),
    )(A_x[0].T, A_w_r.T, A_w_i.T, B_x[0].T, B_wqkv, B_wo, jnp.asarray(_F1), jnp.asarray(_M), jnp.asarray(_FINV))
    return out[None]
```

```python
import functools

import numpy as np
import jax
import jax.numpy as jnp
from jax.experimental import pallas as pl
from jax.experimental.pallas import tpu as pltpu

S, D, H, DH = 2048, 576, 32, 18
DF = D // 2 + 1
HD = D // 2
RE, RO = 160, 144
R = RE + RO
N1, N2 = 16, 128
LOG2E = 1.4426950408889634
BF = jnp.bfloat16
F32 = jnp.float32

TQ, KC, UN = 1024, 128, 2
RC = 16
PC = 512
XC = 4
OC = 512
L5 = 1024
SQ = 128
TB = 40.0


def _consts():
    r = np.arange(R)
    f = np.where(r < RE, 2 * r, 2 * (r - RE) + 1).astype(np.float64)[:, None]
    valid = (f < DF)
    d = np.arange(HD)[None, :].astype(np.float64)
    ang = 2 * np.pi * ((f * d) % D) / D
    c_, s_ = np.where(valid, np.cos(ang), 0.0), np.where(valid, -np.sin(ang), 0.0)
    f1 = np.concatenate([c_[:RE], s_[:RE], c_[RE:], s_[RE:]], axis=0)
    cf = np.where((f == 0) | (f == DF - 1), 1.0, 2.0) / (S * D)
    ci, si = cf * c_, cf * s_
    finv = np.concatenate([ci[:RE], si[:RE], ci[RE:], si[RE:]], axis=0).T
    n2 = np.arange(N2)[:, None]
    k2 = np.arange(N2)[None, :]
    ms = []
    for k1 in range(N1):
        th = 2 * np.pi * ((n2 * (k1 + N1 * k2)) % S) / S
        c, s = np.cos(th), np.sin(th)
        ms.append(np.block([[c, -s], [s, c]]))
    m = np.stack(ms)
    return (f1.astype(BF), m.astype(BF), np.ascontiguousarray(finv).astype(BF))


def _cmul_const(a, w):
    ar, ai = a
    wr, wi = float(np.real(w)), float(np.imag(w))
    eps = 1e-12
    if abs(wi) < eps and abs(wr - 1) < eps:
        return ar, ai
    if abs(wi) < eps and abs(wr + 1) < eps:
        return -ar, -ai
    if abs(wr) < eps and abs(wi + 1) < eps:
        return ai, -ar
    if abs(wr) < eps and abs(wi - 1) < eps:
        return -ai, ar
    if abs(abs(wr) - abs(wi)) < eps:
        c = abs(wr)
        sr, si = np.sign(wr), np.sign(wi)
        t1 = (ar - ai) if sr * si > 0 else (ar + ai)
        t2 = (ar + ai) if sr * si > 0 else (ar - ai)
        return t1 * (c * sr), t2 * (c * si)
    return ar * wr - ai * wi, ar * wi + ai * wr


def _fft_list(xs, sign):
    n = len(xs)
    if n == 1:
        return xs
    ev = _fft_list(xs[0::2], sign)
    od = _fft_list(xs[1::2], sign)
    out = [None] * n
    for k in range(n // 2):
        t = _cmul_const(od[k], np.exp(sign * 2j * np.pi * k / n))
        out[k] = (ev[k][0] + t[0], ev[k][1] + t[1])
        out[k + n // 2] = (ev[k][0] - t[0], ev[k][1] - t[1])
    return out


def _split_heads_rows(a):
    return jnp.concatenate([a[18*h:18*h+16] for h in range(H)] + [a[18*h+16:18*h+17] for h in range(H)]
                           + [a[18*h+17:18*h+18] for h in range(H)], axis=0)


def _kernel(xa_hbm, wr_hbm, wi_hbm, xb_hbm, w_hbm, wo_hbm, f1_hbm, m_hbm, finv_hbm, o_hbm,
            xa_ref, wr_ref, wi_ref, xb_ref, w_ref, wo_ref, f1_ref, m_ref, finv_ref, ob_ref,
            qT_ref, k_ref, vT_ref, oT_ref, xf_ref, t_ref, g_ref, wn_ref, wp_ref, x_ref, wT_ref, am_ref,
            vl_ref, yT_ref, wk_ref, woT_ref, in_sems, out_sems):
    NQ = S // TQ
    NC = S // KC
    NPC = S // PC
    cp_f1 = pltpu.make_async_copy(f1_hbm, f1_ref, in_sems.at[0])
    cp_xa = [pltpu.make_async_copy(xa_hbm.at[:, c*(S//XC):(c+1)*(S//XC)], xa_ref.at[:, c*(S//XC):(c+1)*(S//XC)],
                                   in_sems.at[1 + c]) for c in range(XC)]
    cp_wr = pltpu.make_async_copy(wr_hbm, wr_ref, in_sems.at[5])
    cp_wi = pltpu.make_async_copy(wi_hbm, wi_ref, in_sems.at[6])
    cp_m = pltpu.make_async_copy(m_hbm, m_ref, in_sems.at[7])
    cp_finv = pltpu.make_async_copy(finv_hbm, finv_ref, in_sems.at[8])
    cp_xb = pltpu.make_async_copy(xb_hbm, xb_ref, in_sems.at[9])
    cp_w = pltpu.make_async_copy(w_hbm.at[:, 0:640], w_ref.at[:, 0:640], in_sems.at[10])
    cp_w2 = pltpu.make_async_copy(w_hbm.at[:, 640:3*D], w_ref.at[:, 640:3*D], in_sems.at[12])
    cp_wo = pltpu.make_async_copy(wo_hbm, wo_ref, in_sems.at[11])
    for cp in [cp_f1, cp_xa[0]]:
        cp.start()

    c = (DH ** -0.5) * LOG2E
    am_ref[...] = jnp.zeros_like(am_ref)
    frow = jax.lax.broadcasted_iota(jnp.int32, (R - 256, 128), 0)

    def wperm_a(a):
        wref = (wr_ref, wi_ref)[a]
        wn_ref[a, 0] = wref[0:128, :].T.astype(F32)
        wn_ref[a, 1] = wref[128:256, :].T.astype(F32)
        wn_ref[a, 2, :, 0:DF-256] = wref[256:DF, :].T.astype(F32)

    def wperm_b(a, k1):
        for j in range(2):
            wp_ref[a, k1, j*128:(j+1)*128, :] = wn_ref[a, j, pl.ds(k1, N2, stride=N1), :].T
        blk = wn_ref[a, 2, pl.ds(k1, N2, stride=N1), :].T[0:R-256, :]
        wp_ref[a, k1, 256:R, :] = jnp.where(frow < DF - 256, blk, 0.0)

    def stage_a_fwd(rc):
        r0 = rc * RC
        xs = [(xf_ref[r0:r0+RC, n1*128:(n1+1)*128], xf_ref[R+r0:R+r0+RC, n1*128:(n1+1)*128]) for n1 in range(N1)]
        ys = _fft_list(xs, -1)
        for k1 in range(N1):
            t_ref[k1, r0:r0+RC, 0:128] = ys[k1][0].astype(BF)
            t_ref[k1, r0:r0+RC, 128:256] = ys[k1][1].astype(BF)

    def stage_a_inv(rc):
        r0 = rc * RC
        xs = [(xf_ref[r0:r0+RC, k1*128:(k1+1)*128], xf_ref[R+r0:R+r0+RC, k1*128:(k1+1)*128]) for k1 in range(N1)]
        ys = _fft_list(xs, +1)
        gr0, gi0 = (r0, RE + r0) if r0 < RE else (RE + r0, RE + RO + r0)
        for n1 in range(N1):
            g_ref[gr0:gr0+RC, n1*128:(n1+1)*128] = ys[n1][0].astype(BF)
            g_ref[gi0:gi0+RC, n1*128:(n1+1)*128] = ys[n1][1].astype(BF)

    def track(idx, val):
        a = jnp.abs(val)
        a = jnp.max(a.reshape(a.shape[0] // 8, 8, a.shape[1]), axis=0)
        a = functools.reduce(jnp.maximum, [a[:, l*128:(l+1)*128] for l in range(a.shape[1] // 128)])
        am_ref[idx] = jnp.maximum(am_ref[idx], a)

    def proj_k(g, pc):
        wk = wk_ref[:, 128*g:128*(g+1)]
        kk = jnp.dot(x_ref[pc*PC:(pc+1)*PC, :], wk, preferred_element_type=F32)
        track(1, kk)
        kb = kk.astype(BF)
        k32 = pltpu.bitcast(kb, jnp.uint32)
        for j in range(min(7, H - 7 * g)):
            kr = kb if j == 0 else pltpu.bitcast(pltpu.roll(k32, 128 - 18 * j, 1), BF)
            k_ref[7*g + j, pc*PC:(pc+1)*PC, :] = kr

    def proj_q(g, pc):
        qT = jnp.dot(wT_ref[128*g:128*(g+1), :], xb_ref[:, pc*PC:(pc+1)*PC], preferred_element_type=F32) * c
        track(0, qT)
        for j in range(min(7, H - 7 * g)):
            qT_ref[7*g + j, :, pc*PC:(pc+1)*PC] = jnp.concatenate(
                [qT[18*j:18*j+18], jnp.zeros((14, PC), F32)], axis=0).astype(BF)

    def proj_v(r, pc):
        rr = slice(640 + r*192, 640 + (r+1)*192)
        vv = jnp.dot(wT_ref[rr, :], xb_ref[:, pc*PC:(pc+1)*PC], preferred_element_type=F32)
        track(2, vv)
        vT_ref[r*192:(r+1)*192, pc*PC:(pc+1)*PC] = vv.astype(BF)

    def interleave(mx, vp):
        n = max(len(mx), 1)
        done = 0
        for i, f in enumerate(mx):
            f()
            upto = (i + 1) * len(vp) // n
            for g_ in vp[done:upto]:
                g_()
            done = upto
        for g_ in vp[done:]:
            g_()

    cp_f1.wait()
    cp_xa[0].wait()
    for cp in cp_xa[1:] + [cp_xb, cp_w, cp_w2, cp_wr, cp_wi, cp_m, cp_finv, cp_wo]:
        cp.start()
    for cc in range(XC):
        if cc > 0:
            cp_xa[cc].wait()
        sl = slice(cc*(S//XC), (cc+1)*(S//XC))
        x0 = xa_ref[0:HD, sl].astype(F32)
        x1 = xa_ref[HD:D, sl].astype(F32)
        xe = jnp.dot(f1_ref[0:2*RE, :], (x0 + x1).astype(BF), preferred_element_type=F32)
        xo = jnp.dot(f1_ref[2*RE:2*R, :], (x0 - x1).astype(BF), preferred_element_type=F32)
        xf_ref[0:RE, sl] = xe[0:RE]
        xf_ref[R:R+RE, sl] = xe[RE:2*RE]
        xf_ref[RE:R, sl] = xo[0:RO]
        xf_ref[R+RE:2*R, sl] = xo[RO:2*RO]
    for rc in range(R // RC):
        stage_a_fwd(rc)
    cp_xb.wait()
    cp_w.wait()

    for g in range(5):
        wT_ref[128*g:128*(g+1), :] = w_ref[:, 126*g:126*g+128].T
    x_ref[...] = xb_ref[...].T
    mq = [functools.partial(proj_q, g, pc) for g in range(5) for pc in range(NPC)]
    for f_ in mq[:2*NPC]:
        f_()
    cp_w2.wait()
    wvT = w_ref[:, 1152:1728].T.astype(F32)
    wT_ref[640:640+512, :] = jnp.concatenate([wvT[18*h:18*h+16] for h in range(H)], axis=0).astype(BF)
    wT_ref[640+512:640+D, :] = jnp.concatenate(
        [wvT[18*h+16:18*h+17] for h in range(H)] + [wvT[18*h+17:18*h+18] for h in range(H)], axis=0).astype(BF)
    for g in range(5):
        wk_ref[:, 128*g:128*(g+1)] = w_ref[:, 576+126*g:576+126*g+128]
    for f_ in mq[2*NPC:]:
        f_()
    cp_wr.wait()
    cp_wi.wait()
    vp = ([functools.partial(wperm_a, 0), functools.partial(wperm_a, 1)]
          + [functools.partial(wperm_b, a, k1) for a in range(2) for k1 in range(N1)])
    interleave([functools.partial(proj_v, r, pc) for r in range(3) for pc in range(NPC)], vp)
    cp_m.wait()

    def mid(k1, carry):
        c0 = pl.multiple_of(k1 * 128, 128)
        mk = m_ref[k1]
        z = jnp.dot(t_ref[k1], mk, preferred_element_type=F32)
        zr, zi = z[:, :128], z[:, 128:]
        wr, wi = [jnp.concatenate([wp_ref[a, k1, pl.ds(0, 152, stride=2), :], jnp.zeros((8, 128), F32),
                                   wp_ref[a, k1, pl.ds(1, RO, stride=2), :]], axis=0) for a in range(2)]
        yr = zr * wr - zi * wi
        yi = zr * wi + zi * wr
        y = jnp.concatenate([yr, yi], axis=1).astype(BF)
        tp = jax.lax.dot_general(y, mk, (((1,), (1,)), ((), ())), preferred_element_type=F32)
        xf_ref[0:R, pl.ds(c0, 128)] = tp[:, :128]
        xf_ref[R:2*R, pl.ds(c0, 128)] = tp[:, 128:]
        return carry
    jax.lax.fori_loop(0, N1, mid, 0, unroll=2)

    mx2 = [functools.partial(proj_k, g, pc) for g in range(5) for pc in range(NPC)]
    interleave(mx2, [functools.partial(stage_a_inv, rc) for rc in range(R // RC)])
    vlt = vT_ref[512:D, :].T.astype(F32) * (2.0 ** TB)
    vlt = jnp.concatenate([vlt, jnp.zeros((S, 64), F32)], axis=1)
    vl_ref[0] = vlt
    vl_ref[1] = pltpu.roll(vlt, 96, 1)
    oT_ref[512:D, :] = jnp.zeros((64, S), F32)
    cp_finv.wait()
    cp_wo.wait()
    woT_ref[...] = _split_heads_rows(wo_ref[...].astype(F32)).astype(BF).T

    for pc in range(S // L5):
        sl = slice(pc * L5, (pc + 1) * L5)
        ee = jnp.dot(finv_ref[:, 0:2*RE], g_ref[0:2*RE, sl], preferred_element_type=F32)
        oo = jnp.dot(finv_ref[:, 2*RE:2*R], g_ref[2*RE:2*R, sl], preferred_element_type=F32)
        yT_ref[0:HD, sl] = (ee + oo).astype(BF)
        yT_ref[HD:D, sl] = (ee - oo).astype(BF)
        for t_ in range(4):
            ob_ref[sl, 128*t_:128*(t_+1)] = yT_ref[128*t_:128*(t_+1), sl].T
    cp_oa = pltpu.make_async_copy(ob_ref.at[:, 0:512], o_hbm.at[:, 0:512], out_sems.at[0])
    cp_oa.start()

    def store_left(h, a0, a1, qsl, n):
        o8 = h % 8
        r8 = jax.lax.broadcasted_iota(jnp.int32, (8, n), 0)
        for base, a in ((512, a0), (544, a1)):
            l8 = pl.multiple_of(base + h // 8 * 8, 8)
            oT_ref[pl.ds(l8, 8), qsl] = jnp.where(r8 == o8, a, oT_ref[pl.ds(l8, 8), qsl])

    def finish_store(h, acc, lacc, qt):
        r0 = pl.multiple_of(16 * h, 16)
        l = jnp.sum(lacc[2], axis=0, keepdims=True) * (2.0 ** TB)
        inv = 1.0 / l
        oT_ref[pl.ds(r0, 16), qt*TQ:(qt+1)*TQ] = acc * inv
        store_left(h, jnp.sum(lacc[0], axis=0, keepdims=True) * inv, jnp.sum(lacc[1], axis=0, keepdims=True) * inv,
                   slice(qt*TQ, (qt+1)*TQ), TQ)

    def fast_heads(t, carry):
        items = [(u, qt, cidx) for u in range(UN) for qt in range(NQ) for cidx in range(NC)]
        vws = {}; ss = {}; accs = {}; laccs = {}
        for u in range(UN):
            r0 = pl.multiple_of(16 * (UN * t + u), 16)
            vws[u] = (vT_ref[pl.ds(r0, 16), :].astype(F32) * (2.0 ** TB)).astype(BF)

        def qk(n):
            u, qt, cidx = items[n]
            h = UN * t + u
            ss[n] = jnp.dot(k_ref[h, cidx*KC:(cidx+1)*KC, 0:32], qT_ref[h, :, qt*TQ:(qt+1)*TQ],
                            preferred_element_type=F32)

        def pv(n):
            u, qt, cidx = items[n]
            vw = vws[u]
            p32 = jnp.exp2(ss.pop(n))
            p = p32.astype(BF)
            d = jnp.dot(vw[:, cidx*KC:(cidx+1)*KC], p, preferred_element_type=F32)
            accs[(u, qt)] = d if cidx == 0 else accs[(u, qt)] + d
            la = laccs.get((u, qt), [None, None, None])
            idx = jnp.full((KC, 128), UN * t + u, jnp.int32)
            vbs = [jnp.take_along_axis(vl_ref[r, cidx*KC:(cidx+1)*KC, :], idx, axis=1) for r in range(2)]
            for gi in range(KC // 8):
                pg = p32[gi*8:(gi+1)*8, :]
                la[2] = pg if la[2] is None else la[2] + pg
                for r in range(2):
                    vb = vbs[r][gi*8:(gi+1)*8, :]
                    term = pg * jnp.concatenate([vb] * (TQ // 128), axis=1)
                    la[r] = term if la[r] is None else la[r] + term
            laccs[(u, qt)] = la
            if cidx == NC - 1:
                finish_store(UN * t + u, accs.pop((u, qt)), laccs.pop((u, qt)), qt)

        for n in range(len(items) + 1):
            if n < len(items):
                qk(n)
            if n >= 1:
                pv(n - 1)
        return carry

    def slow_tile(i, carry):
        h = i // (S // SQ)
        q0 = pl.multiple_of((i % (S // SQ)) * SQ, SQ)
        r0 = pl.multiple_of(16 * h, 16)
        l0 = pl.multiple_of(512 + h // 16 * 16, 16)
        off = h % 16
        ones_row = (off + 1) % 16
        row16 = jax.lax.broadcasted_iota(jnp.int32, (16, S), 0)
        vl = vT_ref[pl.ds(l0, 16), :]
        vl = jnp.where(row16 == ones_row, jnp.ones_like(vl), vl)
        vw = jnp.concatenate([vT_ref[pl.ds(r0, 16), :], vl, vT_ref[pl.ds(l0 + 32, 16), :]], axis=0)
        sT = jnp.dot(k_ref[h, :, 0:32], qT_ref[h, :, pl.ds(q0, SQ)], preferred_element_type=F32)
        mx = jnp.max(sT, axis=0, keepdims=True)
        p = jnp.exp2(sT - mx).astype(BF)
        acc = jnp.dot(vw, p, preferred_element_type=F32)
        r16 = jax.lax.broadcasted_iota(jnp.int32, (16, SQ), 0)
        lo = acc[16:32]
        l = jnp.sum(jnp.where(r16 == ones_row, lo, 0.0), axis=0, keepdims=True)
        inv = 1.0 / l
        oT_ref[pl.ds(r0, 16), pl.ds(q0, SQ)] = acc[0:16] * inv
        store_left(h, jnp.sum(jnp.where(r16 == off, lo, 0.0), axis=0, keepdims=True) * inv,
                   jnp.sum(jnp.where(r16 == off, acc[32:48], 0.0), axis=0, keepdims=True) * inv, pl.ds(q0, SQ), SQ)
        return carry

    qmax = jnp.max(am_ref[0])
    kmax = jnp.max(am_ref[1])
    vmax = jnp.max(am_ref[2])
    safe = jnp.logical_and(qmax * kmax * (DH * 1.02) <= TB, vmax <= 2.0 ** 30)

    @pl.when(safe)
    def _():
        jax.lax.fori_loop(0, H // UN, fast_heads, 0)

    @pl.when(jnp.logical_not(safe))
    def _():
        jax.lax.fori_loop(0, H * (S // SQ), slow_tile, 0)

    woT = woT_ref[...]
    cps = []
    for oc in range(S // OC):
        rs = slice(oc*OC, (oc+1)*OC)
        yT_ref[D:2*D, rs] = jnp.dot(woT, oT_ref[:, rs].astype(BF), preferred_element_type=F32).astype(BF)
        for t_ in range(4, 9):
            ob_ref[rs, 128*t_:128*(t_+1)] = yT_ref[128*t_:128*(t_+1), rs].T
        cp = pltpu.make_async_copy(ob_ref.at[rs, 512:1152], o_hbm.at[rs, 512:1152], out_sems.at[1 + oc])
        cp.start()
        cps.append(cp)
    cp_oa.wait()
    for cp in cps:
        cp.wait()


_F1, _M, _FINV = _consts()


@jax.jit
def pallas_concat_heads__spectral_gfnet__mha_block__prompt_kernel(A_x, A_w_r, A_w_i, B_x, B_wqkv, B_wo):
    anyspec = pl.BlockSpec(memory_space=pl.ANY)
    out = pl.pallas_call(
        _kernel,
        out_shape=jax.ShapeDtypeStruct((S, 2 * D), BF),
        in_specs=[anyspec] * 9,
        out_specs=anyspec,
        scratch_shapes=[
            pltpu.VMEM((D, S), BF), pltpu.VMEM((DF, S), BF), pltpu.VMEM((DF, S), BF), pltpu.VMEM((D, S), BF),
            pltpu.VMEM((D, 3 * D), BF), pltpu.VMEM((D, D), BF), pltpu.VMEM((2 * R, HD), BF),
            pltpu.VMEM((N1, 256, 256), BF), pltpu.VMEM((HD, 2 * R), BF), pltpu.VMEM((S, 2 * D), BF),
            pltpu.VMEM((H, 32, S), BF), pltpu.VMEM((H, S, 128), BF),
            pltpu.VMEM((D, S), BF), pltpu.VMEM((D, S), F32),
            pltpu.VMEM((2 * R, S), F32), pltpu.VMEM((N1, R, 256), BF), pltpu.VMEM((2 * R, S), BF),
            pltpu.VMEM((2, 3, S, 128), F32), pltpu.VMEM((2, N1, R, 128), F32),
            pltpu.VMEM((S, D), BF), pltpu.VMEM((640 + D, D), BF), pltpu.VMEM((3, 8, 128), F32),
            pltpu.VMEM((2, S, 128), F32), pltpu.VMEM((2 * D, S), BF), pltpu.VMEM((D, 640), BF), pltpu.VMEM((D, D), BF),
            pltpu.SemaphoreType.DMA((13,)), pltpu.SemaphoreType.DMA((1 + S // OC,)),
        ],
        compiler_params=pltpu.CompilerParams(vmem_limit_bytes=110 << 20),
    )(A_x[0].T, A_w_r.T, A_w_i.T, B_x[0].T, B_wqkv, B_wo, jnp.asarray(_F1), jnp.asarray(_M), jnp.asarray(_FINV))
    return out[None]
```

```python
import functools

import numpy as np
import jax
import jax.numpy as jnp
from jax.experimental import pallas as pl
from jax.experimental.pallas import tpu as pltpu

S, D, H, DH = 2048, 576, 32, 18
DF = D // 2 + 1
HD = D // 2
RE, RO = 160, 144
R = RE + RO
N1, N2 = 16, 128
LOG2E = 1.4426950408889634
BF = jnp.bfloat16
F32 = jnp.float32

TQ, KC, UN = 1024, 128, 2
RC = 16
PC = 512
XC = 4
OC = 512
SQ = 128
TB = 40.0


def _consts():
    r = np.arange(R)
    f = np.where(r < RE, 2 * r, 2 * (r - RE) + 1).astype(np.float64)[:, None]
    valid = (f < DF)
    d = np.arange(HD)[None, :].astype(np.float64)
    ang = 2 * np.pi * ((f * d) % D) / D
    c_, s_ = np.where(valid, np.cos(ang), 0.0), np.where(valid, -np.sin(ang), 0.0)
    f1 = np.concatenate([c_[:RE], s_[:RE], c_[RE:], s_[RE:]], axis=0)
    cf = np.where((f == 0) | (f == DF - 1), 1.0, 2.0) / (S * D)
    ci, si = cf * c_, cf * s_
    finv = np.concatenate([ci[:RE], si[:RE], ci[RE:], si[RE:]], axis=0).T
    n2 = np.arange(N2)[:, None]
    k2 = np.arange(N2)[None, :]
    ms = []
    for k1 in range(N1):
        th = 2 * np.pi * ((n2 * (k1 + N1 * k2)) % S) / S
        c, s = np.cos(th), np.sin(th)
        ms.append(np.block([[c, -s], [s, c]]))
    m = np.stack(ms)
    return (f1.astype(BF), m.astype(BF), np.ascontiguousarray(finv).astype(BF))


def _cmul_const(a, w):
    ar, ai = a
    wr, wi = float(np.real(w)), float(np.imag(w))
    eps = 1e-12
    if abs(wi) < eps and abs(wr - 1) < eps:
        return ar, ai
    if abs(wi) < eps and abs(wr + 1) < eps:
        return -ar, -ai
    if abs(wr) < eps and abs(wi + 1) < eps:
        return ai, -ar
    if abs(wr) < eps and abs(wi - 1) < eps:
        return -ai, ar
    if abs(abs(wr) - abs(wi)) < eps:
        c = abs(wr)
        sr, si = np.sign(wr), np.sign(wi)
        t1 = (ar - ai) if sr * si > 0 else (ar + ai)
        t2 = (ar + ai) if sr * si > 0 else (ar - ai)
        return t1 * (c * sr), t2 * (c * si)
    return ar * wr - ai * wi, ar * wi + ai * wr


def _fft_list(xs, sign):
    n = len(xs)
    if n == 1:
        return xs
    ev = _fft_list(xs[0::2], sign)
    od = _fft_list(xs[1::2], sign)
    out = [None] * n
    for k in range(n // 2):
        t = _cmul_const(od[k], np.exp(sign * 2j * np.pi * k / n))
        out[k] = (ev[k][0] + t[0], ev[k][1] + t[1])
        out[k + n // 2] = (ev[k][0] - t[0], ev[k][1] - t[1])
    return out


def _split_heads_rows(a):
    return jnp.concatenate([a[18*h:18*h+16] for h in range(H)] + [a[18*h+16:18*h+17] for h in range(H)]
                           + [a[18*h+17:18*h+18] for h in range(H)], axis=0)


def _kernel(xa_hbm, wr_hbm, wi_hbm, xb_hbm, w_hbm, wo_hbm, f1_hbm, m_hbm, finv_hbm, o_hbm,
            xa_ref, wr_ref, wi_ref, xb_ref, w_ref, wo_ref, f1_ref, m_ref, finv_ref, ob_ref,
            qT_ref, k_ref, vT_ref, oT_ref, xf_ref, t_ref, g_ref, wn_ref, wp_ref, x_ref, wT_ref, am_ref,
            vl_ref, yT_ref, wk_ref, woT_ref, in_sems, out_sems):
    NQ = S // TQ
    NC = S // KC
    NPC = S // PC
    cp_f1 = pltpu.make_async_copy(f1_hbm, f1_ref, in_sems.at[0])
    cp_xa = [pltpu.make_async_copy(xa_hbm.at[:, c*(S//XC):(c+1)*(S//XC)], xa_ref.at[:, c*(S//XC):(c+1)*(S//XC)],
                                   in_sems.at[1 + c]) for c in range(XC)]
    cp_wr = pltpu.make_async_copy(wr_hbm, wr_ref, in_sems.at[5])
    cp_wi = pltpu.make_async_copy(wi_hbm, wi_ref, in_sems.at[6])
    cp_m = pltpu.make_async_copy(m_hbm, m_ref, in_sems.at[7])
    cp_finv = pltpu.make_async_copy(finv_hbm, finv_ref, in_sems.at[8])
    cp_xb = pltpu.make_async_copy(xb_hbm, xb_ref, in_sems.at[9])
    cp_w = pltpu.make_async_copy(w_hbm.at[:, 0:640], w_ref.at[:, 0:640], in_sems.at[10])
    cp_w2 = pltpu.make_async_copy(w_hbm.at[:, 640:3*D], w_ref.at[:, 640:3*D], in_sems.at[12])
    cp_wo = pltpu.make_async_copy(wo_hbm, wo_ref, in_sems.at[11])
    for cp in [cp_f1, cp_xa[0]]:
        cp.start()

    c = (DH ** -0.5) * LOG2E
    am_ref[...] = jnp.zeros_like(am_ref)
    frow = jax.lax.broadcasted_iota(jnp.int32, (R - 256, 128), 0)

    def wperm_a(a):
        wref = (wr_ref, wi_ref)[a]
        wn_ref[a, 0] = wref[0:128, :].T.astype(F32)
        wn_ref[a, 1] = wref[128:256, :].T.astype(F32)
        wn_ref[a, 2, :, 0:DF-256] = wref[256:DF, :].T.astype(F32)

    def wperm_b(a, k1):
        for j in range(2):
            wp_ref[a, k1, j*128:(j+1)*128, :] = wn_ref[a, j, pl.ds(k1, N2, stride=N1), :].T
        blk = wn_ref[a, 2, pl.ds(k1, N2, stride=N1), :].T[0:R-256, :]
        wp_ref[a, k1, 256:R, :] = jnp.where(frow < DF - 256, blk, 0.0)

    def stage_a_fwd(rc):
        r0 = rc * RC
        xs = [(xf_ref[r0:r0+RC, n1*128:(n1+1)*128], xf_ref[R+r0:R+r0+RC, n1*128:(n1+1)*128]) for n1 in range(N1)]
        ys = _fft_list(xs, -1)
        for k1 in range(N1):
            t_ref[k1, r0:r0+RC, 0:128] = ys[k1][0].astype(BF)
            t_ref[k1, r0:r0+RC, 128:256] = ys[k1][1].astype(BF)

    def stage_a_inv(rc):
        r0 = rc * RC
        xs = [(xf_ref[r0:r0+RC, k1*128:(k1+1)*128], xf_ref[R+r0:R+r0+RC, k1*128:(k1+1)*128]) for k1 in range(N1)]
        ys = _fft_list(xs, +1)
        gr0, gi0 = (r0, RE + r0) if r0 < RE else (RE + r0, RE + RO + r0)
        for n1 in range(N1):
            g_ref[gr0:gr0+RC, n1*128:(n1+1)*128] = ys[n1][0].astype(BF)
            g_ref[gi0:gi0+RC, n1*128:(n1+1)*128] = ys[n1][1].astype(BF)

    def track(idx, val):
        a = jnp.abs(val)
        a = jnp.max(a.reshape(a.shape[0] // 8, 8, a.shape[1]), axis=0)
        a = functools.reduce(jnp.maximum, [a[:, l*128:(l+1)*128] for l in range(a.shape[1] // 128)])
        am_ref[idx] = jnp.maximum(am_ref[idx], a)

    def proj_k(g, pc):
        wk = wk_ref[:, 128*g:128*(g+1)]
        kk = jnp.dot(x_ref[pc*PC:(pc+1)*PC, :], wk, preferred_element_type=F32)
        track(1, kk)
        kb = kk.astype(BF)
        k32 = pltpu.bitcast(kb, jnp.uint32)
        for j in range(min(7, H - 7 * g)):
            kr = kb if j == 0 else pltpu.bitcast(pltpu.roll(k32, 128 - 18 * j, 1), BF)
            k_ref[7*g + j, pc*PC:(pc+1)*PC, :] = kr

    def proj_q(g, pc):
        qT = jnp.dot(wT_ref[128*g:128*(g+1), :], xb_ref[:, pc*PC:(pc+1)*PC], preferred_element_type=F32) * c
        track(0, qT)
        for j in range(min(7, H - 7 * g)):
            qT_ref[7*g + j, :, pc*PC:(pc+1)*PC] = jnp.concatenate(
                [qT[18*j:18*j+18], jnp.zeros((14, PC), F32)], axis=0).astype(BF)

    def proj_v(r, pc):
        rr = slice(640 + r*192, 640 + (r+1)*192)
        vv = jnp.dot(wT_ref[rr, :], xb_ref[:, pc*PC:(pc+1)*PC], preferred_element_type=F32)
        track(2, vv)
        vT_ref[r*192:(r+1)*192, pc*PC:(pc+1)*PC] = vv.astype(BF)

    def interleave(mx, vp):
        n = max(len(mx), 1)
        done = 0
        for i, f in enumerate(mx):
            f()
            upto = (i + 1) * len(vp) // n
            for g_ in vp[done:upto]:
                g_()
            done = upto
        for g_ in vp[done:]:
            g_()

    cp_f1.wait()
    cp_xa[0].wait()
    for cp in cp_xa[1:] + [cp_xb, cp_w, cp_w2, cp_wr, cp_wi, cp_m, cp_finv, cp_wo]:
        cp.start()
    for cc in range(XC):
        if cc > 0:
            cp_xa[cc].wait()
        sl = slice(cc*(S//XC), (cc+1)*(S//XC))
        x0 = xa_ref[0:HD, sl].astype(F32)
        x1 = xa_ref[HD:D, sl].astype(F32)
        xe = jnp.dot(f1_ref[0:2*RE, :], (x0 + x1).astype(BF), preferred_element_type=F32)
        xo = jnp.dot(f1_ref[2*RE:2*R, :], (x0 - x1).astype(BF), preferred_element_type=F32)
        xf_ref[0:RE, sl] = xe[0:RE]
        xf_ref[R:R+RE, sl] = xe[RE:2*RE]
        xf_ref[RE:R, sl] = xo[0:RO]
        xf_ref[R+RE:2*R, sl] = xo[RO:2*RO]
    for rc in range(R // RC):
        stage_a_fwd(rc)
    cp_xb.wait()
    cp_w.wait()

    for g in range(5):
        wT_ref[128*g:128*(g+1), :] = w_ref[:, 126*g:126*g+128].T
    x_ref[...] = xb_ref[...].T
    mq = [functools.partial(proj_q, g, pc) for g in range(5) for pc in range(NPC)]
    for f_ in mq[:2*NPC]:
        f_()
    cp_w2.wait()
    wvT = w_ref[:, 1152:1728].T.astype(F32)
    wT_ref[640:640+512, :] = jnp.concatenate([wvT[18*h:18*h+16] for h in range(H)], axis=0).astype(BF)
    wT_ref[640+512:640+D, :] = jnp.concatenate(
        [wvT[18*h+16:18*h+17] for h in range(H)] + [wvT[18*h+17:18*h+18] for h in range(H)], axis=0).astype(BF)
    for g in range(5):
        wk_ref[:, 128*g:128*(g+1)] = w_ref[:, 576+126*g:576+126*g+128]
    for f_ in mq[2*NPC:]:
        f_()
    cp_wr.wait()
    cp_wi.wait()
    vp = ([functools.partial(wperm_a, 0), functools.partial(wperm_a, 1)]
          + [functools.partial(wperm_b, a, k1) for a in range(2) for k1 in range(N1)])
    interleave([functools.partial(proj_v, r, pc) for r in range(3) for pc in range(NPC)], vp)
    cp_m.wait()

    def mid(k1, carry):
        c0 = pl.multiple_of(k1 * 128, 128)
        mk = m_ref[k1]
        z = jnp.dot(t_ref[k1], mk, preferred_element_type=F32)
        zr, zi = z[:, :128], z[:, 128:]
        wr, wi = [jnp.concatenate([wp_ref[a, k1, pl.ds(0, 152, stride=2), :], jnp.zeros((8, 128), F32),
                                   wp_ref[a, k1, pl.ds(1, RO, stride=2), :]], axis=0) for a in range(2)]
        yr = zr * wr - zi * wi
        yi = zr * wi + zi * wr
        y = jnp.concatenate([yr, yi], axis=1).astype(BF)
        tp = jax.lax.dot_general(y, mk, (((1,), (1,)), ((), ())), preferred_element_type=F32)
        xf_ref[0:R, pl.ds(c0, 128)] = tp[:, :128]
        xf_ref[R:2*R, pl.ds(c0, 128)] = tp[:, 128:]
        return carry
    jax.lax.fori_loop(0, N1, mid, 0, unroll=2)

    mx2 = [functools.partial(proj_k, g, pc) for g in range(5) for pc in range(NPC)]
    interleave(mx2, [functools.partial(stage_a_inv, rc) for rc in range(R // RC)])
    vlt = vT_ref[512:D, :].T.astype(F32) * (2.0 ** TB)
    vlt = jnp.concatenate([vlt, jnp.zeros((S, 64), F32)], axis=1)
    vl_ref[0] = vlt
    vl_ref[1] = pltpu.roll(vlt, 96, 1)
    oT_ref[512:D, :] = jnp.zeros((64, S), F32)
    cp_finv.wait()
    cp_wo.wait()
    woT_ref[...] = _split_heads_rows(wo_ref[...].astype(F32)).astype(BF).T

    def step5_slab(t):
        sl = pl.ds(pl.multiple_of(t * 128, 128), 128)
        ee = jnp.dot(finv_ref[:, 0:2*RE], g_ref[0:2*RE, sl], preferred_element_type=F32)
        oo = jnp.dot(finv_ref[:, 2*RE:2*R], g_ref[2*RE:2*R, sl], preferred_element_type=F32)
        yT_ref[0:HD, sl] = (ee + oo).astype(BF)
        yT_ref[HD:D, sl] = (ee - oo).astype(BF)

    def store_left(h, a0, a1, qsl, n):
        o8 = h % 8
        r8 = jax.lax.broadcasted_iota(jnp.int32, (8, n), 0)
        for base, a in ((512, a0), (544, a1)):
            l8 = pl.multiple_of(base + h // 8 * 8, 8)
            oT_ref[pl.ds(l8, 8), qsl] = jnp.where(r8 == o8, a, oT_ref[pl.ds(l8, 8), qsl])

    def finish_store(h, acc, lacc, qt):
        r0 = pl.multiple_of(16 * h, 16)
        l = jnp.sum(lacc[2], axis=0, keepdims=True) * (2.0 ** TB)
        inv = 1.0 / l
        oT_ref[pl.ds(r0, 16), qt*TQ:(qt+1)*TQ] = acc * inv
        store_left(h, jnp.sum(lacc[0], axis=0, keepdims=True) * inv, jnp.sum(lacc[1], axis=0, keepdims=True) * inv,
                   slice(qt*TQ, (qt+1)*TQ), TQ)

    def fast_heads(t, carry):
        items = [(u, qt, cidx) for u in range(UN) for qt in range(NQ) for cidx in range(NC)]
        vws = {}; ss = {}; accs = {}; laccs = {}
        for u in range(UN):
            r0 = pl.multiple_of(16 * (UN * t + u), 16)
            vws[u] = (vT_ref[pl.ds(r0, 16), :].astype(F32) * (2.0 ** TB)).astype(BF)

        def qk(n):
            u, qt, cidx = items[n]
            h = UN * t + u
            ss[n] = jnp.dot(k_ref[h, cidx*KC:(cidx+1)*KC, 0:32], qT_ref[h, :, qt*TQ:(qt+1)*TQ],
                            preferred_element_type=F32)

        def pv(n):
            u, qt, cidx = items[n]
            vw = vws[u]
            p32 = jnp.exp2(ss.pop(n))
            p = p32.astype(BF)
            d = jnp.dot(vw[:, cidx*KC:(cidx+1)*KC], p, preferred_element_type=F32)
            accs[(u, qt)] = d if cidx == 0 else accs[(u, qt)] + d
            la = laccs.get((u, qt), [None, None, None])
            idx = jnp.full((KC, 128), UN * t + u, jnp.int32)
            vbs = [jnp.take_along_axis(vl_ref[r, cidx*KC:(cidx+1)*KC, :], idx, axis=1) for r in range(2)]
            for gi in range(KC // 8):
                pg = p32[gi*8:(gi+1)*8, :]
                la[2] = pg if la[2] is None else la[2] + pg
                for r in range(2):
                    vb = vbs[r][gi*8:(gi+1)*8, :]
                    term = pg * jnp.concatenate([vb] * (TQ // 128), axis=1)
                    la[r] = term if la[r] is None else la[r] + term
            laccs[(u, qt)] = la
            if cidx == NC - 1:
                finish_store(UN * t + u, accs.pop((u, qt)), laccs.pop((u, qt)), qt)

        for n in range(len(items) + 1):
            if n < len(items):
                qk(n)
            else:
                step5_slab(t)
            if n >= 1:
                pv(n - 1)
        return carry

    def slow_tile(i, carry):
        h = i // (S // SQ)
        q0 = pl.multiple_of((i % (S // SQ)) * SQ, SQ)
        r0 = pl.multiple_of(16 * h, 16)
        l0 = pl.multiple_of(512 + h // 16 * 16, 16)
        off = h % 16
        ones_row = (off + 1) % 16
        row16 = jax.lax.broadcasted_iota(jnp.int32, (16, S), 0)
        vl = vT_ref[pl.ds(l0, 16), :]
        vl = jnp.where(row16 == ones_row, jnp.ones_like(vl), vl)
        vw = jnp.concatenate([vT_ref[pl.ds(r0, 16), :], vl, vT_ref[pl.ds(l0 + 32, 16), :]], axis=0)
        sT = jnp.dot(k_ref[h, :, 0:32], qT_ref[h, :, pl.ds(q0, SQ)], preferred_element_type=F32)
        mx = jnp.max(sT, axis=0, keepdims=True)
        p = jnp.exp2(sT - mx).astype(BF)
        acc = jnp.dot(vw, p, preferred_element_type=F32)
        r16 = jax.lax.broadcasted_iota(jnp.int32, (16, SQ), 0)
        lo = acc[16:32]
        l = jnp.sum(jnp.where(r16 == ones_row, lo, 0.0), axis=0, keepdims=True)
        inv = 1.0 / l
        oT_ref[pl.ds(r0, 16), pl.ds(q0, SQ)] = acc[0:16] * inv
        store_left(h, jnp.sum(jnp.where(r16 == off, lo, 0.0), axis=0, keepdims=True) * inv,
                   jnp.sum(jnp.where(r16 == off, acc[32:48], 0.0), axis=0, keepdims=True) * inv, pl.ds(q0, SQ), SQ)
        return carry

    qmax = jnp.max(am_ref[0])
    kmax = jnp.max(am_ref[1])
    vmax = jnp.max(am_ref[2])
    safe = jnp.logical_and(qmax * kmax * (DH * 1.02) <= TB, vmax <= 2.0 ** 30)

    @pl.when(safe)
    def _():
        jax.lax.fori_loop(0, H // UN, fast_heads, 0)

    @pl.when(jnp.logical_not(safe))
    def _():
        def s5(t, carry):
            step5_slab(t)
            return carry
        jax.lax.fori_loop(0, N1, s5, 0)
        jax.lax.fori_loop(0, H * (S // SQ), slow_tile, 0)

    woT = woT_ref[...]
    cps = []
    for oc in range(S // OC):
        rs = slice(oc*OC, (oc+1)*OC)
        yT_ref[D:2*D, rs] = jnp.dot(woT, oT_ref[:, rs].astype(BF), preferred_element_type=F32).astype(BF)
        if oc == 0:
            for t_ in range(4):
                ob_ref[:, 128*t_:128*(t_+1)] = yT_ref[128*t_:128*(t_+1), :].T
            cp_oa = pltpu.make_async_copy(ob_ref.at[:, 0:512], o_hbm.at[:, 0:512], out_sems.at[0])
            cp_oa.start()
            cps.append(cp_oa)
        for t_ in range(4, 9):
            ob_ref[rs, 128*t_:128*(t_+1)] = yT_ref[128*t_:128*(t_+1), rs].T
        cp = pltpu.make_async_copy(ob_ref.at[rs, 512:1152], o_hbm.at[rs, 512:1152], out_sems.at[1 + oc])
        cp.start()
        cps.append(cp)
    for cp in cps:
        cp.wait()


_F1, _M, _FINV = _consts()


@jax.jit
def pallas_concat_heads__spectral_gfnet__mha_block__prompt_kernel(A_x, A_w_r, A_w_i, B_x, B_wqkv, B_wo):
    anyspec = pl.BlockSpec(memory_space=pl.ANY)
    out = pl.pallas_call(
        _kernel,
        out_shape=jax.ShapeDtypeStruct((S, 2 * D), BF),
        in_specs=[anyspec] * 9,
        out_specs=anyspec,
        scratch_shapes=[
            pltpu.VMEM((D, S), BF), pltpu.VMEM((DF, S), BF), pltpu.VMEM((DF, S), BF), pltpu.VMEM((D, S), BF),
            pltpu.VMEM((D, 3 * D), BF), pltpu.VMEM((D, D), BF), pltpu.VMEM((2 * R, HD), BF),
            pltpu.VMEM((N1, 256, 256), BF), pltpu.VMEM((HD, 2 * R), BF), pltpu.VMEM((S, 2 * D), BF),
            pltpu.VMEM((H, 32, S), BF), pltpu.VMEM((H, S, 128), BF),
            pltpu.VMEM((D, S), BF), pltpu.VMEM((D, S), F32),
            pltpu.VMEM((2 * R, S), F32), pltpu.VMEM((N1, R, 256), BF), pltpu.VMEM((2 * R, S), BF),
            pltpu.VMEM((2, 3, S, 128), F32), pltpu.VMEM((2, N1, R, 128), F32),
            pltpu.VMEM((S, D), BF), pltpu.VMEM((640 + D, D), BF), pltpu.VMEM((3, 8, 128), F32),
            pltpu.VMEM((2, S, 128), F32), pltpu.VMEM((2 * D, S), BF), pltpu.VMEM((D, 640), BF), pltpu.VMEM((D, D), BF),
            pltpu.SemaphoreType.DMA((13,)), pltpu.SemaphoreType.DMA((1 + S // OC,)),
        ],
        compiler_params=pltpu.CompilerParams(vmem_limit_bytes=110 << 20),
    )(A_x[0].T, A_w_r.T, A_w_i.T, B_x[0].T, B_wqkv, B_wo, jnp.asarray(_F1), jnp.asarray(_M), jnp.asarray(_FINV))
    return out[None]
```

```python
import functools

import numpy as np
import jax
import jax.numpy as jnp
from jax.experimental import pallas as pl
from jax.experimental.pallas import tpu as pltpu

S, D, H, DH = 2048, 576, 32, 18
DF = D // 2 + 1
HD = D // 2
RE, RO = 160, 144
R = RE + RO
N1, N2 = 16, 128
LOG2E = 1.4426950408889634
BF = jnp.bfloat16
F32 = jnp.float32

TQ, KC, UN = 1024, 128, 2
RC = 16
PC = 512
XC = 4
OC = 512
SQ = 128
TB = 40.0


def _consts():
    r = np.arange(R)
    f = np.where(r < RE, 2 * r, 2 * (r - RE) + 1).astype(np.float64)[:, None]
    valid = (f < DF)
    d = np.arange(HD)[None, :].astype(np.float64)
    ang = 2 * np.pi * ((f * d) % D) / D
    c_, s_ = np.where(valid, np.cos(ang), 0.0), np.where(valid, -np.sin(ang), 0.0)
    f1 = np.concatenate([c_[:RE], s_[:RE], c_[RE:], s_[RE:]], axis=0)
    cf = np.where((f == 0) | (f == DF - 1), 1.0, 2.0) / (S * D)
    ci, si = cf * c_, cf * s_
    finv = np.concatenate([ci[:RE], si[:RE], ci[RE:], si[RE:]], axis=0).T
    n2 = np.arange(N2)[:, None]
    k2 = np.arange(N2)[None, :]
    ms = []
    for k1 in range(N1):
        th = 2 * np.pi * ((n2 * (k1 + N1 * k2)) % S) / S
        c, s = np.cos(th), np.sin(th)
        ms.append(np.block([[c, -s], [s, c]]))
    m = np.stack(ms)
    return (f1.astype(BF), m.astype(BF), np.ascontiguousarray(finv).astype(BF))


def _cmul_const(a, w):
    ar, ai = a
    wr, wi = float(np.real(w)), float(np.imag(w))
    eps = 1e-12
    if abs(wi) < eps and abs(wr - 1) < eps:
        return ar, ai
    if abs(wi) < eps and abs(wr + 1) < eps:
        return -ar, -ai
    if abs(wr) < eps and abs(wi + 1) < eps:
        return ai, -ar
    if abs(wr) < eps and abs(wi - 1) < eps:
        return -ai, ar
    if abs(abs(wr) - abs(wi)) < eps:
        c = abs(wr)
        sr, si = np.sign(wr), np.sign(wi)
        t1 = (ar - ai) if sr * si > 0 else (ar + ai)
        t2 = (ar + ai) if sr * si > 0 else (ar - ai)
        return t1 * (c * sr), t2 * (c * si)
    return ar * wr - ai * wi, ar * wi + ai * wr


def _fft_list(xs, sign):
    n = len(xs)
    if n == 1:
        return xs
    ev = _fft_list(xs[0::2], sign)
    od = _fft_list(xs[1::2], sign)
    out = [None] * n
    for k in range(n // 2):
        t = _cmul_const(od[k], np.exp(sign * 2j * np.pi * k / n))
        out[k] = (ev[k][0] + t[0], ev[k][1] + t[1])
        out[k + n // 2] = (ev[k][0] - t[0], ev[k][1] - t[1])
    return out


def _split_heads_rows(a):
    return jnp.concatenate([a[18*h:18*h+16] for h in range(H)] + [a[18*h+16:18*h+17] for h in range(H)]
                           + [a[18*h+17:18*h+18] for h in range(H)], axis=0)


def _kernel(xa_hbm, wr_hbm, wi_hbm, xb_hbm, w_hbm, wo_hbm, f1_hbm, m_hbm, finv_hbm, o_hbm,
            xa_ref, wr_ref, wi_ref, xb_ref, w_ref, wo_ref, f1_ref, m_ref, finv_ref, ob_ref,
            qT_ref, k_ref, vT_ref, oT_ref, xf_ref, t_ref, g_ref, wn_ref, wp_ref, x_ref, wT_ref, am_ref,
            vl_ref, yT_ref, wk_ref, woT_ref, in_sems, out_sems):
    NQ = S // TQ
    NC = S // KC
    NPC = S // PC
    cp_f1 = pltpu.make_async_copy(f1_hbm, f1_ref, in_sems.at[0])
    cp_xa = [pltpu.make_async_copy(xa_hbm.at[:, c*(S//XC):(c+1)*(S//XC)], xa_ref.at[:, c*(S//XC):(c+1)*(S//XC)],
                                   in_sems.at[1 + c]) for c in range(XC)]
    cp_wr = pltpu.make_async_copy(wr_hbm, wr_ref, in_sems.at[5])
    cp_wi = pltpu.make_async_copy(wi_hbm, wi_ref, in_sems.at[6])
    cp_m = pltpu.make_async_copy(m_hbm, m_ref, in_sems.at[7])
    cp_finv = pltpu.make_async_copy(finv_hbm, finv_ref, in_sems.at[8])
    cp_xb = pltpu.make_async_copy(xb_hbm, xb_ref, in_sems.at[9])
    cp_w = pltpu.make_async_copy(w_hbm.at[:, 0:640], w_ref.at[:, 0:640], in_sems.at[10])
    cp_w2 = pltpu.make_async_copy(w_hbm.at[:, 640:3*D], w_ref.at[:, 640:3*D], in_sems.at[12])
    cp_wo = pltpu.make_async_copy(wo_hbm, wo_ref, in_sems.at[11])
    for cp in [cp_f1, cp_xa[0]]:
        cp.start()

    c = (DH ** -0.5) * LOG2E
    am_ref[...] = jnp.zeros_like(am_ref)
    frow = jax.lax.broadcasted_iota(jnp.int32, (R - 256, 128), 0)

    def wperm_a(a):
        wref = (wr_ref, wi_ref)[a]
        wn_ref[a, 0] = wref[0:128, :].T.astype(F32)
        wn_ref[a, 1] = wref[128:256, :].T.astype(F32)
        wn_ref[a, 2, :, 0:DF-256] = wref[256:DF, :].T.astype(F32)

    def wperm_b(a, k1):
        for j in range(2):
            wp_ref[a, k1, j*128:(j+1)*128, :] = wn_ref[a, j, pl.ds(k1, N2, stride=N1), :].T
        blk = wn_ref[a, 2, pl.ds(k1, N2, stride=N1), :].T[0:R-256, :]
        wp_ref[a, k1, 256:R, :] = jnp.where(frow < DF - 256, blk, 0.0)

    def stage_a_fwd(rc):
        r0 = rc * RC
        xs = [(xf_ref[r0:r0+RC, n1*128:(n1+1)*128], xf_ref[R+r0:R+r0+RC, n1*128:(n1+1)*128]) for n1 in range(N1)]
        ys = _fft_list(xs, -1)
        for k1 in range(N1):
            t_ref[k1, r0:r0+RC, 0:128] = ys[k1][0].astype(BF)
            t_ref[k1, r0:r0+RC, 128:256] = ys[k1][1].astype(BF)

    def stage_a_inv(rc):
        r0 = rc * RC
        xs = [(xf_ref[r0:r0+RC, k1*128:(k1+1)*128], xf_ref[R+r0:R+r0+RC, k1*128:(k1+1)*128]) for k1 in range(N1)]
        ys = _fft_list(xs, +1)
        gr0, gi0 = (r0, RE + r0) if r0 < RE else (RE + r0, RE + RO + r0)
        for n1 in range(N1):
            g_ref[gr0:gr0+RC, n1*128:(n1+1)*128] = ys[n1][0].astype(BF)
            g_ref[gi0:gi0+RC, n1*128:(n1+1)*128] = ys[n1][1].astype(BF)

    def track(idx, val):
        a = jnp.abs(val)
        a = jnp.max(a.reshape(a.shape[0] // 8, 8, a.shape[1]), axis=0)
        a = functools.reduce(jnp.maximum, [a[:, l*128:(l+1)*128] for l in range(a.shape[1] // 128)])
        am_ref[idx] = jnp.maximum(am_ref[idx], a)

    def proj_k(g, pc):
        wk = wk_ref[:, 128*g:128*(g+1)]
        kk = jnp.dot(x_ref[pc*PC:(pc+1)*PC, :], wk, preferred_element_type=F32)
        track(1, kk)
        kb = kk.astype(BF)
        k32 = pltpu.bitcast(kb, jnp.uint32)
        for j in range(min(7, H - 7 * g)):
            kr = kb if j == 0 else pltpu.bitcast(pltpu.roll(k32, 128 - 18 * j, 1), BF)
            k_ref[7*g + j, pc*PC:(pc+1)*PC, :] = kr

    def proj_q(g, pc):
        qT = jnp.dot(wT_ref[144*g:144*(g+1), :], xb_ref[:, pc*PC:(pc+1)*PC], preferred_element_type=F32) * c
        track(0, qT)
        for j in range(8):
            qT_ref[8*g + j, :, pc*PC:(pc+1)*PC] = jnp.concatenate(
                [qT[18*j:18*j+18], jnp.zeros((14, PC), F32)], axis=0).astype(BF)

    def proj_v(r, pc):
        rr = slice(640 + r*192, 640 + (r+1)*192)
        vv = jnp.dot(wT_ref[rr, :], xb_ref[:, pc*PC:(pc+1)*PC], preferred_element_type=F32)
        track(2, vv)
        vT_ref[r*192:(r+1)*192, pc*PC:(pc+1)*PC] = vv.astype(BF)

    def interleave(mx, vp):
        n = max(len(mx), 1)
        done = 0
        for i, f in enumerate(mx):
            f()
            upto = (i + 1) * len(vp) // n
            for g_ in vp[done:upto]:
                g_()
            done = upto
        for g_ in vp[done:]:
            g_()

    cp_f1.wait()
    cp_xa[0].wait()
    for cp in cp_xa[1:] + [cp_xb, cp_w, cp_w2, cp_wr, cp_wi, cp_m, cp_finv, cp_wo]:
        cp.start()
    for cc in range(XC):
        if cc > 0:
            cp_xa[cc].wait()
        sl = slice(cc*(S//XC), (cc+1)*(S//XC))
        x0 = xa_ref[0:HD, sl].astype(F32)
        x1 = xa_ref[HD:D, sl].astype(F32)
        xe = jnp.dot(f1_ref[0:2*RE, :], (x0 + x1).astype(BF), preferred_element_type=F32)
        xo = jnp.dot(f1_ref[2*RE:2*R, :], (x0 - x1).astype(BF), preferred_element_type=F32)
        xf_ref[0:RE, sl] = xe[0:RE]
        xf_ref[R:R+RE, sl] = xe[RE:2*RE]
        xf_ref[RE:R, sl] = xo[0:RO]
        xf_ref[R+RE:2*R, sl] = xo[RO:2*RO]
    for rc in range(R // RC):
        stage_a_fwd(rc)
    cp_xb.wait()
    cp_w.wait()

    wT_ref[0:640, :] = w_ref[:, 0:640].T
    x_ref[...] = xb_ref[...].T
    mq = [functools.partial(proj_q, g, pc) for g in range(4) for pc in range(NPC)]
    for f_ in mq[:2*NPC]:
        f_()
    cp_w2.wait()
    wvT = w_ref[:, 1152:1728].T.astype(F32)
    wT_ref[640:640+512, :] = jnp.concatenate([wvT[18*h:18*h+16] for h in range(H)], axis=0).astype(BF)
    wT_ref[640+512:640+D, :] = jnp.concatenate(
        [wvT[18*h+16:18*h+17] for h in range(H)] + [wvT[18*h+17:18*h+18] for h in range(H)], axis=0).astype(BF)
    for g in range(5):
        wk_ref[:, 128*g:128*(g+1)] = w_ref[:, 576+126*g:576+126*g+128]
    for f_ in mq[2*NPC:]:
        f_()
    cp_wr.wait()
    cp_wi.wait()
    vp = ([functools.partial(wperm_a, 0), functools.partial(wperm_a, 1)]
          + [functools.partial(wperm_b, a, k1) for a in range(2) for k1 in range(N1)])
    interleave([functools.partial(proj_v, r, pc) for r in range(3) for pc in range(NPC)], vp)
    cp_m.wait()

    def mid(k1, carry):
        c0 = pl.multiple_of(k1 * 128, 128)
        mk = m_ref[k1]
        z = jnp.dot(t_ref[k1], mk, preferred_element_type=F32)
        zr, zi = z[:, :128], z[:, 128:]
        wr, wi = [jnp.concatenate([wp_ref[a, k1, pl.ds(0, 152, stride=2), :], jnp.zeros((8, 128), F32),
                                   wp_ref[a, k1, pl.ds(1, RO, stride=2), :]], axis=0) for a in range(2)]
        yr = zr * wr - zi * wi
        yi = zr * wi + zi * wr
        y = jnp.concatenate([yr, yi], axis=1).astype(BF)
        tp = jax.lax.dot_general(y, mk, (((1,), (1,)), ((), ())), preferred_element_type=F32)
        xf_ref[0:R, pl.ds(c0, 128)] = tp[:, :128]
        xf_ref[R:2*R, pl.ds(c0, 128)] = tp[:, 128:]
        return carry
    jax.lax.fori_loop(0, N1, mid, 0, unroll=2)

    mx2 = [functools.partial(proj_k, g, pc) for g in range(5) for pc in range(NPC)]
    interleave(mx2, [functools.partial(stage_a_inv, rc) for rc in range(R // RC)])
    vlt = vT_ref[512:D, :].T.astype(F32) * (2.0 ** TB)
    vlt = jnp.concatenate([vlt, jnp.zeros((S, 64), F32)], axis=1)
    vl_ref[0] = vlt
    vl_ref[1] = pltpu.roll(vlt, 96, 1)
    oT_ref[512:D, :] = jnp.zeros((64, S), F32)
    cp_finv.wait()
    cp_wo.wait()
    woT_ref[...] = _split_heads_rows(wo_ref[...].astype(F32)).astype(BF).T

    def step5_slab(t):
        sl = pl.ds(pl.multiple_of(t * 128, 128), 128)
        ee = jnp.dot(finv_ref[:, 0:2*RE], g_ref[0:2*RE, sl], preferred_element_type=F32)
        oo = jnp.dot(finv_ref[:, 2*RE:2*R], g_ref[2*RE:2*R, sl], preferred_element_type=F32)
        yT_ref[0:HD, sl] = (ee + oo).astype(BF)
        yT_ref[HD:D, sl] = (ee - oo).astype(BF)

    def store_left(h, a0, a1, qsl, n):
        o8 = h % 8
        r8 = jax.lax.broadcasted_iota(jnp.int32, (8, n), 0)
        for base, a in ((512, a0), (544, a1)):
            l8 = pl.multiple_of(base + h // 8 * 8, 8)
            oT_ref[pl.ds(l8, 8), qsl] = jnp.where(r8 == o8, a, oT_ref[pl.ds(l8, 8), qsl])

    def finish_store(h, acc, lacc, qt):
        r0 = pl.multiple_of(16 * h, 16)
        l = jnp.sum(lacc[2], axis=0, keepdims=True) * (2.0 ** TB)
        inv = 1.0 / l
        oT_ref[pl.ds(r0, 16), qt*TQ:(qt+1)*TQ] = acc * inv
        store_left(h, jnp.sum(lacc[0], axis=0, keepdims=True) * inv, jnp.sum(lacc[1], axis=0, keepdims=True) * inv,
                   slice(qt*TQ, (qt+1)*TQ), TQ)

    def fast_heads(t, carry):
        items = [(u, qt, cidx) for u in range(UN) for qt in range(NQ) for cidx in range(NC)]
        vws = {}; ss = {}; accs = {}; laccs = {}
        for u in range(UN):
            r0 = pl.multiple_of(16 * (UN * t + u), 16)
            vws[u] = (vT_ref[pl.ds(r0, 16), :].astype(F32) * (2.0 ** TB)).astype(BF)

        def qk(n):
            u, qt, cidx = items[n]
            h = UN * t + u
            ss[n] = jnp.dot(k_ref[h, cidx*KC:(cidx+1)*KC, 0:32], qT_ref[h, :, qt*TQ:(qt+1)*TQ],
                            preferred_element_type=F32)

        def pv(n):
            u, qt, cidx = items[n]
            vw = vws[u]
            p32 = jnp.exp2(ss.pop(n))
            p = p32.astype(BF)
            d = jnp.dot(vw[:, cidx*KC:(cidx+1)*KC], p, preferred_element_type=F32)
            accs[(u, qt)] = d if cidx == 0 else accs[(u, qt)] + d
            la = laccs.get((u, qt), [None, None, None])
            idx = jnp.full((KC, 128), UN * t + u, jnp.int32)
            vbs = [jnp.take_along_axis(vl_ref[r, cidx*KC:(cidx+1)*KC, :], idx, axis=1) for r in range(2)]
            for gi in range(KC // 8):
                pg = p32[gi*8:(gi+1)*8, :]
                la[2] = pg if la[2] is None else la[2] + pg
                for r in range(2):
                    vb = vbs[r][gi*8:(gi+1)*8, :]
                    term = pg * jnp.concatenate([vb] * (TQ // 128), axis=1)
                    la[r] = term if la[r] is None else la[r] + term
            laccs[(u, qt)] = la
            if cidx == NC - 1:
                finish_store(UN * t + u, accs.pop((u, qt)), laccs.pop((u, qt)), qt)

        for n in range(len(items) + 1):
            if n < len(items):
                qk(n)
            else:
                step5_slab(t)
            if n >= 1:
                pv(n - 1)
        return carry

    def slow_tile(i, carry):
        h = i // (S // SQ)
        q0 = pl.multiple_of((i % (S // SQ)) * SQ, SQ)
        r0 = pl.multiple_of(16 * h, 16)
        l0 = pl.multiple_of(512 + h // 16 * 16, 16)
        off = h % 16
        ones_row = (off + 1) % 16
        row16 = jax.lax.broadcasted_iota(jnp.int32, (16, S), 0)
        vl = vT_ref[pl.ds(l0, 16), :]
        vl = jnp.where(row16 == ones_row, jnp.ones_like(vl), vl)
        vw = jnp.concatenate([vT_ref[pl.ds(r0, 16), :], vl, vT_ref[pl.ds(l0 + 32, 16), :]], axis=0)
        sT = jnp.dot(k_ref[h, :, 0:32], qT_ref[h, :, pl.ds(q0, SQ)], preferred_element_type=F32)
        mx = jnp.max(sT, axis=0, keepdims=True)
        p = jnp.exp2(sT - mx).astype(BF)
        acc = jnp.dot(vw, p, preferred_element_type=F32)
        r16 = jax.lax.broadcasted_iota(jnp.int32, (16, SQ), 0)
        lo = acc[16:32]
        l = jnp.sum(jnp.where(r16 == ones_row, lo, 0.0), axis=0, keepdims=True)
        inv = 1.0 / l
        oT_ref[pl.ds(r0, 16), pl.ds(q0, SQ)] = acc[0:16] * inv
        store_left(h, jnp.sum(jnp.where(r16 == off, lo, 0.0), axis=0, keepdims=True) * inv,
                   jnp.sum(jnp.where(r16 == off, acc[32:48], 0.0), axis=0, keepdims=True) * inv, pl.ds(q0, SQ), SQ)
        return carry

    qmax = jnp.max(am_ref[0])
    kmax = jnp.max(am_ref[1])
    vmax = jnp.max(am_ref[2])
    safe = jnp.logical_and(qmax * kmax * (DH * 1.02) <= TB, vmax <= 2.0 ** 30)

    @pl.when(safe)
    def _():
        jax.lax.fori_loop(0, H // UN, fast_heads, 0)

    @pl.when(jnp.logical_not(safe))
    def _():
        def s5(t, carry):
            step5_slab(t)
            return carry
        jax.lax.fori_loop(0, N1, s5, 0)
        jax.lax.fori_loop(0, H * (S // SQ), slow_tile, 0)

    woT = woT_ref[...]
    cps = []
    for oc in range(S // OC):
        rs = slice(oc*OC, (oc+1)*OC)
        yT_ref[D:2*D, rs] = jnp.dot(woT, oT_ref[:, rs].astype(BF), preferred_element_type=F32).astype(BF)
        if oc == 0:
            for t_ in range(4):
                ob_ref[:, 128*t_:128*(t_+1)] = yT_ref[128*t_:128*(t_+1), :].T
            cp_oa = pltpu.make_async_copy(ob_ref.at[:, 0:512], o_hbm.at[:, 0:512], out_sems.at[0])
            cp_oa.start()
            cps.append(cp_oa)
        for t_ in range(4, 9):
            ob_ref[rs, 128*t_:128*(t_+1)] = yT_ref[128*t_:128*(t_+1), rs].T
        cp = pltpu.make_async_copy(ob_ref.at[rs, 512:1152], o_hbm.at[rs, 512:1152], out_sems.at[1 + oc])
        cp.start()
        cps.append(cp)
    for cp in cps:
        cp.wait()


_F1, _M, _FINV = _consts()


@jax.jit
def pallas_concat_heads__spectral_gfnet__mha_block__prompt_kernel(A_x, A_w_r, A_w_i, B_x, B_wqkv, B_wo):
    anyspec = pl.BlockSpec(memory_space=pl.ANY)
    out = pl.pallas_call(
        _kernel,
        out_shape=jax.ShapeDtypeStruct((S, 2 * D), BF),
        in_specs=[anyspec] * 9,
        out_specs=anyspec,
        scratch_shapes=[
            pltpu.VMEM((D, S), BF), pltpu.VMEM((DF, S), BF), pltpu.VMEM((DF, S), BF), pltpu.VMEM((D, S), BF),
            pltpu.VMEM((D, 3 * D), BF), pltpu.VMEM((D, D), BF), pltpu.VMEM((2 * R, HD), BF),
            pltpu.VMEM((N1, 256, 256), BF), pltpu.VMEM((HD, 2 * R), BF), pltpu.VMEM((S, 2 * D), BF),
            pltpu.VMEM((H, 32, S), BF), pltpu.VMEM((H, S, 128), BF),
            pltpu.VMEM((D, S), BF), pltpu.VMEM((D, S), F32),
            pltpu.VMEM((2 * R, S), F32), pltpu.VMEM((N1, R, 256), BF), pltpu.VMEM((2 * R, S), BF),
            pltpu.VMEM((2, 3, S, 128), F32), pltpu.VMEM((2, N1, R, 128), F32),
            pltpu.VMEM((S, D), BF), pltpu.VMEM((640 + D, D), BF), pltpu.VMEM((3, 8, 128), F32),
            pltpu.VMEM((2, S, 128), F32), pltpu.VMEM((2 * D, S), BF), pltpu.VMEM((D, 640), BF), pltpu.VMEM((D, D), BF),
            pltpu.SemaphoreType.DMA((13,)), pltpu.SemaphoreType.DMA((1 + S // OC,)),
        ],
        compiler_params=pltpu.CompilerParams(vmem_limit_bytes=110 << 20),
    )(A_x[0].T, A_w_r.T, A_w_i.T, B_x[0].T, B_wqkv, B_wo, jnp.asarray(_F1), jnp.asarray(_M), jnp.asarray(_FINV))
    return out[None]
```

```python
import functools

import numpy as np
import jax
import jax.numpy as jnp
from jax.experimental import pallas as pl
from jax.experimental.pallas import tpu as pltpu

S, D, H, DH = 2048, 576, 32, 18
DF = D // 2 + 1
HD = D // 2
RE, RO = 160, 144
R = RE + RO
N1, N2 = 16, 128
LOG2E = 1.4426950408889634
BF = jnp.bfloat16
F32 = jnp.float32

TQ, KC, UN = 1024, 128, 2
RC = 16
PC = 512
XC = 4
OC = 512
SQ = 128
TB = 40.0
assert H // UN == N1


def _consts():
    r = np.arange(R)
    f = np.where(r < RE, 2 * r, 2 * (r - RE) + 1).astype(np.float64)[:, None]
    valid = (f < DF)
    d = np.arange(HD)[None, :].astype(np.float64)
    ang = 2 * np.pi * ((f * d) % D) / D
    c_, s_ = np.where(valid, np.cos(ang), 0.0), np.where(valid, -np.sin(ang), 0.0)
    f1 = np.concatenate([c_[:RE], s_[:RE], c_[RE:], s_[RE:]], axis=0)
    cf = np.where((f == 0) | (f == DF - 1), 1.0, 2.0) / (S * D)
    ci, si = cf * c_, cf * s_
    finv = np.concatenate([ci[:RE], si[:RE], ci[RE:], si[RE:]], axis=0).T
    n2 = np.arange(N2)[:, None]
    k2 = np.arange(N2)[None, :]
    ms = []
    for k1 in range(N1):
        th = 2 * np.pi * ((n2 * (k1 + N1 * k2)) % S) / S
        c, s = np.cos(th), np.sin(th)
        ms.append(np.block([[c, -s], [s, c]]))
    m = np.stack(ms)
    return (f1.astype(BF), m.astype(BF), np.ascontiguousarray(finv).astype(BF))


def _cmul_const(a, w):
    ar, ai = a
    wr, wi = float(np.real(w)), float(np.imag(w))
    eps = 1e-12
    if abs(wi) < eps and abs(wr - 1) < eps:
        return ar, ai
    if abs(wi) < eps and abs(wr + 1) < eps:
        return -ar, -ai
    if abs(wr) < eps and abs(wi + 1) < eps:
        return ai, -ar
    if abs(wr) < eps and abs(wi - 1) < eps:
        return -ai, ar
    if abs(abs(wr) - abs(wi)) < eps:
        c = abs(wr)
        sr, si = np.sign(wr), np.sign(wi)
        t1 = (ar - ai) if sr * si > 0 else (ar + ai)
        t2 = (ar + ai) if sr * si > 0 else (ar - ai)
        return t1 * (c * sr), t2 * (c * si)
    return ar * wr - ai * wi, ar * wi + ai * wr


def _fft_list(xs, sign):
    n = len(xs)
    if n == 1:
        return xs
    ev = _fft_list(xs[0::2], sign)
    od = _fft_list(xs[1::2], sign)
    out = [None] * n
    for k in range(n // 2):
        t = _cmul_const(od[k], np.exp(sign * 2j * np.pi * k / n))
        out[k] = (ev[k][0] + t[0], ev[k][1] + t[1])
        out[k + n // 2] = (ev[k][0] - t[0], ev[k][1] - t[1])
    return out


def _split_heads_rows(a):
    return jnp.concatenate([a[18*h:18*h+16] for h in range(H)] + [a[18*h+16:18*h+17] for h in range(H)]
                           + [a[18*h+17:18*h+18] for h in range(H)], axis=0)


def _kernel(xa_hbm, wr_hbm, wi_hbm, xb_hbm, w_hbm, wo_hbm, f1_hbm, m_hbm, finv_hbm, o_hbm,
            xa_ref, wr_ref, wi_ref, xb_ref, w_ref, wo_ref, f1_ref, m_ref, finv_ref, ob_ref,
            qT_ref, k_ref, vT_ref, oT_ref, xf_ref, t_ref, g_ref, wn_ref, wp_ref, x_ref, wT_ref, am_ref,
            vl_ref, yT_ref, wk_ref, woT_ref, lr_ref, in_sems, out_sems):
    NQ = S // TQ
    NC = S // KC
    NPC = S // PC
    cp_f1 = pltpu.make_async_copy(f1_hbm, f1_ref, in_sems.at[0])
    cp_xa = [pltpu.make_async_copy(xa_hbm.at[:, c*(S//XC):(c+1)*(S//XC)], xa_ref.at[:, c*(S//XC):(c+1)*(S//XC)],
                                   in_sems.at[1 + c]) for c in range(XC)]
    cp_wr = pltpu.make_async_copy(wr_hbm, wr_ref, in_sems.at[5])
    cp_wi = pltpu.make_async_copy(wi_hbm, wi_ref, in_sems.at[6])
    cp_m = pltpu.make_async_copy(m_hbm, m_ref, in_sems.at[7])
    cp_finv = pltpu.make_async_copy(finv_hbm, finv_ref, in_sems.at[8])
    cp_xb = pltpu.make_async_copy(xb_hbm, xb_ref, in_sems.at[9])
    cp_w = pltpu.make_async_copy(w_hbm.at[:, 0:640], w_ref.at[:, 0:640], in_sems.at[10])
    cp_w2 = pltpu.make_async_copy(w_hbm.at[:, 640:3*D], w_ref.at[:, 640:3*D], in_sems.at[12])
    cp_wo = pltpu.make_async_copy(wo_hbm, wo_ref, in_sems.at[11])
    for cp in [cp_f1, cp_xa[0]]:
        cp.start()

    c = (DH ** -0.5) * LOG2E
    am_ref[...] = jnp.zeros_like(am_ref)
    frow = jax.lax.broadcasted_iota(jnp.int32, (R - 256, 128), 0)

    def wperm_a(a):
        wref = (wr_ref, wi_ref)[a]
        wn_ref[a, 0] = wref[0:128, :].T.astype(F32)
        wn_ref[a, 1] = wref[128:256, :].T.astype(F32)
        wn_ref[a, 2, :, 0:DF-256] = wref[256:DF, :].T.astype(F32)

    def wperm_b(a, k1):
        for j in range(2):
            wp_ref[a, k1, j*128:(j+1)*128, :] = wn_ref[a, j, pl.ds(k1, N2, stride=N1), :].T
        blk = wn_ref[a, 2, pl.ds(k1, N2, stride=N1), :].T[0:R-256, :]
        wp_ref[a, k1, 256:R, :] = jnp.where(frow < DF - 256, blk, 0.0)

    def stage_a_fwd(rc):
        r0 = rc * RC
        xs = [(xf_ref[r0:r0+RC, n1*128:(n1+1)*128], xf_ref[R+r0:R+r0+RC, n1*128:(n1+1)*128]) for n1 in range(N1)]
        ys = _fft_list(xs, -1)
        for k1 in range(N1):
            t_ref[k1, r0:r0+RC, 0:128] = ys[k1][0].astype(BF)
            t_ref[k1, r0:r0+RC, 128:256] = ys[k1][1].astype(BF)

    def stage_a_inv(rc):
        r0 = rc * RC
        xs = [(xf_ref[r0:r0+RC, k1*128:(k1+1)*128], xf_ref[R+r0:R+r0+RC, k1*128:(k1+1)*128]) for k1 in range(N1)]
        ys = _fft_list(xs, +1)
        gr0, gi0 = (r0, RE + r0) if r0 < RE else (RE + r0, RE + RO + r0)
        for n1 in range(N1):
            g_ref[gr0:gr0+RC, n1*128:(n1+1)*128] = ys[n1][0].astype(BF)
            g_ref[gi0:gi0+RC, n1*128:(n1+1)*128] = ys[n1][1].astype(BF)

    def track(idx, val):
        a = jnp.abs(val)
        a = jnp.max(a.reshape(a.shape[0] // 8, 8, a.shape[1]), axis=0)
        a = functools.reduce(jnp.maximum, [a[:, l*128:(l+1)*128] for l in range(a.shape[1] // 128)])
        am_ref[idx] = jnp.maximum(am_ref[idx], a)

    def proj_k(g, pc):
        wk = wk_ref[:, 128*g:128*(g+1)]
        kk = jnp.dot(x_ref[pc*PC:(pc+1)*PC, :], wk, preferred_element_type=F32)
        track(1, kk)
        kb = kk.astype(BF)
        k32 = pltpu.bitcast(kb, jnp.uint32)
        for j in range(min(7, H - 7 * g)):
            kr = kb if j == 0 else pltpu.bitcast(pltpu.roll(k32, 128 - 18 * j, 1), BF)
            k_ref[7*g + j, pc*PC:(pc+1)*PC, :] = kr

    def proj_q(g, pc):
        qT = jnp.dot(wT_ref[144*g:144*(g+1), :], xb_ref[:, pc*PC:(pc+1)*PC], preferred_element_type=F32) * c
        track(0, qT)
        for j in range(8):
            qT_ref[8*g + j, :, pc*PC:(pc+1)*PC] = jnp.concatenate(
                [qT[18*j:18*j+18], jnp.zeros((14, PC), F32)], axis=0).astype(BF)

    def proj_v(r, pc):
        rr = slice(640 + r*192, 640 + (r+1)*192)
        vv = jnp.dot(wT_ref[rr, :], xb_ref[:, pc*PC:(pc+1)*PC], preferred_element_type=F32)
        track(2, vv)
        vT_ref[r*192:(r+1)*192, pc*PC:(pc+1)*PC] = vv.astype(BF)

    def interleave(mx, vp):
        n = max(len(mx), 1)
        done = 0
        for i, f in enumerate(mx):
            f()
            upto = (i + 1) * len(vp) // n
            for g_ in vp[done:upto]:
                g_()
            done = upto
        for g_ in vp[done:]:
            g_()

    cp_f1.wait()
    cp_xa[0].wait()
    for cp in cp_xa[1:] + [cp_xb, cp_w, cp_w2, cp_wr, cp_wi, cp_m, cp_finv, cp_wo]:
        cp.start()
    for cc in range(XC):
        if cc > 0:
            cp_xa[cc].wait()
        sl = slice(cc*(S//XC), (cc+1)*(S//XC))
        x0 = xa_ref[0:HD, sl].astype(F32)
        x1 = xa_ref[HD:D, sl].astype(F32)
        xe = jnp.dot(f1_ref[0:2*RE, :], (x0 + x1).astype(BF), preferred_element_type=F32)
        xo = jnp.dot(f1_ref[2*RE:2*R, :], (x0 - x1).astype(BF), preferred_element_type=F32)
        xf_ref[0:RE, sl] = xe[0:RE]
        xf_ref[R:R+RE, sl] = xe[RE:2*RE]
        xf_ref[RE:R, sl] = xo[0:RO]
        xf_ref[R+RE:2*R, sl] = xo[RO:2*RO]
    for rc in range(R // RC):
        stage_a_fwd(rc)
    cp_xb.wait()
    cp_w.wait()

    wT_ref[0:640, :] = w_ref[:, 0:640].T
    x_ref[...] = xb_ref[...].T
    mq = [functools.partial(proj_q, g, pc) for g in range(4) for pc in range(NPC)]
    for f_ in mq[:2*NPC]:
        f_()
    cp_w2.wait()
    wvT = w_ref[:, 1152:1728].T.astype(F32)
    wT_ref[640:640+512, :] = jnp.concatenate([wvT[18*h:18*h+16] for h in range(H)], axis=0).astype(BF)
    wT_ref[640+512:640+D, :] = jnp.concatenate(
        [wvT[18*h+16:18*h+17] for h in range(H)] + [wvT[18*h+17:18*h+18] for h in range(H)], axis=0).astype(BF)
    for g in range(5):
        wk_ref[:, 128*g:128*(g+1)] = w_ref[:, 576+126*g:576+126*g+128]
    for f_ in mq[2*NPC:]:
        f_()
    cp_wr.wait()
    cp_wi.wait()
    vp = ([functools.partial(wperm_a, 0), functools.partial(wperm_a, 1)]
          + [functools.partial(wperm_b, a, k1) for a in range(2) for k1 in range(N1)])
    interleave([functools.partial(proj_v, r, pc) for r in range(3) for pc in range(NPC)], vp)
    cp_m.wait()

    def mid(k1, carry):
        c0 = pl.multiple_of(k1 * 128, 128)
        mk = m_ref[k1]
        z = jnp.dot(t_ref[k1], mk, preferred_element_type=F32)
        zr, zi = z[:, :128], z[:, 128:]
        wr, wi = [jnp.concatenate([wp_ref[a, k1, pl.ds(0, 152, stride=2), :], jnp.zeros((8, 128), F32),
                                   wp_ref[a, k1, pl.ds(1, RO, stride=2), :]], axis=0) for a in range(2)]
        yr = zr * wr - zi * wi
        yi = zr * wi + zi * wr
        y = jnp.concatenate([yr, yi], axis=1).astype(BF)
        tp = jax.lax.dot_general(y, mk, (((1,), (1,)), ((), ())), preferred_element_type=F32)
        xf_ref[0:R, pl.ds(c0, 128)] = tp[:, :128]
        xf_ref[R:2*R, pl.ds(c0, 128)] = tp[:, 128:]
        return carry
    jax.lax.fori_loop(0, N1, mid, 0, unroll=4)

    mx2 = [functools.partial(proj_k, g, pc) for g in range(5) for pc in range(NPC)]
    interleave(mx2, [functools.partial(stage_a_inv, rc) for rc in range(R // RC)])
    vlt = vT_ref[512:D, :].T.astype(F32) * (2.0 ** TB)
    vlt = jnp.concatenate([vlt, jnp.zeros((S, 64), F32)], axis=1)
    vl_ref[0] = vlt
    vl_ref[1] = pltpu.roll(vlt, 96, 1)
    cp_finv.wait()
    cp_wo.wait()
    woT_ref[...] = _split_heads_rows(wo_ref[...].astype(F32)).astype(BF).T

    def step5_slab(t):
        sl = pl.ds(pl.multiple_of(t * 128, 128), 128)
        ee = jnp.dot(finv_ref[:, 0:2*RE], g_ref[0:2*RE, sl], preferred_element_type=F32)
        oo = jnp.dot(finv_ref[:, 2*RE:2*R], g_ref[2*RE:2*R, sl], preferred_element_type=F32)
        yT_ref[0:HD, sl] = (ee + oo).astype(BF)
        yT_ref[HD:D, sl] = (ee - oo).astype(BF)

    def finish_store(h, acc, lacc, qt):
        r0 = pl.multiple_of(16 * h, 16)
        oT_ref[pl.ds(r0, 16), qt*TQ:(qt+1)*TQ] = acc
        for r in range(3):
            lr_ref[r, h, :, qt*TQ:(qt+1)*TQ] = lacc[r]

    def fast_heads(t, carry):
        items = [(u, qt, cidx) for u in range(UN) for qt in range(NQ) for cidx in range(NC)]
        vws = {}; ss = {}; accs = {}; laccs = {}
        for u in range(UN):
            r0 = pl.multiple_of(16 * (UN * t + u), 16)
            vws[u] = (vT_ref[pl.ds(r0, 16), :].astype(F32) * (2.0 ** TB)).astype(BF)

        def qk(n):
            u, qt, cidx = items[n]
            h = UN * t + u
            ss[n] = jnp.dot(k_ref[h, cidx*KC:(cidx+1)*KC, 0:32], qT_ref[h, :, qt*TQ:(qt+1)*TQ],
                            preferred_element_type=F32)

        def pv(n):
            u, qt, cidx = items[n]
            vw = vws[u]
            p32 = jnp.exp2(ss.pop(n))
            p = p32.astype(BF)
            d = jnp.dot(vw[:, cidx*KC:(cidx+1)*KC], p, preferred_element_type=F32)
            accs[(u, qt)] = d if cidx == 0 else accs[(u, qt)] + d
            la = laccs.get((u, qt), [None, None, None])
            idx = jnp.full((KC, 128), UN * t + u, jnp.int32)
            vbs = [jnp.take_along_axis(vl_ref[r, cidx*KC:(cidx+1)*KC, :], idx, axis=1) for r in range(2)]
            for gi in range(KC // 8):
                pg = p32[gi*8:(gi+1)*8, :]
                la[2] = pg if la[2] is None else la[2] + pg
                for r in range(2):
                    vb = vbs[r][gi*8:(gi+1)*8, :]
                    term = pg * jnp.concatenate([vb] * (TQ // 128), axis=1)
                    la[r] = term if la[r] is None else la[r] + term
            laccs[(u, qt)] = la
            if cidx == NC - 1:
                finish_store(UN * t + u, accs.pop((u, qt)), laccs.pop((u, qt)), qt)

        for n in range(len(items) + 1):
            if n < len(items):
                qk(n)
            else:
                step5_slab(t)
            if n >= 1:
                pv(n - 1)
        return carry

    def slow_tile(i, carry):
        h = i // (S // SQ)
        q0 = pl.multiple_of((i % (S // SQ)) * SQ, SQ)
        r0 = pl.multiple_of(16 * h, 16)
        l0 = pl.multiple_of(512 + h // 16 * 16, 16)
        off = h % 16
        ones_row = (off + 1) % 16
        row16 = jax.lax.broadcasted_iota(jnp.int32, (16, S), 0)
        vl = vT_ref[pl.ds(l0, 16), :]
        vl = jnp.where(row16 == ones_row, jnp.ones_like(vl), vl)
        vw = jnp.concatenate([vT_ref[pl.ds(r0, 16), :], vl, vT_ref[pl.ds(l0 + 32, 16), :]], axis=0)
        sT = jnp.dot(k_ref[h, :, 0:32], qT_ref[h, :, pl.ds(q0, SQ)], preferred_element_type=F32)
        mx = jnp.max(sT, axis=0, keepdims=True)
        p = jnp.exp2(sT - mx).astype(BF)
        acc = jnp.dot(vw, p, preferred_element_type=F32)
        r16 = jax.lax.broadcasted_iota(jnp.int32, (16, SQ), 0)
        lo = acc[16:32]
        oT_ref[pl.ds(r0, 16), pl.ds(q0, SQ)] = acc[0:16]
        hi = acc[32:48]
        for r, part in enumerate((jnp.where(r16 == off, lo, 0.0), jnp.where(r16 == off, hi, 0.0),
                                  jnp.where(r16 == ones_row, lo, 0.0) * (2.0 ** -TB))):
            lr_ref[r, h, :, pl.ds(q0, SQ)] = part[0:8] + part[8:16]
        return carry

    qmax = jnp.max(am_ref[0])
    kmax = jnp.max(am_ref[1])
    vmax = jnp.max(am_ref[2])
    safe = jnp.logical_and(qmax * kmax * (DH * 1.02) <= TB, vmax <= 2.0 ** 30)

    @pl.when(safe)
    def _():
        jax.lax.fori_loop(0, H // UN, fast_heads, 0)

    @pl.when(jnp.logical_not(safe))
    def _():
        def s5(t, carry):
            step5_slab(t)
            return carry
        jax.lax.fori_loop(0, N1, s5, 0)
        jax.lax.fori_loop(0, H * (S // SQ), slow_tile, 0)

    woT = woT_ref[...]
    cps = []
    for oc in range(S // OC):
        rs = slice(oc*OC, (oc+1)*OC)
        sums = [jnp.sum(lr_ref[r, :, :, rs], axis=1) for r in range(3)]
        inv = 1.0 / (sums[2] * (2.0 ** TB))
        main = (oT_ref[0:512, rs].reshape(H, 16, OC) * inv[:, None, :]).reshape(512, OC)
        on = jnp.concatenate([main, sums[0] * inv, sums[1] * inv], axis=0).astype(BF)
        yT_ref[D:2*D, rs] = jnp.dot(woT, on, preferred_element_type=F32).astype(BF)
        if oc == 0:
            for t_ in range(4):
                ob_ref[:, 128*t_:128*(t_+1)] = yT_ref[128*t_:128*(t_+1), :].T
            cp_oa = pltpu.make_async_copy(ob_ref.at[:, 0:512], o_hbm.at[:, 0:512], out_sems.at[0])
            cp_oa.start()
            cps.append(cp_oa)
        for t_ in range(4, 9):
            ob_ref[rs, 128*t_:128*(t_+1)] = yT_ref[128*t_:128*(t_+1), rs].T
        cp = pltpu.make_async_copy(ob_ref.at[rs, 512:1152], o_hbm.at[rs, 512:1152], out_sems.at[1 + oc])
        cp.start()
        cps.append(cp)
    for cp in cps:
        cp.wait()


_F1, _M, _FINV = _consts()


@jax.jit
def pallas_concat_heads__spectral_gfnet__mha_block__prompt_kernel(A_x, A_w_r, A_w_i, B_x, B_wqkv, B_wo):
    anyspec = pl.BlockSpec(memory_space=pl.ANY)
    out = pl.pallas_call(
        _kernel,
        out_shape=jax.ShapeDtypeStruct((S, 2 * D), BF),
        in_specs=[anyspec] * 9,
        out_specs=anyspec,
        scratch_shapes=[
            pltpu.VMEM((D, S), BF), pltpu.VMEM((DF, S), BF), pltpu.VMEM((DF, S), BF), pltpu.VMEM((D, S), BF),
            pltpu.VMEM((D, 3 * D), BF), pltpu.VMEM((D, D), BF), pltpu.VMEM((2 * R, HD), BF),
            pltpu.VMEM((N1, 256, 256), BF), pltpu.VMEM((HD, 2 * R), BF), pltpu.VMEM((S, 2 * D), BF),
            pltpu.VMEM((H, 32, S), BF), pltpu.VMEM((H, S, 128), BF),
            pltpu.VMEM((D, S), BF), pltpu.VMEM((512, S), F32),
            pltpu.VMEM((2 * R, S), F32), pltpu.VMEM((N1, R, 256), BF), pltpu.VMEM((2 * R, S), BF),
            pltpu.VMEM((2, 3, S, 128), F32), pltpu.VMEM((2, N1, R, 128), F32),
            pltpu.VMEM((S, D), BF), pltpu.VMEM((640 + D, D), BF), pltpu.VMEM((3, 8, 128), F32),
            pltpu.VMEM((2, S, 128), F32), pltpu.VMEM((2 * D, S), BF), pltpu.VMEM((D, 640), BF), pltpu.VMEM((D, D), BF), pltpu.VMEM((3, H, 8, S), F32),
            pltpu.SemaphoreType.DMA((13,)), pltpu.SemaphoreType.DMA((1 + S // OC,)),
        ],
        compiler_params=pltpu.CompilerParams(vmem_limit_bytes=110 << 20),
    )(A_x[0].T, A_w_r.T, A_w_i.T, B_x[0].T, B_wqkv, B_wo, jnp.asarray(_F1), jnp.asarray(_M), jnp.asarray(_FINV))
    return out[None]
```

```python
import functools

import numpy as np
import jax
import jax.numpy as jnp
from jax.experimental import pallas as pl
from jax.experimental.pallas import tpu as pltpu

S, D, H, DH = 2048, 576, 32, 18
DF = D // 2 + 1
HD = D // 2
RE, RO = 160, 144
R = RE + RO
N1, N2 = 16, 128
LOG2E = 1.4426950408889634
BF = jnp.bfloat16
F32 = jnp.float32

TQ, KC, UN = 1024, 128, 2
RC = 16
PC = 512
XC = 4
OC = 512
SQ = 128
TB = 40.0
assert H // UN == N1


def _consts():
    r = np.arange(R)
    f = np.where(r < RE, 2 * r, 2 * (r - RE) + 1).astype(np.float64)[:, None]
    valid = (f < DF)
    d = np.arange(HD)[None, :].astype(np.float64)
    ang = 2 * np.pi * ((f * d) % D) / D
    c_, s_ = np.where(valid, np.cos(ang), 0.0), np.where(valid, -np.sin(ang), 0.0)
    f1 = np.concatenate([c_[:RE], s_[:RE], c_[RE:], s_[RE:]], axis=0)
    cf = np.where((f == 0) | (f == DF - 1), 1.0, 2.0) / (S * D)
    ci, si = cf * c_, cf * s_
    finv = np.concatenate([ci[:RE], si[:RE], ci[RE:], si[RE:]], axis=0).T
    n2 = np.arange(N2)[:, None]
    k2 = np.arange(N2)[None, :]
    ms = []
    for k1 in range(N1):
        th = 2 * np.pi * ((n2 * (k1 + N1 * k2)) % S) / S
        c, s = np.cos(th), np.sin(th)
        ms.append(np.block([[c, -s], [s, c]]))
    m = np.stack(ms)
    return (f1.astype(BF), m.astype(BF), np.ascontiguousarray(finv).astype(BF))


def _cmul_const(a, w):
    ar, ai = a
    wr, wi = float(np.real(w)), float(np.imag(w))
    eps = 1e-12
    if abs(wi) < eps and abs(wr - 1) < eps:
        return ar, ai
    if abs(wi) < eps and abs(wr + 1) < eps:
        return -ar, -ai
    if abs(wr) < eps and abs(wi + 1) < eps:
        return ai, -ar
    if abs(wr) < eps and abs(wi - 1) < eps:
        return -ai, ar
    if abs(abs(wr) - abs(wi)) < eps:
        c = abs(wr)
        sr, si = np.sign(wr), np.sign(wi)
        t1 = (ar - ai) if sr * si > 0 else (ar + ai)
        t2 = (ar + ai) if sr * si > 0 else (ar - ai)
        return t1 * (c * sr), t2 * (c * si)
    return ar * wr - ai * wi, ar * wi + ai * wr


def _fft_list(xs, sign):
    n = len(xs)
    if n == 1:
        return xs
    ev = _fft_list(xs[0::2], sign)
    od = _fft_list(xs[1::2], sign)
    out = [None] * n
    for k in range(n // 2):
        t = _cmul_const(od[k], np.exp(sign * 2j * np.pi * k / n))
        out[k] = (ev[k][0] + t[0], ev[k][1] + t[1])
        out[k + n // 2] = (ev[k][0] - t[0], ev[k][1] - t[1])
    return out


def _split_heads_rows(a):
    return jnp.concatenate([a[18*h:18*h+16] for h in range(H)] + [a[18*h+16:18*h+17] for h in range(H)]
                           + [a[18*h+17:18*h+18] for h in range(H)], axis=0)


def _kernel(xa_hbm, wr_hbm, wi_hbm, xb_hbm, w_hbm, wo_hbm, f1_hbm, m_hbm, finv_hbm, o_hbm,
            xa_ref, wr_ref, wi_ref, xb_ref, w_ref, wo_ref, f1_ref, m_ref, finv_ref, ob_ref,
            qT_ref, k_ref, vT_ref, oT_ref, xf_ref, t_ref, g_ref, wn_ref, wp_ref, x_ref, wT_ref, am_ref,
            vl_ref, yT_ref, wk_ref, woT_ref, lr_ref, in_sems, out_sems):
    NQ = S // TQ
    NC = S // KC
    NPC = S // PC
    cp_f1 = pltpu.make_async_copy(f1_hbm, f1_ref, in_sems.at[0])
    cp_xa = [pltpu.make_async_copy(xa_hbm.at[:, c*(S//XC):(c+1)*(S//XC)], xa_ref.at[:, c*(S//XC):(c+1)*(S//XC)],
                                   in_sems.at[1 + c]) for c in range(XC)]
    cp_wr = pltpu.make_async_copy(wr_hbm, wr_ref, in_sems.at[5])
    cp_wi = pltpu.make_async_copy(wi_hbm, wi_ref, in_sems.at[6])
    cp_m = pltpu.make_async_copy(m_hbm, m_ref, in_sems.at[7])
    cp_finv = pltpu.make_async_copy(finv_hbm, finv_ref, in_sems.at[8])
    cp_xb = [pltpu.make_async_copy(xb_hbm.at[:, c*PC:(c+1)*PC], xb_ref.at[:, c*PC:(c+1)*PC], in_sems.at[13 + c]) for c in range(NPC)]
    cp_w = pltpu.make_async_copy(w_hbm.at[:, 0:640], w_ref.at[:, 0:640], in_sems.at[10])
    cp_w2 = pltpu.make_async_copy(w_hbm.at[:, 640:3*D], w_ref.at[:, 640:3*D], in_sems.at[12])
    cp_wo = pltpu.make_async_copy(wo_hbm, wo_ref, in_sems.at[11])
    for cp in [cp_f1, cp_xa[0]]:
        cp.start()

    c = (DH ** -0.5) * LOG2E
    am_ref[...] = jnp.zeros_like(am_ref)
    frow = jax.lax.broadcasted_iota(jnp.int32, (R - 256, 128), 0)

    def wperm_a(a):
        wref = (wr_ref, wi_ref)[a]
        wn_ref[a, 0] = wref[0:128, :].T.astype(F32)
        wn_ref[a, 1] = wref[128:256, :].T.astype(F32)
        wn_ref[a, 2, :, 0:DF-256] = wref[256:DF, :].T.astype(F32)

    def wperm_b(a, k1):
        for j in range(2):
            wp_ref[a, k1, j*128:(j+1)*128, :] = wn_ref[a, j, pl.ds(k1, N2, stride=N1), :].T
        blk = wn_ref[a, 2, pl.ds(k1, N2, stride=N1), :].T[0:R-256, :]
        wp_ref[a, k1, 256:R, :] = jnp.where(frow < DF - 256, blk, 0.0)

    def stage_a_fwd(rc):
        r0 = rc * RC
        xs = [(xf_ref[r0:r0+RC, n1*128:(n1+1)*128], xf_ref[R+r0:R+r0+RC, n1*128:(n1+1)*128]) for n1 in range(N1)]
        ys = _fft_list(xs, -1)
        for k1 in range(N1):
            t_ref[k1, r0:r0+RC, 0:128] = ys[k1][0].astype(BF)
            t_ref[k1, r0:r0+RC, 128:256] = ys[k1][1].astype(BF)

    def stage_a_inv(rc):
        r0 = rc * RC
        xs = [(xf_ref[r0:r0+RC, k1*128:(k1+1)*128], xf_ref[R+r0:R+r0+RC, k1*128:(k1+1)*128]) for k1 in range(N1)]
        ys = _fft_list(xs, +1)
        gr0, gi0 = (r0, RE + r0) if r0 < RE else (RE + r0, RE + RO + r0)
        for n1 in range(N1):
            g_ref[gr0:gr0+RC, n1*128:(n1+1)*128] = ys[n1][0].astype(BF)
            g_ref[gi0:gi0+RC, n1*128:(n1+1)*128] = ys[n1][1].astype(BF)

    def track(idx, val):
        a = jnp.abs(val)
        a = jnp.max(a.reshape(a.shape[0] // 8, 8, a.shape[1]), axis=0)
        a = functools.reduce(jnp.maximum, [a[:, l*128:(l+1)*128] for l in range(a.shape[1] // 128)])
        am_ref[idx] = jnp.maximum(am_ref[idx], a)

    def proj_k(g, pc):
        wk = wk_ref[:, 128*g:128*(g+1)]
        kk = jnp.dot(x_ref[pc*PC:(pc+1)*PC, :], wk, preferred_element_type=F32)
        track(1, kk)
        kb = kk.astype(BF)
        k32 = pltpu.bitcast(kb, jnp.uint32)
        for j in range(min(7, H - 7 * g)):
            kr = kb if j == 0 else pltpu.bitcast(pltpu.roll(k32, 128 - 18 * j, 1), BF)
            k_ref[7*g + j, pc*PC:(pc+1)*PC, :] = kr

    def proj_q(g, pc):
        qT = jnp.dot(wT_ref[144*g:144*(g+1), :], xb_ref[:, pc*PC:(pc+1)*PC], preferred_element_type=F32) * c
        track(0, qT)
        for j in range(8):
            qT_ref[8*g + j, :, pc*PC:(pc+1)*PC] = jnp.concatenate(
                [qT[18*j:18*j+18], jnp.zeros((14, PC), F32)], axis=0).astype(BF)

    def proj_v(r, pc):
        rr = slice(640 + r*192, 640 + (r+1)*192)
        vv = jnp.dot(wT_ref[rr, :], xb_ref[:, pc*PC:(pc+1)*PC], preferred_element_type=F32)
        track(2, vv)
        vT_ref[r*192:(r+1)*192, pc*PC:(pc+1)*PC] = vv.astype(BF)

    def interleave(mx, vp):
        n = max(len(mx), 1)
        done = 0
        for i, f in enumerate(mx):
            f()
            upto = (i + 1) * len(vp) // n
            for g_ in vp[done:upto]:
                g_()
            done = upto
        for g_ in vp[done:]:
            g_()

    cp_f1.wait()
    cp_xa[0].wait()
    for cp in cp_xa[1:] + [cp_w] + cp_xb + [cp_w2, cp_wr, cp_wi, cp_m, cp_finv, cp_wo]:
        cp.start()
    for cc in range(XC):
        if cc > 0:
            cp_xa[cc].wait()
        sl = slice(cc*(S//XC), (cc+1)*(S//XC))
        x0 = xa_ref[0:HD, sl].astype(F32)
        x1 = xa_ref[HD:D, sl].astype(F32)
        xe = jnp.dot(f1_ref[0:2*RE, :], (x0 + x1).astype(BF), preferred_element_type=F32)
        xo = jnp.dot(f1_ref[2*RE:2*R, :], (x0 - x1).astype(BF), preferred_element_type=F32)
        xf_ref[0:RE, sl] = xe[0:RE]
        xf_ref[R:R+RE, sl] = xe[RE:2*RE]
        xf_ref[RE:R, sl] = xo[0:RO]
        xf_ref[R+RE:2*R, sl] = xo[RO:2*RO]
    for rc in range(R // RC):
        stage_a_fwd(rc)
    cp_w.wait()

    wT_ref[0:640, :] = w_ref[:, 0:640].T
    for pc in range(NPC):
        cp_xb[pc].wait()
        if pc == 2:
            cp_w2.wait()
            wvT = w_ref[:, 1152:1728].T.astype(F32)
            wT_ref[640:640+512, :] = jnp.concatenate([wvT[18*h:18*h+16] for h in range(H)], axis=0).astype(BF)
            wT_ref[640+512:640+D, :] = jnp.concatenate(
                [wvT[18*h+16:18*h+17] for h in range(H)] + [wvT[18*h+17:18*h+18] for h in range(H)], axis=0).astype(BF)
            for g in range(5):
                wk_ref[:, 128*g:128*(g+1)] = w_ref[:, 576+126*g:576+126*g+128]
        x_ref[pc*PC:(pc+1)*PC, :] = xb_ref[:, pc*PC:(pc+1)*PC].T
        for g in range(4):
            proj_q(g, pc)
    cp_wr.wait()
    cp_wi.wait()
    vp = ([functools.partial(wperm_a, 0), functools.partial(wperm_a, 1)]
          + [functools.partial(wperm_b, a, k1) for a in range(2) for k1 in range(N1)])
    interleave([functools.partial(proj_v, r, pc) for r in range(3) for pc in range(NPC)], vp)
    cp_m.wait()

    def mid(k1, carry):
        c0 = pl.multiple_of(k1 * 128, 128)
        mk = m_ref[k1]
        z = jnp.dot(t_ref[k1], mk, preferred_element_type=F32)
        zr, zi = z[:, :128], z[:, 128:]
        wr, wi = [jnp.concatenate([wp_ref[a, k1, pl.ds(0, 152, stride=2), :], jnp.zeros((8, 128), F32),
                                   wp_ref[a, k1, pl.ds(1, RO, stride=2), :]], axis=0) for a in range(2)]
        yr = zr * wr - zi * wi
        yi = zr * wi + zi * wr
        y = jnp.concatenate([yr, yi], axis=1).astype(BF)
        tp = jax.lax.dot_general(y, mk, (((1,), (1,)), ((), ())), preferred_element_type=F32)
        xf_ref[0:R, pl.ds(c0, 128)] = tp[:, :128]
        xf_ref[R:2*R, pl.ds(c0, 128)] = tp[:, 128:]
        return carry
    jax.lax.fori_loop(0, N1, mid, 0, unroll=4)

    mx2 = [functools.partial(proj_k, g, pc) for g in range(5) for pc in range(NPC)]
    interleave(mx2, [functools.partial(stage_a_inv, rc) for rc in range(R // RC)])
    vlt = vT_ref[512:D, :].T.astype(F32) * (2.0 ** TB)
    vlt = jnp.concatenate([vlt, jnp.zeros((S, 64), F32)], axis=1)
    vl_ref[0] = vlt
    vl_ref[1] = pltpu.roll(vlt, 96, 1)
    cp_finv.wait()
    cp_wo.wait()
    woT_ref[...] = _split_heads_rows(wo_ref[...].astype(F32)).astype(BF).T

    def step5_slab(t):
        sl = pl.ds(pl.multiple_of(t * 128, 128), 128)
        ee = jnp.dot(finv_ref[:, 0:2*RE], g_ref[0:2*RE, sl], preferred_element_type=F32)
        oo = jnp.dot(finv_ref[:, 2*RE:2*R], g_ref[2*RE:2*R, sl], preferred_element_type=F32)
        yT_ref[0:HD, sl] = (ee + oo).astype(BF)
        yT_ref[HD:D, sl] = (ee - oo).astype(BF)

    def finish_store(h, acc, lacc, qt):
        r0 = pl.multiple_of(16 * h, 16)
        oT_ref[pl.ds(r0, 16), qt*TQ:(qt+1)*TQ] = acc
        for r in range(3):
            lr_ref[r, h, :, qt*TQ:(qt+1)*TQ] = lacc[r]

    def fast_heads(t, carry):
        items = [(u, qt, cidx) for u in range(UN) for qt in range(NQ) for cidx in range(NC)]
        vws = {}; ss = {}; accs = {}; laccs = {}
        for u in range(UN):
            r0 = pl.multiple_of(16 * (UN * t + u), 16)
            vws[u] = (vT_ref[pl.ds(r0, 16), :].astype(F32) * (2.0 ** TB)).astype(BF)

        def qk(n):
            u, qt, cidx = items[n]
            h = UN * t + u
            ss[n] = jnp.dot(k_ref[h, cidx*KC:(cidx+1)*KC, 0:32], qT_ref[h, :, qt*TQ:(qt+1)*TQ],
                            preferred_element_type=F32)

        def pv(n):
            u, qt, cidx = items[n]
            vw = vws[u]
            p32 = jnp.exp2(ss.pop(n))
            p = p32.astype(BF)
            d = jnp.dot(vw[:, cidx*KC:(cidx+1)*KC], p, preferred_element_type=F32)
            accs[(u, qt)] = d if cidx == 0 else accs[(u, qt)] + d
            la = laccs.get((u, qt), [None, None, None])
            idx = jnp.full((KC, 128), UN * t + u, jnp.int32)
            vbs = [jnp.take_along_axis(vl_ref[r, cidx*KC:(cidx+1)*KC, :], idx, axis=1) for r in range(2)]
            for gi in range(KC // 8):
                pg = p32[gi*8:(gi+1)*8, :]
                la[2] = pg if la[2] is None else la[2] + pg
                for r in range(2):
                    vb = vbs[r][gi*8:(gi+1)*8, :]
                    term = pg * jnp.concatenate([vb] * (TQ // 128), axis=1)
                    la[r] = term if la[r] is None else la[r] + term
            laccs[(u, qt)] = la
            if cidx == NC - 1:
                finish_store(UN * t + u, accs.pop((u, qt)), laccs.pop((u, qt)), qt)

        for n in range(len(items) + 1):
            if n < len(items):
                qk(n)
            else:
                step5_slab(t)
            if n >= 1:
                pv(n - 1)
        return carry

    def slow_tile(i, carry):
        h = i // (S // SQ)
        q0 = pl.multiple_of((i % (S // SQ)) * SQ, SQ)
        r0 = pl.multiple_of(16 * h, 16)
        l0 = pl.multiple_of(512 + h // 16 * 16, 16)
        off = h % 16
        ones_row = (off + 1) % 16
        row16 = jax.lax.broadcasted_iota(jnp.int32, (16, S), 0)
        vl = vT_ref[pl.ds(l0, 16), :]
        vl = jnp.where(row16 == ones_row, jnp.ones_like(vl), vl)
        vw = jnp.concatenate([vT_ref[pl.ds(r0, 16), :], vl, vT_ref[pl.ds(l0 + 32, 16), :]], axis=0)
        sT = jnp.dot(k_ref[h, :, 0:32], qT_ref[h, :, pl.ds(q0, SQ)], preferred_element_type=F32)
        mx = jnp.max(sT, axis=0, keepdims=True)
        p = jnp.exp2(sT - mx).astype(BF)
        acc = jnp.dot(vw, p, preferred_element_type=F32)
        r16 = jax.lax.broadcasted_iota(jnp.int32, (16, SQ), 0)
        lo = acc[16:32]
        oT_ref[pl.ds(r0, 16), pl.ds(q0, SQ)] = acc[0:16]
        hi = acc[32:48]
        for r, part in enumerate((jnp.where(r16 == off, lo, 0.0), jnp.where(r16 == off, hi, 0.0),
                                  jnp.where(r16 == ones_row, lo, 0.0) * (2.0 ** -TB))):
            lr_ref[r, h, :, pl.ds(q0, SQ)] = part[0:8] + part[8:16]
        return carry

    qmax = jnp.max(am_ref[0])
    kmax = jnp.max(am_ref[1])
    vmax = jnp.max(am_ref[2])
    safe = jnp.logical_and(qmax * kmax * (DH * 1.02) <= TB, vmax <= 2.0 ** 30)

    @pl.when(safe)
    def _():
        jax.lax.fori_loop(0, H // UN, fast_heads, 0)

    @pl.when(jnp.logical_not(safe))
    def _():
        def s5(t, carry):
            step5_slab(t)
            return carry
        jax.lax.fori_loop(0, N1, s5, 0)
        jax.lax.fori_loop(0, H * (S // SQ), slow_tile, 0)

    woT = woT_ref[...]
    cps = []
    for oc in range(S // OC):
        rs = slice(oc*OC, (oc+1)*OC)
        sums = [jnp.sum(lr_ref[r, :, :, rs], axis=1) for r in range(3)]
        inv = 1.0 / (sums[2] * (2.0 ** TB))
        main = (oT_ref[0:512, rs].reshape(H, 16, OC) * inv[:, None, :]).reshape(512, OC)
        on = jnp.concatenate([main, sums[0] * inv, sums[1] * inv], axis=0).astype(BF)
        yT_ref[D:2*D, rs] = jnp.dot(woT, on, preferred_element_type=F32).astype(BF)
        if oc == 0:
            for t_ in range(4):
                ob_ref[:, 128*t_:128*(t_+1)] = yT_ref[128*t_:128*(t_+1), :].T
            cp_oa = pltpu.make_async_copy(ob_ref.at[:, 0:512], o_hbm.at[:, 0:512], out_sems.at[0])
            cp_oa.start()
            cps.append(cp_oa)
        for t_ in range(4, 9):
            ob_ref[rs, 128*t_:128*(t_+1)] = yT_ref[128*t_:128*(t_+1), rs].T
        cp = pltpu.make_async_copy(ob_ref.at[rs, 512:1152], o_hbm.at[rs, 512:1152], out_sems.at[1 + oc])
        cp.start()
        cps.append(cp)
    for cp in cps:
        cp.wait()


_F1, _M, _FINV = _consts()


@jax.jit
def pallas_concat_heads__spectral_gfnet__mha_block__prompt_kernel(A_x, A_w_r, A_w_i, B_x, B_wqkv, B_wo):
    anyspec = pl.BlockSpec(memory_space=pl.ANY)
    out = pl.pallas_call(
        _kernel,
        out_shape=jax.ShapeDtypeStruct((S, 2 * D), BF),
        in_specs=[anyspec] * 9,
        out_specs=anyspec,
        scratch_shapes=[
            pltpu.VMEM((D, S), BF), pltpu.VMEM((DF, S), BF), pltpu.VMEM((DF, S), BF), pltpu.VMEM((D, S), BF),
            pltpu.VMEM((D, 3 * D), BF), pltpu.VMEM((D, D), BF), pltpu.VMEM((2 * R, HD), BF),
            pltpu.VMEM((N1, 256, 256), BF), pltpu.VMEM((HD, 2 * R), BF), pltpu.VMEM((S, 2 * D), BF),
            pltpu.VMEM((H, 32, S), BF), pltpu.VMEM((H, S, 128), BF),
            pltpu.VMEM((D, S), BF), pltpu.VMEM((512, S), F32),
            pltpu.VMEM((2 * R, S), F32), pltpu.VMEM((N1, R, 256), BF), pltpu.VMEM((2 * R, S), BF),
            pltpu.VMEM((2, 3, S, 128), F32), pltpu.VMEM((2, N1, R, 128), F32),
            pltpu.VMEM((S, D), BF), pltpu.VMEM((640 + D, D), BF), pltpu.VMEM((3, 8, 128), F32),
            pltpu.VMEM((2, S, 128), F32), pltpu.VMEM((2 * D, S), BF), pltpu.VMEM((D, 640), BF), pltpu.VMEM((D, D), BF), pltpu.VMEM((3, H, 8, S), F32),
            pltpu.SemaphoreType.DMA((17,)), pltpu.SemaphoreType.DMA((1 + S // OC,)),
        ],
        compiler_params=pltpu.CompilerParams(vmem_limit_bytes=110 << 20),
    )(A_x[0].T, A_w_r.T, A_w_i.T, B_x[0].T, B_wqkv, B_wo, jnp.asarray(_F1), jnp.asarray(_M), jnp.asarray(_FINV))
    return out[None]
```
